```python
import jax
import jax.numpy as jnp

def _softmax(x, axis=-1):
    return jax.nn.softmax(x, axis=axis)

def _gelu(x):
    return jax.nn.gelu(x, approximate=True)

def _silu(x):
    return jax.nn.silu(x)

def _sigmoid(x):
    return jax.nn.sigmoid(x)

def _layernorm(x, axis=-1, eps=1e-05):
    m = jnp.mean(x, axis=axis, keepdims=True)
    v = jnp.var(x, axis=axis, keepdims=True)
    return (x - m) / jnp.sqrt(v + eps)

def _scatter_add(tgt, idx, src, axis=0):
    return tgt.at[idx].add(src)

def _segment_sum(src, seg, n):
    return jax.ops.segment_sum(src, seg, n)

class _Rng:

    def __init__(self, key):
        self._k = key

    def _next(self):
        self._k, sub = jax.random.split(self._k)
        return sub

    def normal(self, shape):
        return jax.random.normal(self._next(), shape, dtype=jnp.bfloat16)

    def randint(self, lo, hi, shape):
        return jax.random.randint(self._next(), shape, lo, hi, dtype=jnp.int32)

    def uniform(self, shape, lo=0.0, hi=1.0):
        return jax.random.uniform(self._next(), shape, jnp.bfloat16, lo, hi)

    def permutation(self, n):
        return jax.random.permutation(self._next(), n)
kernel_name = 'concat_heads__spectral_gfnet__memory_aug_recurrent_mem_tr__prompt'

def setup_inputs():
    _rng = _Rng(jax.random.key(int.from_bytes(__import__("os").urandom(4), "little")))
    _w = lambda a: (lambda t: t.astype(jnp.bfloat16) if jnp.issubdtype(t.dtype, jnp.floating) else t)(jnp.asarray(a))

    def _A_setup():
        B, S, D = (1, 2048, 1024)
        Df = D // 2 + 1
        return {'x': _w((lambda *s: _rng.normal(s) * 0.05)(B, S, D)), 'w_r': _w((lambda *s: _rng.normal(s) * 0.05)(S, Df) * 0.02), 'w_i': _w((lambda *s: _rng.normal(s) * 0.05)(S, Df) * 0.02)}
    _A_in = _A_setup()

    def _B_setup():
        B, S, Dm = (1, 2048, 1024)
        H, Dh = (32, 128)
        M, seg = (8, 32)
        seg = min(seg, S)
        S = S // seg * seg
        return {'x': _w((lambda *s: _rng.normal(s) * 0.05)(B, S, Dm)), 'mem0': _w((lambda *s: _rng.normal(s) * 0.05)(B, M, Dm)), 'Wq': _w((lambda *s: _rng.normal(s) * 0.05)(Dm, H, Dh) * Dm ** (-0.5)), 'Wk': _w((lambda *s: _rng.normal(s) * 0.05)(Dm, H, Dh) * Dm ** (-0.5)), 'Wv': _w((lambda *s: _rng.normal(s) * 0.05)(Dm, H, Dh) * Dm ** (-0.5)), 'Wo': _w((lambda *s: _rng.normal(s) * 0.05)(H, Dh, Dm) * (H * Dh) ** (-0.5)), 'seg_len': seg}
    _B_in = _B_setup()
    return {'A_x': _A_in['x'], 'A_w_r': _A_in['w_r'], 'A_w_i': _A_in['w_i'], 'B_x': _B_in['x'], 'B_mem0': _B_in['mem0'], 'B_Wq': _B_in['Wq'], 'B_Wk': _B_in['Wk'], 'B_Wv': _B_in['Wv'], 'B_Wo': _B_in['Wo'], 'B_seg_len': _B_in['seg_len']}

def reference(A_x, A_w_r, A_w_i, B_x, B_mem0, B_Wq, B_Wk, B_Wv, B_Wo, B_seg_len):

    def _A_ref(x, w_r, w_i):
        B, S, D = x.shape
        X = (lambda x, axes=(-2, -1): jnp.fft.rfft2(x.astype(jnp.float32), axes=axes))(x, axes=(-2, -1))
        W = w_r + 1j * w_i
        X = X * W
        y = (lambda x, s, axes=(-2, -1): jnp.fft.irfft2(x, s=s, axes=axes).astype(jnp.bfloat16))(X, (S, D), axes=(-2, -1))
        return y

    def _B_ref(x, mem0, Wq, Wk, Wv, Wo, seg_len):
        B, S, Dm = x.shape
        H, Dh = (Wq.shape[1], Wq.shape[2])
        M = mem0.shape[1]
        scale = Dh ** (-0.5)
        n_seg = S // seg_len
        L = M + seg_len
        idx = jnp.arange(L)
        mask = (idx[:, None] < M) | (idx[:, None] >= idx[None, :])
        mem = mem0
        outs = []
        for s in range(n_seg):
            xs = x[:, s * seg_len:(s + 1) * seg_len, :].copy()
            h = jnp.concatenate([mem, xs], axis=1)
            q = jnp.einsum('btd,dhe->bhte', h, Wq)
            k = jnp.einsum('btd,dhe->bhte', h, Wk)
            v = jnp.einsum('btd,dhe->bhte', h, Wv)
            scores = jnp.einsum('bhqe,bhke->bhqk', q, k) * scale
            scores = jnp.where(mask[None, None], scores, -1000000000.0)
            p = _softmax(scores, axis=-1)
            o = jnp.einsum('bhqk,bhke->bhqe', p, v)
            o = jnp.einsum('bhte,hed->btd', o, Wo)
            mem = o[:, :M, :].copy()
            outs.append(o[:, M:, :])
        return jnp.concatenate(outs, axis=1)
    a = _A_ref(A_x, A_w_r, A_w_i)
    b = _B_ref(B_x, B_mem0, B_Wq, B_Wk, B_Wv, B_Wo, B_seg_len)
    return jnp.concatenate([a, b], axis=-1)
```

```python
import functools

import jax
import jax.numpy as jnp
import numpy as np
from jax.experimental import pallas as pl
from jax.experimental.pallas import tpu as pltpu

F32 = jnp.float32
BF16 = jnp.bfloat16
U32 = jnp.uint32

S = 2048
D = 1024
H = 32
E = 128
M = 8
LANES = 128
RS = S // LANES
RD = D // LANES
KH = D // 2
KROWS = KH + 8
K_CLASSES = (0, 4, 1, 7, 2, 6, 3, 5)
X_HEAD_SEGS = 8


@functools.lru_cache(maxsize=None)
def _tables():
    bf16 = jnp.dtype(BF16)
    h = np.sqrt(0.5)
    butterfly = np.array([
        [1, 1, 1, 1, 1, 1, 1, 1],
        [1, -1, 1, -1, 1, -1, 1, -1],
        [1, h, 0, -h, -1, -h, 0, h],
        [0, h, 1, h, 0, -h, -1, -h],
        [1, 0, -1, 0, 1, 0, -1, 0],
        [0, 1, 0, -1, 0, 1, 0, -1],
        [1, -h, 0, h, -1, h, 0, -h],
        [0, -h, 1, -h, 0, h, -1, h],
    ], dtype=np.float64)
    norm = (butterfly ** 2).sum(axis=1)
    d = np.arange(D)
    ftab = np.zeros((4, 2 * LANES, 2 * LANES))
    for g in range(4):
        k = np.concatenate([K_CLASSES[2 * g + i] + 8 * np.arange(KH // 8) for i in range(2)])
        ang = 2.0 * np.pi * ((k[:, None] * d[None, :]) % D) / D
        rows = np.concatenate([np.cos(ang), -np.sin(ang)]).reshape(2 * LANES, RD, LANES)
        proj = np.einsum("rjd,cj->rcd", rows, butterfly) / norm[None, :, None]
        ftab[g] = proj[:, 2 * g:2 * g + 2].reshape(2 * LANES, 2 * LANES)
    nyq = np.tile(1.0 - 2.0 * (np.arange(LANES) % 2), (16, 1))
    b = np.arange(LANES)
    ang = 2.0 * np.pi * ((b[:, None] * b[None, :]) % LANES) / LANES
    fr, fi = np.cos(ang), -np.sin(ang)
    f128 = np.block([[fr, fi], [-fi, fr]])
    mats = np.concatenate([ftab.reshape(8 * LANES, 2 * LANES), f128])
    mats = np.stack([mats[:, :LANES], mats[:, LANES:]])
    ang = 2.0 * np.pi * (np.arange(RS)[:, None] * b[None, :]) / S
    tw = np.concatenate([np.cos(ang), -np.sin(ang)])
    tw = np.concatenate([tw, tw * (2.0 / (S * D)), nyq])
    return mats.astype(bf16), tw.astype(np.float32)


def _lo(v):
    return pltpu.bitcast(v << 16, F32)


def _hi(v):
    return pltpu.bitcast(v & np.uint32(0xFFFF0000), F32)


def _dot(a, b):
    return jnp.dot(a, b, preferred_element_type=F32)


def _dot_nt(a, b):
    return jax.lax.dot_general(a, b, (((1,), (1,)), ((), ())), preferred_element_type=F32)


_H8 = float(np.sqrt(0.5))


def _radix8_fwd(x):
    s04, d04 = x[0] + x[4], x[0] - x[4]
    s26, d26 = x[2] + x[6], x[2] - x[6]
    s15, d15 = x[1] + x[5], x[1] - x[5]
    s37, d37 = x[3] + x[7], x[3] - x[7]
    e0, e1 = s04 + s26, s15 + s37
    p, q = (d15 - d37) * _H8, (d15 + d37) * _H8
    return [e0 + e1, e0 - e1, d04 + p, d26 + q, s04 - s26, s15 - s37, d04 - p, d26 - q]


def _radix8_adj(p):
    e0, e1 = p[0] + p[1], p[0] - p[1]
    s04, s26 = e0 + p[4], e0 - p[4]
    s15, s37 = e1 + p[5], e1 - p[5]
    d04, d26 = p[2] + p[6], p[3] + p[7]
    m, n = (p[2] - p[6]) * _H8, (p[3] - p[7]) * _H8
    d15, d37 = m + n, n - m
    return [s04 + d04, s15 + d15, s26 + d26, s37 + d37,
            s04 - d04, s15 - d15, s26 - d26, s37 - d37]


def _cmul(a, b):
    return a[0] * b[0] - a[1] * b[1], a[0] * b[1] + a[1] * b[0]


def _cmul_conj(a, b):
    return a[0] * b[0] + a[1] * b[1], a[1] * b[0] - a[0] * b[1]


def _dft4(z):
    ar, ai = z[0][0] + z[2][0], z[0][1] + z[2][1]
    br, bi = z[0][0] - z[2][0], z[0][1] - z[2][1]
    cr, ci = z[1][0] + z[3][0], z[1][1] + z[3][1]
    dr, di = z[1][0] - z[3][0], z[1][1] - z[3][1]
    return [(ar + cr, ai + ci), (br + di, bi - dr), (ar - cr, ai - ci), (br - di, bi + dr)]


def _rot16(z, n):
    re, im = z
    if n == 0:
        return z
    if n == 4:
        return im, -re
    if n == 2:
        return (re + im) * _H8, (im - re) * _H8
    if n == 6:
        return (im - re) * _H8, (re + im) * (-_H8)
    c, s = float(np.cos(np.pi * n / 8)), float(np.sin(np.pi * n / 8))
    return re * c + im * s, im * c - re * s


def _dft16(z):
    cols = [_dft4([z[n2 + 4 * n1] for n1 in range(4)]) for n2 in range(4)]
    out = [None] * 16
    for k1 in range(4):
        r = _dft4([_rot16(cols[n2][k1], n2 * k1) for n2 in range(4)])
        for k2 in range(4):
            out[k1 + 4 * k2] = r[k2]
    return out


def _idft16(z):
    return [(im, re) for re, im in _dft16([(im, re) for re, im in z])]


def _kernel(ax_hbm, wr_hbm, wi_hbm, bx_hbm, mem_hbm, wq_hbm, wk_hbm, wv_hbm, wo_hbm,
            mats_hbm, tw_hbm, out_hbm,
            xa, wr, wi, mats, tw, ubuf, tbuf, ya,
            raw, wqkv, wo, bx, mem0, hbuf, yb, sems, *, seg, n_seg):
    L = M + seg
    sem_ids = iter(range(sems.shape[0]))

    def copies(pairs):
        sem = sems.at[next(sem_ids)]
        return [pltpu.make_async_copy(src, dst, sem) for src, dst in pairs]

    def start(group):
        for c in group:
            c.start()

    def wait(group):
        for c in group:
            c.wait()

    def col(j):
        return pl.ds(j * LANES, LANES)

    head_rows = X_HEAD_SEGS * seg
    ax32 = ax_hbm.bitcast(U32)
    wo32 = wo_hbm.bitcast(U32)
    cp_tab = copies([(mats_hbm.bitcast(U32), mats), (tw_hbm, tw), (mem_hbm, mem0)])
    cp_ax = copies([(ax32.at[:, col(j)], xa.at[j]) for j in range(RD)])
    cp_w = copies([(src.at[:, col(f)], dst.at[f])
                   for src, dst in ((wr_hbm, wr), (wi_hbm, wi)) for f in range(RS)])
    cp_raw = [copies([(w.bitcast(U32).at[:, pl.ds(8 * g, 8), :], raw.at[m, g])])
              for m, w in enumerate((wq_hbm, wk_hbm, wv_hbm)) for g in range(2)]
    cp_wo = copies([(wo32.at[:, col(j)], wo.at[j]) for j in range(RD)])
    cp_bx0 = copies([(bx_hbm.at[pl.ds(0, head_rows)], bx.at[pl.ds(0, head_rows)])])
    cp_bx1 = copies([(bx_hbm.at[pl.ds(head_rows, S - head_rows)],
                      bx.at[pl.ds(head_rows, S - head_rows)])])
    cp_ya = copies([(ya.at[j], out_hbm.bitcast(U32).at[:, col(j)]) for j in range(RD)])
    yb_sem = sems.at[next(sem_ids)]

    for group in (cp_tab, cp_ax, cp_w, *cp_raw, cp_wo, cp_bx0):
        start(group)

    def table(i):
        rows = pl.ds(i * LANES, LANES)
        return pltpu.bitcast(
            jnp.concatenate([mats[0, rows, :], mats[1, rows, :]], axis=1), BF16)

    wait(cp_tab)
    wait(cp_ax)

    def fwd(ap, carry):
        for c in range(LANES // 16):
            v = [xa[j, pl.ds(ap + 128 * c, 16, stride=8), :] for j in range(RD)]
            for par, half in enumerate((_lo, _hi)):
                u = _radix8_fwd([half(t) for t in v])
                for i in range(RD):
                    ubuf[par, i, pl.ds(8 * c, 8), :] = pltpu.bitcast(u[i].astype(BF16), U32)
        for par in range(2):
            a = 2 * ap + par
            u = [pltpu.bitcast(ubuf[par, i], BF16) for i in range(RD)]
            f128 = table(4)
            for g in range(4):
                y = _dot_nt(table(g), jnp.concatenate(u[2 * g:2 * g + 2], axis=1))
                t = _dot(jnp.concatenate([y[:LANES], y[LANES:]], axis=1), f128)
                tbuf[0, a, pl.ds(g * LANES, LANES), :] = t[:, :LANES]
                tbuf[1, a, pl.ds(g * LANES, LANES), :] = t[:, LANES:]
            y = _dot_nt(tw[pl.ds(4 * RS, 8), :], u[0])
            t = _dot(y, f128[:LANES])
            tbuf[0, a, pl.ds(KH, 8), :] = t[:, :LANES]
            tbuf[1, a, pl.ds(KH, 8), :] = t[:, LANES:]
        return carry

    jax.lax.fori_loop(0, RS // 2, fwd, 0)

    wait(cp_w)

    def tw_row(i):
        return jnp.broadcast_to(tw[pl.ds(i, 1), :], (8, LANES))

    def filter_rows(rows, filt):
        z = [(tbuf[0, a, rows, :], tbuf[1, a, rows, :]) for a in range(RS)]
        z = [z[0]] + [_cmul(z[a], (tw_row(a), tw_row(RS + a))) for a in range(1, RS)]
        z = _dft16(z)
        z = _idft16([_cmul(z[f], filt(f)) for f in range(RS)])
        for a in range(RS):
            if a == 0:
                re, im = z[0][0] * tw_row(2 * RS), z[0][1] * tw_row(2 * RS)
            else:
                re, im = _cmul_conj(z[a], (tw_row(2 * RS + a), tw_row(3 * RS + a)))
            tbuf[0, a, rows, :] = re
            tbuf[1, a, rows, :] = im

    wr32 = wr.at[:, pl.ds(0, KH), :].bitcast(U32)
    wi32 = wi.at[:, pl.ds(0, KH), :].bitcast(U32)
    for pair in range(4):
        def mid(mb, carry, pair=pair):
            block = pl.ds(pl.multiple_of(32 * mb, 32), 32)
            src = pl.ds(pair, 8, stride=4)
            for par, half in enumerate((_lo, _hi)):
                cls = 2 * pair + par
                rows = pl.ds(pl.multiple_of(64 * K_CLASSES.index(cls) + 8 * mb, 8), 8)

                def filt(f, half=half, cls=cls):
                    re = half(wr32.at[f, block][src, :])
                    im = half(wi32.at[f, block][src, :])
                    if cls == 0:
                        sub = jax.lax.broadcasted_iota(jnp.int32, (8, LANES), 0)
                        c = jnp.where(sub + mb == 0, 0.5, 1.0)
                        re, im = re * c, im * c
                    return re, im

                filter_rows(rows, filt)
            return carry

        jax.lax.fori_loop(0, 8, mid, 0)

    def nyq_row(ref, f):
        return jnp.broadcast_to(ref[f, pl.ds(KH, 1), :].astype(F32), (8, LANES))

    filter_rows(pl.ds(KH, 8), lambda f: (nyq_row(wr, f), nyq_row(wi, f)))

    def inv(ap, carry):
        p = []
        for par in range(2):
            a = 2 * ap + par
            f128 = table(4)
            pa = []
            for g in range(4):
                rows = pl.ds(g * LANES, LANES)
                u = jnp.concatenate([tbuf[0, a, rows, :], tbuf[1, a, rows, :]], axis=1)
                v = _dot_nt(f128, u.astype(BF16))
                pg = _dot(jnp.concatenate([v[:LANES], v[LANES:]], axis=1), table(g))
                pa += [pg[:, :LANES], pg[:, LANES:]]
            u = jnp.concatenate([tbuf[0, a, pl.ds(KH, 8), :], tbuf[1, a, pl.ds(KH, 8), :]], axis=1)
            u = jnp.concatenate([u] * (LANES // 8), axis=0).astype(BF16)
            v = _dot_nt(f128[:LANES], u)
            pa[0] = pa[0] + v * (0.5 * tw[pl.ds(4 * RS, 1), :])
            p.append(pa)
        for c in range(LANES // 8):
            rows = slice(8 * c, 8 * c + 8)
            y = [_radix8_adj([t[rows] for t in pa]) for pa in p]
            for j in range(RD):
                ya[j, pl.ds(ap + 64 * c, 8, stride=8), :] = pltpu.pack_elementwise(
                    [y[0][j], y[1][j]], packed_dtype=BF16)
        return carry

    jax.lax.fori_loop(0, RS // 2, inv, 0)

    for i, group in enumerate(cp_raw):
        m, g = divmod(i, 2)
        wait(group)
        src = raw.at[m, g].reshape(D * 8, LANES)

        def repack(kt, carry, m=m, g=g, src=src):
            rows = pl.ds(pl.multiple_of(kt * 64, 64), 64)
            for hp in range(8):
                v = src[pl.ds(kt * 1024 + hp, LANES, stride=8), :]
                for par, half in enumerate((_lo, _hi)):
                    wqkv[m, 16 * g + 2 * hp + par, rows, :] = pltpu.bitcast(
                        half(v).astype(BF16), U32)
            return carry

        jax.lax.fori_loop(0, D // LANES, repack, 0)

    wait(cp_wo)
    wait(cp_bx0)
    start(cp_bx1)
    start(cp_ya)

    hbuf[pl.ds(0, M), :] = mem0[...].astype(F32)
    scale = E ** -0.5

    def yb_copy(s):
        rows = pl.ds(pl.multiple_of(s * seg, seg), seg)
        return pltpu.make_async_copy(yb.at[rows], out_hbm.at[rows, pl.ds(D, D)], yb_sem)

    def segment(s, carry):
        @pl.when(s == X_HEAD_SEGS)
        def _():
            wait(cp_bx1)

        @pl.when(s > 0)
        def _():
            yb_copy(s - 1).start()

        rows = pl.ds(pl.multiple_of(s * seg, seg), seg)
        hbuf[pl.ds(M, seg), :] = bx[rows, :].astype(F32)
        qi = jax.lax.broadcasted_iota(jnp.int32, (L, L), 0)
        ki = jax.lax.broadcasted_iota(jnp.int32, (L, L), 1)
        mask = (qi < M) | (qi >= ki)
        qkv, probs, ctx = {}, {}, {}

        def project(h):
            x = hbuf[...]
            qkv[h] = [_dot(x, pltpu.bitcast(wqkv[m, h], BF16)) for m in range(3)]

        def scores(h):
            q, k, v = qkv.pop(h)
            sc = jnp.where(mask, _dot_nt(q, k) * scale, -1000000000.0)
            e = jnp.exp(sc - jnp.max(sc, axis=-1, keepdims=True))
            probs[h] = e, jnp.sum(e, axis=-1, keepdims=True), v

        def mix(h):
            e, l, v = probs.pop(h)
            ctx[h] = _dot(e, v) * (1.0 / l)

        def output(h):
            w = jnp.concatenate(
                [wo[j, pl.ds(h * (E // 2), E // 2), :] for j in range(RD)], axis=1)
            return _dot(ctx.pop(h), pltpu.bitcast(w, BF16))

        acc = None
        for t in range(H + 4):
            if t < H:
                project(t)
            if 0 <= t - 1 < H:
                scores(t - 1)
            if 0 <= t - 2 < H:
                mix(t - 2)
            if 0 <= t - 4 < H:
                y = output(t - 4)
                acc = y if acc is None else acc + y
        hbuf[pl.ds(0, M), :] = acc[:M]
        yb[rows, :] = acc[M:].astype(BF16)
        return carry

    jax.lax.fori_loop(0, n_seg, segment, 0)
    yb_copy(n_seg - 1).start()
    wait(cp_ya)
    pltpu.make_async_copy(yb, out_hbm.at[:, pl.ds(D, D)], yb_sem).wait()


@functools.partial(jax.jit, static_argnames=("B_seg_len",))
def pallas_concat_heads__spectral_gfnet__memory_aug_recurrent_mem_tr__prompt_kernel(
    A_x: jax.Array,
    A_w_r: jax.Array,
    A_w_i: jax.Array,
    B_x: jax.Array,
    B_mem0: jax.Array,
    B_Wq: jax.Array,
    B_Wk: jax.Array,
    B_Wv: jax.Array,
    B_Wo: jax.Array,
    B_seg_len: int,
):
    assert A_x.shape == (1, S, D) and B_x.shape == (1, S, D) and B_mem0.shape == (1, M, D)
    assert B_Wq.shape == (D, H, E) and B_Wo.shape == (H, E, D)
    seg = int(B_seg_len)
    n_seg = S // seg
    assert seg % 16 == 0 and n_seg * seg == S and n_seg > X_HEAD_SEGS
    mats, tw = _tables()
    vmem = pltpu.VMEM
    out = pl.pallas_call(
        functools.partial(_kernel, seg=seg, n_seg=n_seg),
        out_shape=jax.ShapeDtypeStruct((S, 2 * D), BF16),
        in_specs=[pl.BlockSpec(memory_space=pl.ANY)] * 11,
        out_specs=pl.BlockSpec(memory_space=pl.ANY),
        scratch_shapes=[
            vmem((RD, S // 2, LANES), U32),
            vmem((RS, KH + 1, LANES), BF16),
            vmem((RS, KH + 1, LANES), BF16),
            vmem((2, mats.shape[1] // 2, LANES), U32),
            vmem(tw.shape, F32),
            vmem((2, RD, LANES // 2, LANES), U32),
            vmem((2, RS, KROWS, LANES), F32),
            vmem((RD, S // 2, LANES), U32),
            vmem((3, 2, D, 8, LANES), U32),
            vmem((3, H, D // 2, LANES), U32),
            vmem((RD, H * E // 2, LANES), U32),
            vmem((S, D), BF16),
            vmem((M, D), BF16),
            vmem((M + seg, D), F32),
            vmem((S, D), BF16),
            pltpu.SemaphoreType.DMA((16,)),
        ],
        compiler_params=pltpu.CompilerParams(vmem_limit_bytes=112 * 1024 * 1024),
        name="gfnet_rmt",
    )(A_x.reshape(S, D), A_w_r.T, A_w_i.T, B_x.reshape(S, D), B_mem0.reshape(M, D),
      B_Wq, B_Wk, B_Wv, B_Wo.reshape(H * E, D), mats, tw)
    return out.reshape(1, S, 2 * D)
```

```python
import functools

import jax
import jax.numpy as jnp
import numpy as np
from jax.experimental import pallas as pl
from jax.experimental.pallas import tpu as pltpu

F32 = jnp.float32
BF16 = jnp.bfloat16
U32 = jnp.uint32

S = 2048
D = 1024
H = 32
E = 128
M = 8
LANES = 128
RS = S // LANES
RD = D // LANES
KH = D // 2
KROWS = KH + 8
K_CLASSES = (0, 4, 1, 7, 2, 6, 3, 5)
_ROOT_NORM = 2.0 ** -10
TW_ROW = 2 * LANES
NYQ_ROW = TW_ROW + 2 * RS
X_CHUNKS = 4
WO_CHUNKS = 4


@functools.lru_cache(maxsize=None)
def _tables():
    bf16 = jnp.dtype(BF16)
    h = np.sqrt(0.5)
    butterfly = np.array([
        [1, 1, 1, 1, 1, 1, 1, 1],
        [1, -1, 1, -1, 1, -1, 1, -1],
        [1, h, 0, -h, -1, -h, 0, h],
        [0, h, 1, h, 0, -h, -1, -h],
        [1, 0, -1, 0, 1, 0, -1, 0],
        [0, 1, 0, -1, 0, 1, 0, -1],
        [1, -h, 0, h, -1, h, 0, -h],
        [0, -h, 1, -h, 0, h, -1, h],
    ], dtype=np.float64)
    norm = (butterfly ** 2).sum(axis=1)
    d = np.arange(D)
    ftab = np.zeros((4, 2 * LANES, 2 * LANES))
    for g in range(4):
        k = np.concatenate([K_CLASSES[2 * g + i] + 8 * np.arange(KH // 8) for i in range(2)])
        ang = 2.0 * np.pi * ((k[:, None] * d[None, :]) % D) / D
        rows = np.concatenate([np.cos(ang), -np.sin(ang)]).reshape(2 * LANES, RD, LANES)
        proj = np.einsum("rjd,cj->rcd", rows, butterfly) / norm[None, :, None]
        ftab[g] = proj[:, 2 * g:2 * g + 2].reshape(2 * LANES, 2 * LANES)
    ftab = ftab.reshape(8 * LANES, 2 * LANES) * _ROOT_NORM
    mats = np.stack([ftab[:, :LANES], ftab[:, LANES:]])
    nyq = np.tile(1.0 - 2.0 * (np.arange(LANES) % 2), (8, 1)) * _ROOT_NORM
    b = np.arange(LANES)
    ang = 2.0 * np.pi * ((b[:, None] * b[None, :]) % LANES) / LANES
    twang = 2.0 * np.pi * (np.arange(RS)[:, None] * b[None, :]) / S
    tw = np.concatenate([np.cos(ang), -np.sin(ang), np.cos(twang), -np.sin(twang), nyq])
    return mats.astype(bf16), tw.astype(np.float32)


def _lo(v):
    return pltpu.bitcast(v << 16, F32)


def _hi(v):
    return pltpu.bitcast(v & np.uint32(0xFFFF0000), F32)


def _dot(a, b):
    return jnp.dot(a, b, preferred_element_type=F32)


def _dot_nt(a, b):
    return jax.lax.dot_general(a, b, (((1,), (1,)), ((), ())), preferred_element_type=F32)


_H8 = float(np.sqrt(0.5))


def _radix8_fwd(x):
    s04, d04 = x[0] + x[4], x[0] - x[4]
    s26, d26 = x[2] + x[6], x[2] - x[6]
    s15, d15 = x[1] + x[5], x[1] - x[5]
    s37, d37 = x[3] + x[7], x[3] - x[7]
    e0, e1 = s04 + s26, s15 + s37
    p, q = (d15 - d37) * _H8, (d15 + d37) * _H8
    return [e0 + e1, e0 - e1, d04 + p, d26 + q, s04 - s26, s15 - s37, d04 - p, d26 - q]


def _radix8_adj(p):
    e0, e1 = p[0] + p[1], p[0] - p[1]
    s04, s26 = e0 + p[4], e0 - p[4]
    s15, s37 = e1 + p[5], e1 - p[5]
    d04, d26 = p[2] + p[6], p[3] + p[7]
    m, n = (p[2] - p[6]) * _H8, (p[3] - p[7]) * _H8
    d15, d37 = m + n, n - m
    return [s04 + d04, s15 + d15, s26 + d26, s37 + d37,
            s04 - d04, s15 - d15, s26 - d26, s37 - d37]


def _cmul(a, b):
    return a[0] * b[0] - a[1] * b[1], a[0] * b[1] + a[1] * b[0]


def _cmul_conj(a, b):
    return a[0] * b[0] + a[1] * b[1], a[1] * b[0] - a[0] * b[1]


def _dft4(z):
    ar, ai = z[0][0] + z[2][0], z[0][1] + z[2][1]
    br, bi = z[0][0] - z[2][0], z[0][1] - z[2][1]
    cr, ci = z[1][0] + z[3][0], z[1][1] + z[3][1]
    dr, di = z[1][0] - z[3][0], z[1][1] - z[3][1]
    return [(ar + cr, ai + ci), (br + di, bi - dr), (ar - cr, ai - ci), (br - di, bi + dr)]


def _rot16(z, n):
    re, im = z
    if n == 0:
        return z
    if n == 4:
        return im, -re
    if n == 2:
        return (re + im) * _H8, (im - re) * _H8
    if n == 6:
        return (im - re) * _H8, (re + im) * (-_H8)
    c, s = float(np.cos(np.pi * n / 8)), float(np.sin(np.pi * n / 8))
    return re * c + im * s, im * c - re * s


def _dft16(z):
    cols = [_dft4([z[n2 + 4 * n1] for n1 in range(4)]) for n2 in range(4)]
    out = [None] * 16
    for k1 in range(4):
        r = _dft4([_rot16(cols[n2][k1], n2 * k1) for n2 in range(4)])
        for k2 in range(4):
            out[k1 + 4 * k2] = r[k2]
    return out


def _idft16(z):
    return [(im, re) for re, im in _dft16([(im, re) for re, im in z])]


def _kernel(ax_hbm, wr_hbm, wi_hbm, bx3_hbm, mem_hbm, wq_hbm, wk_hbm, wv_hbm, wo_hbm,
            mats_hbm, tw_hbm, out_hbm,
            xa, wr, wi, mats, tw, ftw, ubuf, tbuf, ya,
            raw, w_early, w_late, wo_raw, wo, bx, mem0, hbuf, yb, xpre_raw, xpre, pre, sems, raw_sems, *, seg, n_seg):
    L = M + seg
    unroll = 3
    assert (n_seg - 1) % unroll == 0
    sem_ids = iter(range(sems.shape[0]))

    def copies(pairs):
        sem = sems.at[next(sem_ids)]
        return [pltpu.make_async_copy(src, dst, sem) for src, dst in pairs]

    def start(group):
        for c in group:
            c.start()

    def wait(group):
        for c in group:
            c.wait()

    def col(j):
        return pl.ds(j * LANES, LANES)

    head_segs = 1 + unroll
    wo_rows = H * E // WO_CHUNKS
    ax32 = ax_hbm.bitcast(U32)
    cp_tab = copies([(mats_hbm.bitcast(U32), mats), (tw_hbm, tw)])
    x_rows32 = S // 2 // X_CHUNKS
    cp_ax = [copies([(ax32.at[pl.ds(q * x_rows32, x_rows32), col(j)],
                      xa.at[j, pl.ds(q * x_rows32, x_rows32)]) for j in range(RD)])
             for q in range(X_CHUNKS)]
    cp_w = copies([(src.at[:, col(f)], dst.at[f])
                   for src, dst in ((wr_hbm, wr), (wi_hbm, wi)) for f in range(RS)])
    cp_bx0 = copies([(bx3_hbm.at[pl.ds(0, head_segs)], bx.at[pl.ds(0, head_segs)]),
                     (mem_hbm, mem0)])
    cp_raw = [[pltpu.make_async_copy(
        (wq_hbm, wk_hbm, wv_hbm)[p % 3].bitcast(U32).at[:, pl.ds(8 * (p // 3), 8), :],
        raw.at[p], raw_sems.at[p])] for p in range(6)]
    cp_xpre = copies([(bx3_hbm.at[:, pl.ds(seg - 8, 8), :], xpre_raw)])
    cp_wo = [copies([(wo_hbm.at[pl.ds(c * wo_rows, wo_rows)],
                      wo_raw.at[pl.ds(c * wo_rows, wo_rows)])]) for c in range(WO_CHUNKS)]
    cp_bx1 = copies([(bx3_hbm.at[pl.ds(head_segs, n_seg - head_segs)],
                      bx.at[pl.ds(head_segs, n_seg - head_segs)])])
    cp_ya = copies([(ya.at[j], out_hbm.bitcast(U32).at[:, col(j)]) for j in range(RD)])
    yb_sem = sems.at[next(sem_ids)]

    for group in (cp_tab, *cp_ax, cp_w, cp_xpre, *cp_raw, cp_bx0):
        start(group)
    for group in cp_wo:
        for c in group:
            c.start(priority=1)

    def table(i):
        rows = pl.ds(i * LANES, LANES)
        return pltpu.bitcast(
            jnp.concatenate([mats[0, rows, :], mats[1, rows, :]], axis=1), BF16)

    def pipelined(items, first, second, lag):
        pending = []
        for item in items:
            pending.append((item, first(item)))
            if len(pending) > lag:
                second(*pending.pop(0))
        for p in pending:
            second(*p)

    wait(cp_tab)

    def twiddled_dft(a, carry):
        fr, fi = tw[pl.ds(0, LANES), :], tw[pl.ds(LANES, LANES), :]
        re, im = _cmul((fr, fi), (tw[pl.ds(TW_ROW + a, 1), :], tw[pl.ds(TW_ROW + RS + a, 1), :]))
        ftw[a, 0], ftw[a, 1], ftw[a, 2] = re, im, -im
        return carry

    jax.lax.fori_loop(0, RS, twiddled_dft, 0)

    def sequence_matrix(a):
        return jnp.concatenate([jnp.concatenate([ftw[a, 0], ftw[a, 1]], axis=1),
                                jnp.concatenate([ftw[a, 2], ftw[a, 0]], axis=1)], axis=0)

    for q in range(X_CHUNKS):
        wait(cp_ax[q])

        def butterflies(ap, carry, q=q):
            n = LANES // X_CHUNKS
            for b in range(q * n, (q + 1) * n, 8):
                v = [xa[j, pl.ds(ap + 8 * b, 8, stride=8), :] for j in range(RD)]
                for par, half in enumerate((_lo, _hi)):
                    u = _radix8_fwd([half(t) for t in v])
                    for i in range(RD):
                        ubuf[2 * ap + par, i, pl.ds(b, 8), :] = u[i]
            return carry

        jax.lax.fori_loop(0, RS // 2, butterflies, 0)

    def fwd(ap, carry):
        def feature_dft(item):
            a, g = item
            if g == 4:
                return _dot_nt(tw[pl.ds(NYQ_ROW, 8), :], ubuf[a, 0])
            u = jnp.concatenate([ubuf[a, 2 * g], ubuf[a, 2 * g + 1]], axis=1)
            return _dot_nt(table(g), u)

        def sequence_dft(item, y):
            a, g = item
            f = sequence_matrix(a)
            if g == 4:
                rows, t = pl.ds(KH, 8), _dot(y, f[:LANES])
            else:
                rows = pl.ds(g * LANES, LANES)
                t = _dot(jnp.concatenate([y[:LANES], y[LANES:]], axis=1), f)
            tbuf[0, a, rows, :] = t[:, :LANES]
            tbuf[1, a, rows, :] = t[:, LANES:]

        pipelined([(2 * ap + par, g) for par in range(2) for g in range(5)],
                  feature_dft, sequence_dft, 1)
        return carry

    jax.lax.fori_loop(0, RS // 2, fwd, 0)

    wait(cp_w)

    def filter_rows(rows, filt):
        z = _dft16([(tbuf[0, a, rows, :], tbuf[1, a, rows, :]) for a in range(RS)])
        z = _idft16([_cmul(z[f], filt(f)) for f in range(RS)])
        for a in range(RS):
            tbuf[0, a, rows, :], tbuf[1, a, rows, :] = z[a]

    wr32 = wr.at[:, pl.ds(0, KH), :].bitcast(U32)
    wi32 = wi.at[:, pl.ds(0, KH), :].bitcast(U32)
    for pair in range(4):
        def mid(mb, carry, pair=pair):
            block = pl.ds(pl.multiple_of(32 * mb, 32), 32)
            src = pl.ds(pair, 8, stride=4)
            for par, half in enumerate((_lo, _hi)):
                cls = 2 * pair + par
                rows = pl.ds(pl.multiple_of(64 * K_CLASSES.index(cls) + 8 * mb, 8), 8)

                def filt(f, half=half, cls=cls):
                    re = half(wr32.at[f, block][src, :])
                    im = half(wi32.at[f, block][src, :])
                    if cls == 0:
                        sub = jax.lax.broadcasted_iota(jnp.int32, (8, LANES), 0)
                        c = jnp.where(sub + mb == 0, 0.5, 1.0)
                        re, im = re * c, im * c
                    return re, im

                filter_rows(rows, filt)
            return carry

        jax.lax.fori_loop(0, 8, mid, 0)

    def nyq_row(ref, f):
        return jnp.broadcast_to(ref[f, pl.ds(KH, 1), :].astype(F32), (8, LANES))

    filter_rows(pl.ds(KH, 8), lambda f: (nyq_row(wr, f), nyq_row(wi, f)))

    def repack(p, kt, dst, unit):
        src = raw.at[p].reshape(D * 8, LANES)
        rows = pl.ds(pl.multiple_of(kt * 64, 64), 64)
        for hp in range(8):
            v = src[pl.ds(kt * 8 * LANES + hp, LANES, stride=8), :]
            for par, half in enumerate((v, v >> 16)):
                dst[unit + 2 * hp + par, rows, :] = pltpu.bitcast(half.astype(jnp.uint16), U32)

    def finish(ap):
        for b in range(0, LANES, 8):
            y = [_radix8_adj([ubuf[2 * ap + par, i, pl.ds(b, 8), :] for i in range(RD)])
                 for par in range(2)]
            for j in range(RD):
                ya[j, pl.ds(ap + 8 * b, 8, stride=8), :] = pltpu.pack_elementwise(
                    [y[0][j], y[1][j]], packed_dtype=BF16)

    def inv(ap, carry):
        for p in range(2):
            repack(p, ap, w_early, 16 * p)

        def sequence_idft(item):
            par, g = item
            a = 2 * ap + par
            rows = pl.ds(KH, 8) if g == 4 else pl.ds(g * LANES, LANES)
            u = jnp.concatenate([tbuf[0, a, rows, :], tbuf[1, a, rows, :]], axis=1)
            if g == 4:
                u = jnp.concatenate([u] * (LANES // 8), axis=0)
                return _dot_nt(sequence_matrix(a)[:LANES], u)
            return _dot_nt(sequence_matrix(a), u)

        nyquist = {}

        def feature_idft(item, v):
            par, g = item
            if g == 4:
                nyquist[par] = v * (0.5 * tw[pl.ds(NYQ_ROW, 1), :])
                return
            p = _dot(jnp.concatenate([v[:LANES], v[LANES:]], axis=1), table(g))
            a = 2 * ap + par
            ubuf[a, 2 * g] = p[:, :LANES] + nyquist.pop(par) if g == 0 else p[:, :LANES]
            ubuf[a, 2 * g + 1] = p[:, LANES:]

        pipelined([(par, g) for par in range(2) for g in (4, 0, 1, 2, 3)],
                  sequence_idft, feature_idft, 1)
        return carry

    wait(cp_raw[0])
    wait(cp_raw[1])
    jax.lax.fori_loop(0, RS // 2, inv, 0)

    scale = E ** -0.5
    x_rows, mem_rows = pl.ds(0, seg), pl.ds(seg, M)

    def yb_copy(s, n):
        rows = pl.ds(pl.multiple_of(s * seg, seg), n * seg)
        return pltpu.make_async_copy(yb.at[rows], out_hbm.at[rows, pl.ds(D, D)], yb_sem)

    wait(cp_xpre)

    def widen(i, carry):
        xpre[pl.ds(pl.multiple_of(32 * i, 32), 32), :] = pltpu.bitcast(
            xpre_raw[pl.ds(8 * i, 8)].reshape(64, D), U32)
        return carry

    jax.lax.fori_loop(0, n_seg // 8, widen, 0)

    def precompute(unit):
        pre[unit] = _dot(pltpu.bitcast(xpre[...], BF16), pltpu.bitcast(w_early[unit], BF16))

    def late(i, carry):
        p = 2 + i
        pltpu.make_async_copy(raw.at[p], raw.at[p], raw_sems.at[p]).wait()
        per = pre.shape[0] // 4
        for unit in range(per):
            precompute(per * i + unit)
        for kt in range(8):
            repack(p, kt, w_late, 16 * i)
        finish(2 * i)
        finish(2 * i + 1)
        return carry

    jax.lax.fori_loop(0, 4, late, 0)

    def retile(h):
        if h % (H // WO_CHUNKS) == 0:
            wait(cp_wo[h // (H // WO_CHUNKS)])
        wo[h] = pltpu.bitcast(wo_raw[pl.ds(h * E, E), :], U32)

    def segment(s, first=False):
        rows = pl.ds(pl.multiple_of(s * seg, seg), seg)
        hbuf[x_rows, :] = bx[s].astype(F32)
        qi = jax.lax.broadcasted_iota(jnp.int32, (L, L), 0)
        ki = jax.lax.broadcasted_iota(jnp.int32, (L, L), 1)
        mask = (qi >= seg) | (ki >= seg) | (qi >= ki)
        qkv, probs, ctx = {}, {}, {}

        def project(h):
            qkv[h] = []
            for m in range(3):
                unit = 16 * (3 * (h // 16) + m) + h % 16
                w = pltpu.bitcast(w_early[unit] if unit < 32 else w_late[unit - 32], BF16)
                if unit < pre.shape[0]:
                    x = jnp.concatenate([hbuf[pl.ds(0, seg - 8), :], hbuf[mem_rows, :]], axis=0)
                    r = _dot(x, w)
                    done = pre[unit, pl.ds(pl.multiple_of(8 * s, 8), 8), :]
                    qkv[h].append(jnp.concatenate([r[:seg - 8], done, r[seg - 8:]], axis=0))
                else:
                    qkv[h].append(_dot(hbuf[...], w))

        def scores(h):
            q, k, v = qkv.pop(h)
            sc = jnp.where(mask, _dot_nt(q, k) * scale, -1000000000.0)
            e = jnp.exp(sc - jnp.max(sc, axis=-1, keepdims=True))
            probs[h] = e, jnp.sum(e, axis=-1, keepdims=True), v

        def mix(h):
            e, l, v = probs.pop(h)
            o = _dot(e, v) * (1.0 / l)
            ctx[h] = jnp.concatenate([o[seg:], o[:seg]], axis=0)

        lag_s, lag_m, lag_o = 2, 5, 7
        if first:
            lag_o = H + lag_m
        acc = None
        for t in range(H + lag_o):
            if t < H:
                project(t)
            if 0 <= t - lag_s < H:
                scores(t - lag_s)
            if 0 <= t - lag_m < H:
                mix(t - lag_m)
            if 0 <= t - lag_o < H:
                if first:
                    retile(t - lag_o)
                y = _dot(ctx.pop(t - lag_o), pltpu.bitcast(wo[t - lag_o], BF16))
                acc = y if acc is None else acc + y
        hbuf[mem_rows, :] = acc[:M]
        yb[rows, :] = acc[M:].astype(BF16)

    wait(cp_bx0)
    hbuf[mem_rows, :] = mem0[...].astype(F32)
    segment(0, first=True)
    start(cp_bx1)
    start(cp_ya)
    yb_copy(0, 1).start()

    def segments(i, carry):
        s0 = 1 + i * unroll

        @pl.when(i == 1)
        def _():
            wait(cp_bx1)

        @pl.when(i > 0)
        def _():
            yb_copy(s0 - unroll, unroll).start()

        for u in range(unroll):
            segment(s0 + u)
        return carry

    jax.lax.fori_loop(0, (n_seg - 1) // unroll, segments, 0)
    yb_copy(n_seg - unroll, unroll).start()
    wait(cp_ya)
    pltpu.make_async_copy(yb, out_hbm.at[:, pl.ds(D, D)], yb_sem).wait()


@functools.partial(jax.jit, static_argnames=("B_seg_len",))
def pallas_concat_heads__spectral_gfnet__memory_aug_recurrent_mem_tr__prompt_kernel(
    A_x: jax.Array,
    A_w_r: jax.Array,
    A_w_i: jax.Array,
    B_x: jax.Array,
    B_mem0: jax.Array,
    B_Wq: jax.Array,
    B_Wk: jax.Array,
    B_Wv: jax.Array,
    B_Wo: jax.Array,
    B_seg_len: int,
):
    assert A_x.shape == (1, S, D) and B_x.shape == (1, S, D) and B_mem0.shape == (1, M, D)
    assert B_Wq.shape == (D, H, E) and B_Wo.shape == (H, E, D)
    seg = int(B_seg_len)
    n_seg = S // seg
    assert seg % 16 == 0 and n_seg * seg == S
    mats, tw = _tables()
    vmem = pltpu.VMEM
    out = pl.pallas_call(
        functools.partial(_kernel, seg=seg, n_seg=n_seg),
        out_shape=jax.ShapeDtypeStruct((S, 2 * D), BF16),
        in_specs=[pl.BlockSpec(memory_space=pl.ANY)] * 11,
        out_specs=pl.BlockSpec(memory_space=pl.ANY),
        scratch_shapes=[
            vmem((RD, S // 2, LANES), U32),
            vmem((RS, KH + 1, LANES), BF16),
            vmem((RS, KH + 1, LANES), BF16),
            vmem((2, mats.shape[1] // 2, LANES), U32),
            vmem(tw.shape, F32),
            vmem((RS, 3, LANES, LANES), F32),
            vmem((RS, RD, LANES, LANES), F32),
            vmem((2, RS, KROWS, LANES), F32),
            vmem((RD, S // 2, LANES), U32),
            vmem((6, D, 8, LANES), U32),
            vmem((32, D // 2, LANES), U32),
            vmem((64, D // 2, LANES), U32),
            vmem((H * E, D), BF16),
            vmem((H, E // 2, D), U32),
            vmem((n_seg, seg, D), BF16),
            vmem((M, D), BF16),
            vmem((M + seg, D), F32),
            vmem((S, D), BF16),
            vmem((n_seg, 8, D), BF16),
            vmem((4 * n_seg, D), U32),
            vmem((12, 8 * n_seg, LANES), F32),
            pltpu.SemaphoreType.DMA((24,)),
            pltpu.SemaphoreType.DMA((6,)),
        ],
        compiler_params=pltpu.CompilerParams(vmem_limit_bytes=120 * 1024 * 1024),
        name="gfnet_rmt",
    )(A_x.reshape(S, D), A_w_r.T, A_w_i.T, B_x.reshape(n_seg, seg, D), B_mem0.reshape(M, D),
      B_Wq, B_Wk, B_Wv, B_Wo.reshape(H * E, D), mats, tw)
    return out.reshape(1, S, 2 * D)
```

```python
import functools

import jax
import jax.numpy as jnp
import numpy as np
from jax.experimental import pallas as pl
from jax.experimental.pallas import tpu as pltpu

F32 = jnp.float32
BF16 = jnp.bfloat16
U32 = jnp.uint32

S = 2048
D = 1024
H = 32
E = 128
M = 8
LANES = 128
RS = S // LANES
RD = D // LANES
KH = D // 2
KROWS = KH + 8
K_CLASSES = (0, 4, 1, 7, 2, 6, 5, 3)
_ROOT_NORM = 2.0 ** -10
TW_ROW = 2 * LANES
NYQ_ROW = TW_ROW + 2 * RS
CLASS_SIGN = (-1.0, 1.0)
X_CHUNKS = 4
WO_CHUNKS = 4


@functools.lru_cache(maxsize=None)
def _tables():
    bf16 = jnp.dtype(BF16)
    h = np.sqrt(0.5)
    butterfly = np.array([
        [1, 1, 1, 1, 1, 1, 1, 1],
        [1, -1, 1, -1, 1, -1, 1, -1],
        [1, h, 0, -h, -1, -h, 0, h],
        [0, h, 1, h, 0, -h, -1, -h],
        [1, 0, -1, 0, 1, 0, -1, 0],
        [0, 1, 0, -1, 0, 1, 0, -1],
        [1, -h, 0, h, -1, h, 0, -h],
        [0, -h, 1, -h, 0, h, -1, h],
    ], dtype=np.float64)
    norm = (butterfly ** 2).sum(axis=1)
    d = np.arange(D)
    half = LANES // 2
    mats = []
    for g in range(4):
        k = np.concatenate([K_CLASSES[2 * g + i] + 8 * np.arange(KH // 8) for i in range(2)])
        ang = 2.0 * np.pi * ((k[:, None] * d[None, :]) % D) / D
        rows = np.concatenate([np.cos(ang), -np.sin(ang)]).reshape(2 * LANES, RD, LANES)
        proj = np.einsum("rjd,cj->rcd", rows, butterfly) / norm[None, :, None]
        p, q = proj[:LANES, 2 * g], proj[:LANES, 2 * g + 1]
        r, t = proj[LANES:, 2 * g], proj[LANES:, 2 * g + 1]
        if g == 0:
            mats += [np.concatenate([p[:half], r[:half]]), np.concatenate([q[half:], t[half:]])]
        else:
            sign = np.repeat(CLASS_SIGN, half)[:, None]
            assert np.allclose(t, sign * p) and np.allclose(q, -sign * r)
            mats += [p, r - sign * p, p + sign * r]
    mats = np.concatenate(mats) * _ROOT_NORM
    nyq = np.tile(1.0 - 2.0 * (np.arange(LANES) % 2), (8, 1)) * _ROOT_NORM
    b = np.arange(LANES)
    ang = 2.0 * np.pi * ((b[:, None] * b[None, :]) % LANES) / LANES
    twang = 2.0 * np.pi * (np.arange(RS)[:, None] * b[None, :]) / S
    tw = np.concatenate([np.cos(ang), -np.sin(ang), np.cos(twang), -np.sin(twang), nyq])
    return mats.astype(bf16), tw.astype(np.float32)


def _lo(v):
    return pltpu.bitcast(v << 16, F32)


def _hi(v):
    return pltpu.bitcast(v & np.uint32(0xFFFF0000), F32)


def _dot(a, b):
    return jnp.dot(a, b, preferred_element_type=F32)


def _dot_nt(a, b):
    return jax.lax.dot_general(a, b, (((1,), (1,)), ((), ())), preferred_element_type=F32)


_H8 = float(np.sqrt(0.5))


def _radix8_fwd(x):
    s04, d04 = x[0] + x[4], x[0] - x[4]
    s26, d26 = x[2] + x[6], x[2] - x[6]
    s15, d15 = x[1] + x[5], x[1] - x[5]
    s37, d37 = x[3] + x[7], x[3] - x[7]
    e0, e1 = s04 + s26, s15 + s37
    p, q = (d15 - d37) * _H8, (d15 + d37) * _H8
    return [e0 + e1, e0 - e1, d04 + p, d26 + q, s04 - s26, s15 - s37, d04 - p, d26 - q]


def _radix8_adj(p):
    e0, e1 = p[0] + p[1], p[0] - p[1]
    s04, s26 = e0 + p[4], e0 - p[4]
    s15, s37 = e1 + p[5], e1 - p[5]
    d04, d26 = p[2] + p[6], p[3] + p[7]
    m, n = (p[2] - p[6]) * _H8, (p[3] - p[7]) * _H8
    d15, d37 = m + n, n - m
    return [s04 + d04, s15 + d15, s26 + d26, s37 + d37,
            s04 - d04, s15 - d15, s26 - d26, s37 - d37]


def _cmul(a, b):
    return a[0] * b[0] - a[1] * b[1], a[0] * b[1] + a[1] * b[0]


def _cmul_conj(a, b):
    return a[0] * b[0] + a[1] * b[1], a[1] * b[0] - a[0] * b[1]


def _dft4(z):
    ar, ai = z[0][0] + z[2][0], z[0][1] + z[2][1]
    br, bi = z[0][0] - z[2][0], z[0][1] - z[2][1]
    cr, ci = z[1][0] + z[3][0], z[1][1] + z[3][1]
    dr, di = z[1][0] - z[3][0], z[1][1] - z[3][1]
    return [(ar + cr, ai + ci), (br + di, bi - dr), (ar - cr, ai - ci), (br - di, bi + dr)]


def _rot16(z, n):
    re, im = z
    if n == 0:
        return z
    if n == 4:
        return im, -re
    if n == 2:
        return (re + im) * _H8, (im - re) * _H8
    if n == 6:
        return (im - re) * _H8, (re + im) * (-_H8)
    c, s = float(np.cos(np.pi * n / 8)), float(np.sin(np.pi * n / 8))
    return re * c + im * s, im * c - re * s


def _dft16(z):
    cols = [_dft4([z[n2 + 4 * n1] for n1 in range(4)]) for n2 in range(4)]
    out = [None] * 16
    for k1 in range(4):
        r = _dft4([_rot16(cols[n2][k1], n2 * k1) for n2 in range(4)])
        for k2 in range(4):
            out[k1 + 4 * k2] = r[k2]
    return out


def _idft16(z):
    return [(im, re) for re, im in _dft16([(im, re) for re, im in z])]


def _kernel(ax_hbm, wr_hbm, wi_hbm, bx3_hbm, mem_hbm, wq_hbm, wk_hbm, wv_hbm, wo_hbm,
            mats_hbm, tw_hbm, out_hbm,
            xa, wr, wi, mats, tw, ftw, ubuf, tbuf, ya,
            raw, w_a, w_b, w_c, wo, bx, mem0, hbuf, yb, xpre_raw, xpre, pre, sems, raw_sems, *, seg, n_seg):
    L = M + seg
    unroll = 4
    assert n_seg % unroll == 0
    sem_ids = iter(range(sems.shape[0]))

    def copies(pairs):
        sem = sems.at[next(sem_ids)]
        return [pltpu.make_async_copy(src, dst, sem) for src, dst in pairs]

    def start(group):
        for c in group:
            c.start()

    def wait(group):
        for c in group:
            c.wait()

    def col(j):
        return pl.ds(j * LANES, LANES)

    head_segs = unroll
    ax32 = ax_hbm.bitcast(U32)
    cp_tab = copies([(mats_hbm.bitcast(U32), mats), (tw_hbm, tw)])
    x_rows32 = S // 2 // X_CHUNKS
    cp_ax = [copies([(ax32.at[pl.ds(q * x_rows32, x_rows32), col(j)],
                      xa.at[j, pl.ds(q * x_rows32, x_rows32)]) for j in range(RD)])
             for q in range(X_CHUNKS)]
    cp_w = copies([(src.at[:, col(f)], dst.at[f])
                   for src, dst in ((wr_hbm, wr), (wi_hbm, wi)) for f in range(RS)])
    cp_bx0 = copies([(bx3_hbm.at[pl.ds(0, head_segs)], bx.at[pl.ds(0, head_segs)]),
                     (mem_hbm, mem0)])
    cp_raw = [[pltpu.make_async_copy(
        (wq_hbm, wk_hbm, wv_hbm)[p % 3].bitcast(U32).at[:, pl.ds(8 * (p // 3), 8), :],
        raw.at[p], raw_sems.at[p])] for p in range(6)]
    cp_xpre = copies([(bx3_hbm.at[:, pl.ds(seg - 8, 8), :], xpre_raw)])
    cp_wo = copies([(wo_hbm.bitcast(U32).at[:, col(j)], wo.at[j]) for j in range(RD)])
    cp_bx1 = copies([(bx3_hbm.at[pl.ds(head_segs, n_seg - head_segs)],
                      bx.at[pl.ds(head_segs, n_seg - head_segs)])])
    cp_ya = copies([(ya.at[j], out_hbm.bitcast(U32).at[:, col(j)]) for j in range(RD)])
    yb_sem = sems.at[next(sem_ids)]

    for group in (cp_tab, *cp_ax, cp_w, cp_xpre, *cp_raw, cp_bx0):
        start(group)
    for c in cp_wo:
        c.start(priority=1)

    def table(g, i):
        first = 0 if g == 0 else 3 * g - 1
        return pltpu.bitcast(mats[pl.ds((first + i) * (LANES // 2), LANES // 2), :], BF16)

    def pipelined(items, first, second, lag):
        pending = []
        for item in items:
            pending.append((item, first(item)))
            if len(pending) > lag:
                second(*pending.pop(0))
        for p in pending:
            second(*p)

    wait(cp_tab)

    def twiddled_dft(a, carry):
        fr, fi = tw[pl.ds(0, LANES), :], tw[pl.ds(LANES, LANES), :]
        re, im = _cmul((fr, fi), (tw[pl.ds(TW_ROW + a, 1), :], tw[pl.ds(TW_ROW + RS + a, 1), :]))
        ftw[a, 0], ftw[a, 1], ftw[a, 2] = re, im - re, im + re
        return carry

    jax.lax.fori_loop(0, RS, twiddled_dft, 0)

    for q in range(X_CHUNKS):
        wait(cp_ax[q])

        def butterflies(ap, carry, q=q):
            n = LANES // X_CHUNKS
            for b in range(q * n, (q + 1) * n, 8):
                v = [xa[j, pl.ds(ap + 8 * b, 8, stride=8), :] for j in range(RD)]
                for par, half in enumerate((_lo, _hi)):
                    u = _radix8_fwd([half(t) for t in v])
                    for i in range(RD):
                        ubuf[2 * ap + par, i, pl.ds(b, 8), :] = u[i]
            return carry

        jax.lax.fori_loop(0, RS // 2, butterflies, 0)

    def fwd(ap, carry):
        half = LANES // 2

        def feature_dft(item):
            a, g = item
            if g == 4:
                return _dot_nt(tw[pl.ds(NYQ_ROW, 8), :], ubuf[a, 0])
            u0, u1 = ubuf[a, 2 * g], ubuf[a, 2 * g + 1]
            if g == 0:
                y0, y1 = _dot_nt(table(0, 0), u0), _dot_nt(table(0, 1), u1)
                return (jnp.concatenate([y0[:half], y1[:half]], axis=0),
                        jnp.concatenate([y0[half:], y1[half:]], axis=0))
            both = _dot_nt(table(g, 0), u0 + u1)
            im = _dot_nt(table(g, 1), u0)
            re = both - _dot_nt(table(g, 2), u1)
            return re, jnp.concatenate([im[:half] - both[:half], im[half:] + both[half:]], axis=0)

        def sequence_dft(item, y):
            a, g = item
            if g == 4:
                rows = pl.ds(KH, 8)
                both = _dot(y, ftw[a, 0])
                re, im = both, both + _dot(y, ftw[a, 1])
            else:
                rows = pl.ds(g * LANES, LANES)
                both = _dot(y[0] + y[1], ftw[a, 0])
                re, im = both - _dot(y[1], ftw[a, 2]), both + _dot(y[0], ftw[a, 1])
            tbuf[0, a, rows, :], tbuf[1, a, rows, :] = re, im

        pipelined([(2 * ap + par, g) for par in range(2) for g in range(5)],
                  feature_dft, sequence_dft, 2)
        return carry

    jax.lax.fori_loop(0, RS // 2, fwd, 0)

    wait(cp_w)

    def filter_rows(rows, filt):
        z = _dft16([(tbuf[0, a, rows, :], tbuf[1, a, rows, :]) for a in range(RS)])
        z = _idft16([_cmul(z[f], filt(f)) for f in range(RS)])
        for a in range(RS):
            tbuf[0, a, rows, :], tbuf[1, a, rows, :] = z[a]

    wr32 = wr.at[:, pl.ds(0, KH), :].bitcast(U32)
    wi32 = wi.at[:, pl.ds(0, KH), :].bitcast(U32)
    for pair in range(4):
        def mid(mb, carry, pair=pair):
            block = pl.ds(pl.multiple_of(32 * mb, 32), 32)
            src = pl.ds(pair, 8, stride=4)
            for par, half in enumerate((_lo, _hi)):
                cls = 2 * pair + par
                rows = pl.ds(pl.multiple_of(64 * K_CLASSES.index(cls) + 8 * mb, 8), 8)

                def filt(f, half=half, cls=cls):
                    re = half(wr32.at[f, block][src, :])
                    im = half(wi32.at[f, block][src, :])
                    if cls == 0:
                        sub = jax.lax.broadcasted_iota(jnp.int32, (8, LANES), 0)
                        c = jnp.where(sub + mb == 0, 0.5, 1.0)
                        re, im = re * c, im * c
                    return re, im

                filter_rows(rows, filt)
            return carry

        jax.lax.fori_loop(0, 8, mid, 0)

    def nyq_row(ref, f):
        return jnp.broadcast_to(ref[f, pl.ds(KH, 1), :].astype(F32), (8, LANES))

    filter_rows(pl.ds(KH, 8), lambda f: (nyq_row(wr, f), nyq_row(wi, f)))

    def repack(p, kt, dst, unit):
        src = raw.at[p].reshape(D * 8, LANES)
        rows = pl.ds(pl.multiple_of(kt * 64, 64), 64)
        for hp in range(8):
            v = src[pl.ds(kt * 8 * LANES + hp, LANES, stride=8), :]
            for par, half in enumerate((v, v >> 16)):
                dst[unit + 2 * hp + par, rows, :] = pltpu.bitcast(half.astype(jnp.uint16), U32)

    def finish(ap):
        for b in range(0, LANES, 8):
            y = [_radix8_adj([ubuf[2 * ap + par, i, pl.ds(b, 8), :] for i in range(RD)])
                 for par in range(2)]
            for j in range(RD):
                ya[j, pl.ds(ap + 8 * b, 8, stride=8), :] = pltpu.pack_elementwise(
                    [y[0][j], y[1][j]], packed_dtype=BF16)

    def inv(ap, carry):
        repack(0, ap, w_a, 0)

        def sequence_idft(item):
            par, g = item
            a = 2 * ap + par
            if g == 4:
                re, im = (jnp.concatenate([tbuf[i, a, pl.ds(KH, 8), :]] * (LANES // 8), axis=0)
                          for i in range(2))
                return _dot_nt(ftw[a, 0], re + im) + _dot_nt(ftw[a, 1], im)
            rows = pl.ds(g * LANES, LANES)
            re, im = tbuf[0, a, rows, :], tbuf[1, a, rows, :]
            both = _dot_nt(ftw[a, 0], re + im)
            return both + _dot_nt(ftw[a, 1], im), both - _dot_nt(ftw[a, 2], re)

        nyquist = {}
        low = jax.lax.broadcasted_iota(jnp.int32, (LANES, LANES), 1) < LANES // 2

        def feature_idft(item, v):
            par, g = item
            a = 2 * ap + par
            if g == 4:
                nyquist[par] = v * (0.5 * tw[pl.ds(NYQ_ROW, 1), :])
            elif g == 0:
                re, im = v
                v0 = jnp.where(low, re, pltpu.roll(im, LANES // 2, 1))
                v1 = jnp.where(low, pltpu.roll(re, LANES // 2, 1), im)
                ubuf[a, 0] = _dot(v0, table(0, 0)) + nyquist.pop(par)
                ubuf[a, 1] = _dot(v1, table(0, 1))
            else:
                re, im = v
                both = _dot(jnp.where(low, re - im, re + im), table(g, 0))
                ubuf[a, 2 * g] = both + _dot(im, table(g, 1))
                ubuf[a, 2 * g + 1] = both - _dot(re, table(g, 2))

        pipelined([(par, g) for par in range(2) for g in (4, 0, 1, 2, 3)],
                  sequence_idft, feature_idft, 3)
        return carry

    wait(cp_raw[0])
    jax.lax.fori_loop(0, RS // 2, inv, 0)

    scale = E ** -0.5
    x_rows, mem_rows = pl.ds(0, seg), pl.ds(seg, M)

    def yb_copy(s, n):
        rows = pl.ds(pl.multiple_of(s * seg, seg), n * seg)
        return pltpu.make_async_copy(yb.at[rows], out_hbm.at[rows, pl.ds(D, D)], yb_sem)

    wait(cp_xpre)

    def widen(i, carry):
        xpre[pl.ds(pl.multiple_of(32 * i, 32), 32), :] = pltpu.bitcast(
            xpre_raw[pl.ds(8 * i, 8)].reshape(64, D), U32)
        return carry

    jax.lax.fori_loop(0, n_seg // 8, widen, 0)

    def precompute(unit, w):
        pre[unit] = _dot(pltpu.bitcast(xpre[...], BF16), pltpu.bitcast(w, BF16))

    def early(i, carry):
        for p, first in ((1, 0), (2, 2), (3, 5)):
            pl.when(i == first)(functools.partial(wait, cp_raw[p]))
        for unit in range(2):
            precompute(2 * i + unit, w_a[2 * i + unit])
        for j in range(3):
            j = 3 * i + j
            repack(1 + j // 8, j % 8, w_b, 16 * (j // 8))
        finish(i)
        return carry

    jax.lax.fori_loop(0, 8, early, 0)

    def late(i, carry):
        for p, first in ((4, 0), (5, 4)):
            pl.when(i == first)(functools.partial(wait, cp_raw[p]))
        per = (pre.shape[0] - 16) // 8
        for unit in range(per):
            precompute(16 + per * i + unit, w_b[per * i + unit])
        for j in range(2):
            j = 2 * i + j
            repack(4 + j // 8, j % 8, w_c, 16 * (j // 8))
        return carry

    jax.lax.fori_loop(0, 8, late, 0)

    def segment(s):
        rows = pl.ds(pl.multiple_of(s * seg, seg), seg)
        hbuf[x_rows, :] = bx[s].astype(F32)
        qi = jax.lax.broadcasted_iota(jnp.int32, (L, L), 0)
        ki = jax.lax.broadcasted_iota(jnp.int32, (L, L), 1)
        mask = (qi >= seg) | (ki >= seg) | (qi >= ki)
        qkv, probs, ctx = {}, {}, {}

        def project(h):
            qkv[h] = []
            for m in range(3):
                unit = 16 * (3 * (h // 16) + m) + h % 16
                w = w_a[unit] if unit < 16 else w_b[unit - 16] if unit < 64 else w_c[unit - 64]
                w = pltpu.bitcast(w, BF16)
                if unit < pre.shape[0]:
                    x = jnp.concatenate([hbuf[pl.ds(0, seg - 8), :], hbuf[mem_rows, :]], axis=0)
                    r = _dot(x, w)
                    done = pre[unit, pl.ds(pl.multiple_of(8 * s, 8), 8), :]
                    qkv[h].append(jnp.concatenate([r[:seg - 8], done, r[seg - 8:]], axis=0))
                else:
                    qkv[h].append(_dot(hbuf[...], w))

        def scores(h):
            q, k, v = qkv.pop(h)
            sc = jnp.where(mask, _dot_nt(q, k) * scale, -1000000000.0)
            e = jnp.exp(sc - jnp.max(sc, axis=-1, keepdims=True))
            probs[h] = e, jnp.sum(e, axis=-1, keepdims=True), v

        def mix(h):
            e, l, v = probs.pop(h)
            o = _dot(e, v) * (1.0 / l)
            ctx[h] = jnp.concatenate([o[seg:], o[:seg]], axis=0)

        lag_s, lag_m, lag_o = 2, 5, 7
        acc = None
        for t in range(H + lag_o):
            if t < H:
                project(t)
            if 0 <= t - lag_s < H:
                scores(t - lag_s)
            if 0 <= t - lag_m < H:
                mix(t - lag_m)
            if 0 <= t - lag_o < H:
                rows_o = pl.ds((t - lag_o) * (E // 2), E // 2)
                w = jnp.concatenate([wo[j, rows_o, :] for j in range(RD)], axis=1)
                y = _dot(ctx.pop(t - lag_o), pltpu.bitcast(w, BF16))
                acc = y if acc is None else acc + y
        hbuf[mem_rows, :] = acc[:M]
        yb[rows, :] = acc[M:].astype(BF16)

    wait(cp_bx0)
    wait(cp_wo)
    hbuf[mem_rows, :] = mem0[...].astype(F32)
    start(cp_bx1)
    start(cp_ya)

    def segments(i, carry):
        s0 = i * unroll

        @pl.when(i == 1)
        def _():
            wait(cp_bx1)

        @pl.when(i > 0)
        def _():
            yb_copy(s0 - unroll, unroll).start()

        for u in range(unroll):
            segment(s0 + u)
        return carry

    jax.lax.fori_loop(0, n_seg // unroll, segments, 0)
    yb_copy(n_seg - unroll, unroll).start()
    wait(cp_ya)
    pltpu.make_async_copy(yb, out_hbm.at[:, pl.ds(D, D)], yb_sem).wait()


@functools.partial(jax.jit, static_argnames=("B_seg_len",))
def pallas_concat_heads__spectral_gfnet__memory_aug_recurrent_mem_tr__prompt_kernel(
    A_x: jax.Array,
    A_w_r: jax.Array,
    A_w_i: jax.Array,
    B_x: jax.Array,
    B_mem0: jax.Array,
    B_Wq: jax.Array,
    B_Wk: jax.Array,
    B_Wv: jax.Array,
    B_Wo: jax.Array,
    B_seg_len: int,
):
    assert A_x.shape == (1, S, D) and B_x.shape == (1, S, D) and B_mem0.shape == (1, M, D)
    assert B_Wq.shape == (D, H, E) and B_Wo.shape == (H, E, D)
    seg = int(B_seg_len)
    n_seg = S // seg
    assert seg % 16 == 0 and n_seg * seg == S
    mats, tw = _tables()
    vmem = pltpu.VMEM
    out = pl.pallas_call(
        functools.partial(_kernel, seg=seg, n_seg=n_seg),
        out_shape=jax.ShapeDtypeStruct((S, 2 * D), BF16),
        in_specs=[pl.BlockSpec(memory_space=pl.ANY)] * 11,
        out_specs=pl.BlockSpec(memory_space=pl.ANY),
        scratch_shapes=[
            vmem((RD, S // 2, LANES), U32),
            vmem((RS, KH + 1, LANES), BF16),
            vmem((RS, KH + 1, LANES), BF16),
            vmem((mats.shape[0] // 2, LANES), U32),
            vmem(tw.shape, F32),
            vmem((RS, 3, LANES, LANES), F32),
            vmem((RS, RD, LANES, LANES), F32),
            vmem((2, RS, KROWS, LANES), F32),
            vmem((RD, S // 2, LANES), U32),
            vmem((6, D, 8, LANES), U32),
            vmem((16, D // 2, LANES), U32),
            vmem((48, D // 2, LANES), U32),
            vmem((32, D // 2, LANES), U32),
            vmem((RD, H * E // 2, LANES), U32),
            vmem((n_seg, seg, D), BF16),
            vmem((M, D), BF16),
            vmem((M + seg, D), F32),
            vmem((S, D), BF16),
            vmem((n_seg, 8, D), BF16),
            vmem((4 * n_seg, D), U32),
            vmem((32, 8 * n_seg, LANES), F32),
            pltpu.SemaphoreType.DMA((24,)),
            pltpu.SemaphoreType.DMA((6,)),
        ],
        compiler_params=pltpu.CompilerParams(vmem_limit_bytes=120 * 1024 * 1024),
        name="gfnet_rmt",
    )(A_x.reshape(S, D), A_w_r.T, A_w_i.T, B_x.reshape(n_seg, seg, D), B_mem0.reshape(M, D),
      B_Wq, B_Wk, B_Wv, B_Wo.reshape(H * E, D), mats, tw)
    return out.reshape(1, S, 2 * D)
```

```python
import functools

import jax
import jax.numpy as jnp
import numpy as np
from jax.experimental import pallas as pl
from jax.experimental.pallas import tpu as pltpu

F32 = jnp.float32
BF16 = jnp.bfloat16
U32 = jnp.uint32

S = 2048
D = 1024
H = 32
E = 128
M = 8
LANES = 128
RS = S // LANES
RD = D // LANES
KH = D // 2
KROWS = KH + 8
K_CLASSES = (0, 4, 1, 7, 2, 6, 5, 3)
_ROOT_NORM = 2.0 ** -10
TW_ROW = 2 * LANES
NYQ_ROW = TW_ROW + 2 * RS
CLASS_SIGN = (-1.0, 1.0)
KT = D // LANES
GROUP = H // 2
AHEAD = 8
UNROLL = 4


@functools.lru_cache(maxsize=None)
def _tables():
    bf16 = jnp.dtype(BF16)
    h = np.sqrt(0.5)
    butterfly = np.array([
        [1, 1, 1, 1, 1, 1, 1, 1],
        [1, -1, 1, -1, 1, -1, 1, -1],
        [1, h, 0, -h, -1, -h, 0, h],
        [0, h, 1, h, 0, -h, -1, -h],
        [1, 0, -1, 0, 1, 0, -1, 0],
        [0, 1, 0, -1, 0, 1, 0, -1],
        [1, -h, 0, h, -1, h, 0, -h],
        [0, -h, 1, -h, 0, h, -1, h],
    ], dtype=np.float64)
    norm = (butterfly ** 2).sum(axis=1)
    d = np.arange(D)
    half = LANES // 2
    mats = []
    for g in range(4):
        k = np.concatenate([K_CLASSES[2 * g + i] + 8 * np.arange(KH // 8) for i in range(2)])
        ang = 2.0 * np.pi * ((k[:, None] * d[None, :]) % D) / D
        rows = np.concatenate([np.cos(ang), -np.sin(ang)]).reshape(2 * LANES, RD, LANES)
        proj = np.einsum("rjd,cj->rcd", rows, butterfly) / norm[None, :, None]
        p, q = proj[:LANES, 2 * g], proj[:LANES, 2 * g + 1]
        r, t = proj[LANES:, 2 * g], proj[LANES:, 2 * g + 1]
        if g == 0:
            mats += [np.concatenate([p[:half], r[:half]]), np.concatenate([q[half:], t[half:]])]
        else:
            sign = np.repeat(CLASS_SIGN, half)[:, None]
            assert np.allclose(t, sign * p) and np.allclose(q, -sign * r)
            mats += [p, r - sign * p, p + sign * r]
    mats = np.concatenate(mats) * _ROOT_NORM
    nyq = np.tile(1.0 - 2.0 * (np.arange(LANES) % 2), (8, 1)) * _ROOT_NORM
    b = np.arange(LANES)
    ang = 2.0 * np.pi * ((b[:, None] * b[None, :]) % LANES) / LANES
    twang = 2.0 * np.pi * (np.arange(RS)[:, None] * b[None, :]) / S
    tw = np.concatenate([np.cos(ang), -np.sin(ang), np.cos(twang), -np.sin(twang), nyq])
    return mats.astype(bf16), tw.astype(np.float32)


def _lo(v):
    return pltpu.bitcast(v << 16, F32)


def _hi(v):
    return pltpu.bitcast(v & np.uint32(0xFFFF0000), F32)


def _dot(a, b):
    return jnp.dot(a, b, preferred_element_type=F32)


def _dot_nt(a, b):
    return jax.lax.dot_general(a, b, (((1,), (1,)), ((), ())), preferred_element_type=F32)


_H8 = float(np.sqrt(0.5))


def _radix8_fwd(x):
    s04, d04 = x[0] + x[4], x[0] - x[4]
    s26, d26 = x[2] + x[6], x[2] - x[6]
    s15, d15 = x[1] + x[5], x[1] - x[5]
    s37, d37 = x[3] + x[7], x[3] - x[7]
    e0, e1 = s04 + s26, s15 + s37
    p, q = (d15 - d37) * _H8, (d15 + d37) * _H8
    return [e0 + e1, e0 - e1, d04 + p, d26 + q, s04 - s26, s15 - s37, d04 - p, d26 - q]


def _radix8_adj(p):
    e0, e1 = p[0] + p[1], p[0] - p[1]
    s04, s26 = e0 + p[4], e0 - p[4]
    s15, s37 = e1 + p[5], e1 - p[5]
    d04, d26 = p[2] + p[6], p[3] + p[7]
    m, n = (p[2] - p[6]) * _H8, (p[3] - p[7]) * _H8
    d15, d37 = m + n, n - m
    return [s04 + d04, s15 + d15, s26 + d26, s37 + d37,
            s04 - d04, s15 - d15, s26 - d26, s37 - d37]


def _cmul(a, b):
    return a[0] * b[0] - a[1] * b[1], a[0] * b[1] + a[1] * b[0]


def _dft4(z):
    ar, ai = z[0][0] + z[2][0], z[0][1] + z[2][1]
    br, bi = z[0][0] - z[2][0], z[0][1] - z[2][1]
    cr, ci = z[1][0] + z[3][0], z[1][1] + z[3][1]
    dr, di = z[1][0] - z[3][0], z[1][1] - z[3][1]
    return [(ar + cr, ai + ci), (br + di, bi - dr), (ar - cr, ai - ci), (br - di, bi + dr)]


def _rot16(z, n):
    re, im = z
    if n == 0:
        return z
    if n == 4:
        return im, -re
    if n == 2:
        return (re + im) * _H8, (im - re) * _H8
    if n == 6:
        return (im - re) * _H8, (re + im) * (-_H8)
    c, s = float(np.cos(np.pi * n / 8)), float(np.sin(np.pi * n / 8))
    return re * c + im * s, im * c - re * s


def _kernel(ax_hbm, wr_hbm, wi_hbm, bx_hbm, mem_hbm, wq_hbm, wk_hbm, wv_hbm, wo_hbm,
            mats_hbm, tw_hbm, out_hbm,
            ua, wr, wi, mats, tw, ftw, tbuf,
            raw, w_even, w_odd, w_1, w_23, w_45, wo,
            bx, mem0, hbuf, yb, xpre_raw, xpre, pre, sems, *, seg, n_seg):
    sem_ids = iter(range(sems.shape[0]))

    def copies(pairs):
        sem = sems.at[next(sem_ids)]
        return [pltpu.make_async_copy(src, dst, sem) for src, dst in pairs]

    def start(group, **kwargs):
        for c in group:
            c.start(**kwargs)

    def wait(group):
        for c in group:
            c.wait()

    def col(j):
        return pl.ds(j * LANES, LANES)

    def pipelined(items, first, second, lag):
        pending = []
        for item in items:
            pending.append((item, first(item)))
            if len(pending) > lag:
                second(*pending.pop(0))
        for p in pending:
            second(*p)

    def u_load(a, i, first=0, n=LANES):
        return pltpu.bitcast(ua[a, pl.ds(i * LANES + first, n), :], F32)

    def u_store(a, i, value, first=0):
        ua[a, pl.ds(i * LANES + first, value.shape[0]), :] = pltpu.bitcast(value, U32)

    def piece(p, rows):
        src = (wq_hbm, wk_hbm, wv_hbm)[p % 3].bitcast(U32)
        return src.at[rows, pl.ds(GROUP // 2 * (p // 3), GROUP // 2), :], raw.at[p, rows]

    quarter = S // 8
    cp_tw = copies([(tw_hbm, tw)])
    cp_mats = copies([(mats_hbm.bitcast(U32), mats)])
    cp_xpre = copies([(bx_hbm.at[:, pl.ds(seg - AHEAD, AHEAD), :], xpre_raw)])
    cp_tile = [copies([piece(0, pl.ds(kt * LANES, LANES))]) for kt in range(KT)]
    cp_ax = [copies([(ax_hbm.bitcast(U32).at[pl.ds(q * quarter, quarter), col(j)],
                      ua.at[RS + j, pl.ds(q * quarter, quarter)]) for j in range(RD)])
             for q in range(4)]
    cp_piece = {p: copies([piece(p, pl.ds(0, D))]) for p in range(1, 6)}
    cp_w = copies([(src.at[:, col(f)], dst.at[f])
                   for src, dst in ((wr_hbm, wr), (wi_hbm, wi)) for f in range(RS)])
    cp_bx0 = copies([(bx_hbm.at[pl.ds(0, UNROLL)], bx.at[pl.ds(0, UNROLL)]), (mem_hbm, mem0)])
    cp_bx1 = copies([(bx_hbm.at[pl.ds(UNROLL, n_seg - UNROLL)],
                      bx.at[pl.ds(UNROLL, n_seg - UNROLL)])])
    cp_wo = copies([(wo_hbm.bitcast(U32).at[:, col(j)], wo.at[j]) for j in range(RD)])
    cp_ya = copies([(ua.at[RS + j], out_hbm.bitcast(U32).at[:, col(j)]) for j in range(RD)])
    yb_sem = sems.at[next(sem_ids)]

    for group in (cp_tw, cp_xpre, cp_tile[0], cp_tile[1], cp_tile[2], cp_ax[0], cp_tile[3],
                  cp_tile[4], cp_ax[1], cp_tile[5], cp_tile[6], cp_ax[2], cp_tile[7], cp_mats,
                  cp_ax[3], cp_piece[1]):
        start(group)

    def repack(p, kt, dst, unit, tile):
        src = raw.at[p].reshape(D * GROUP // 2, LANES)
        rows = pl.ds(pl.multiple_of(tile * (LANES // 2), LANES // 2), LANES // 2)
        for hp in range(GROUP // 2):
            v = src[pl.ds(kt * (GROUP // 2 * LANES) + hp, LANES, stride=GROUP // 2), :]
            for par, half in enumerate((v, v >> 16)):
                dst[unit + 2 * hp + par, rows, :] = pltpu.bitcast(half.astype(jnp.uint16), U32)

    def precompute(unit, w):
        x = jnp.concatenate([xpre[kt] for kt in range(KT)], axis=1)
        pre[unit] = _dot(pltpu.bitcast(x, BF16), pltpu.bitcast(w, BF16))

    def clear(unit, carry):
        pre[unit] = jnp.zeros(pre.shape[1:], F32)
        return carry

    jax.lax.fori_loop(0, GROUP, clear, 0)

    wait(cp_tw)

    def twiddled_dft(a, carry):
        dft = tw[pl.ds(0, LANES), :], tw[pl.ds(LANES, LANES), :]
        re, im = _cmul(dft, (tw[pl.ds(TW_ROW + a, 1), :], tw[pl.ds(TW_ROW + RS + a, 1), :]))
        ftw[a, 0], ftw[a, 1], ftw[a, 2] = re, im - re, im + re
        return carry

    jax.lax.fori_loop(0, RS, twiddled_dft, 0)
    wait(cp_xpre)

    def gather_tokens(i, carry):
        v = pltpu.bitcast(xpre_raw[pl.ds(8 * i, 8)].reshape(8 * AHEAD, D), U32)
        rows = pl.ds(pl.multiple_of(4 * AHEAD * i, 4 * AHEAD), 4 * AHEAD)
        for kt in range(KT):
            xpre[kt, rows, :] = v[:, kt * LANES:(kt + 1) * LANES]
        return carry

    jax.lax.fori_loop(0, n_seg // 8, gather_tokens, 0)

    def butterflies(q):
        for ap in range(RS // 2):
            for b in range(0, LANES // 4, 8):
                b = pl.multiple_of(q * (LANES // 4) + b, 8)
                v = [ua[RS + j, pl.ds(ap + 8 * b, 8, stride=8), :] for j in range(RD)]
                for par, half in enumerate((_lo, _hi)):
                    for i, u in enumerate(_radix8_fwd([half(t) for t in v])):
                        u_store(2 * ap + par, i, u, b)

    w_0 = (w_even, w_odd)
    wait(cp_tile[0])
    repack(0, 0, w_even, 0, 0)

    def first_piece(i, carry):
        for par in range(2):
            kt = 2 * i + par
            for n in range(1 + par, KT, 2):
                pl.when(kt + 1 == n)(functools.partial(wait, cp_tile[n]))
            if par:
                for q in range(4):
                    pl.when(i == q)(functools.partial(wait, cp_ax[q]))
            x = pltpu.bitcast(xpre[kt], BF16)
            rows = pl.ds(pl.multiple_of(i * (LANES // 2), LANES // 2), LANES // 2)
            for unit in range(GROUP):
                pre[unit] += _dot(x, pltpu.bitcast(w_0[par][unit, rows, :], BF16))
            repack(0, jnp.minimum(kt + 1, KT - 1), w_0[1 - par], 0, i + par)
            if par:
                butterflies(i)
        return carry

    jax.lax.fori_loop(0, KT // 2, first_piece, 0)

    wait(cp_mats)

    def table(g, i):
        first = 0 if g == 0 else 3 * g - 1
        return pltpu.bitcast(mats[pl.ds((first + i) * (LANES // 2), LANES // 2), :], BF16)

    def forward(ap):
        half = LANES // 2

        def feature_dft(item):
            a, g = item
            if g == 4:
                return _dot_nt(tw[pl.ds(NYQ_ROW, 8), :], u_load(a, 0))
            u0, u1 = u_load(a, 2 * g), u_load(a, 2 * g + 1)
            if g == 0:
                y0, y1 = _dot_nt(table(0, 0), u0), _dot_nt(table(0, 1), u1)
                return (jnp.concatenate([y0[:half], y1[:half]], axis=0),
                        jnp.concatenate([y0[half:], y1[half:]], axis=0))
            both = _dot_nt(table(g, 0), u0 + u1)
            im = _dot_nt(table(g, 1), u0)
            re = both - _dot_nt(table(g, 2), u1)
            return re, jnp.concatenate([im[:half] - both[:half], im[half:] + both[half:]], axis=0)

        def sequence_dft(item, y):
            a, g = item
            if g == 4:
                rows = pl.ds(KH, 8)
                both = _dot(y, ftw[a, 0])
                re, im = both, both + _dot(y, ftw[a, 1])
            else:
                rows = pl.ds(g * LANES, LANES)
                both = _dot(y[0] + y[1], ftw[a, 0])
                re, im = both - _dot(y[1], ftw[a, 2]), both + _dot(y[0], ftw[a, 1])
            tbuf[0, a, rows, :], tbuf[1, a, rows, :] = re, im

        pipelined([(2 * ap + par, g) for par in range(2) for g in range(5)],
                  feature_dft, sequence_dft, 2)

    def forward_first(ap, carry):
        forward(ap)
        return carry

    def forward_second(i, carry):
        for kt in range(2):
            repack(1, 2 * i + kt, w_1, 0, 2 * i + kt)
        forward(RS // 4 + i)
        return carry

    jax.lax.fori_loop(0, RS // 4, forward_first, 0)
    wait(cp_piece[1])
    for group in (cp_w, *(cp_piece[p] for p in range(2, 6)), cp_bx0):
        start(group)
    start(cp_wo, priority=1)
    jax.lax.fori_loop(0, RS // 4, forward_second, 0)

    def load(slots, rows):
        return [(tbuf[0, a, rows, :], tbuf[1, a, rows, :]) for a in slots]

    def store(slots, rows, z):
        for a, v in zip(slots, z):
            tbuf[0, a, rows, :], tbuf[1, a, rows, :] = v

    def swap(z):
        return [(im, re) for re, im in z]

    def rotate(z, n):
        return [_rot16(v, n * k) for k, v in enumerate(z)]

    def dft_columns(rows, filt):
        for n in range(4):
            slots = range(n, RS, 4)
            store(slots, rows, rotate(_dft4(load(slots, rows)), n))

    def dft_rows_filter(rows, filt):
        for n in range(4):
            slots = range(4 * n, 4 * n + 4)
            z = _dft4(load(slots, rows))
            store(slots, rows, [_cmul(v, filt(n + 4 * k)) for k, v in enumerate(z)])

    def idft_rows(rows, filt):
        for n in range(4):
            slots = range(4 * n, 4 * n + 4)
            store(slots, rows, rotate(_dft4(swap(load(slots, rows))), n))

    def idft_columns(rows, filt):
        for n in range(4):
            slots = range(n, RS, 4)
            store(slots, rows, swap(_dft4(load(slots, rows))))

    def filter_rows(cls, mb, f):
        block = pl.ds(pl.multiple_of(32 * mb, 32), 32)
        half, src = (_lo, _hi)[cls % 2], pl.ds(cls // 2, 8, stride=4)
        re, im = (half(ref.at[:, pl.ds(0, KH), :].bitcast(U32).at[f, block][src, :])
                  for ref in (wr, wi))
        if cls == 0:
            row = jax.lax.broadcasted_iota(jnp.int32, (8, LANES), 0)
            weight = jnp.where(row + mb == 0, 0.5, 1.0)
            re, im = re * weight, im * weight
        return re, im

    def filter_nyquist(f):
        return tuple(jnp.broadcast_to(ref[f, pl.ds(KH, 1), :].astype(F32), (8, LANES))
                     for ref in (wr, wi))

    for index, step in enumerate((dft_columns, dft_rows_filter, idft_rows, idft_columns)):
        if step is dft_rows_filter:
            wait(cp_w)

        def middle(i, carry, index=index, step=step):
            precompute(GROUP + 4 * index + i, w_1[4 * index + i])
            for mb in (2 * i, 2 * i + 1):
                for cls in range(8):
                    first = 64 * K_CLASSES.index(cls) + 8 * mb
                    step(pl.ds(pl.multiple_of(first, 8), 8),
                         functools.partial(filter_rows, cls, mb))
            return carry

        jax.lax.fori_loop(0, 4, middle, 0)
        step(pl.ds(KH, 8), filter_nyquist)

    def inverse(ap, carry):
        for p in (2, 3):
            repack(p, ap, w_23, GROUP * (p - 2), ap)

        def sequence_idft(item):
            a, g, _ = item
            if g == 4:
                re, im = (jnp.concatenate([tbuf[i, a, pl.ds(KH, 8), :]] * (LANES // 8), axis=0)
                          for i in range(2))
                return _dot_nt(ftw[a, 0], re + im) + _dot_nt(ftw[a, 1], im)
            rows = pl.ds(g * LANES, LANES)
            re, im = tbuf[0, a, rows, :], tbuf[1, a, rows, :]
            both = _dot_nt(ftw[a, 0], re + im)
            return both + _dot_nt(ftw[a, 1], im), both - _dot_nt(ftw[a, 2], re)

        nyquist = {}
        low = jax.lax.broadcasted_iota(jnp.int32, (LANES, LANES), 1) < LANES // 2

        def feature_idft(item, v):
            a, g, par = item
            if g == 4:
                nyquist[par] = v * (0.5 * tw[pl.ds(NYQ_ROW, 1), :])
            elif g == 0:
                re, im = v
                v0 = jnp.where(low, re, pltpu.roll(im, LANES // 2, 1))
                v1 = jnp.where(low, pltpu.roll(re, LANES // 2, 1), im)
                u_store(a, 0, _dot(v0, table(0, 0)) + nyquist.pop(par))
                u_store(a, 1, _dot(v1, table(0, 1)))
            else:
                re, im = v
                both = _dot(jnp.where(low, re - im, re + im), table(g, 0))
                u_store(a, 2 * g, both + _dot(im, table(g, 1)))
                u_store(a, 2 * g + 1, both - _dot(re, table(g, 2)))

        pipelined([(2 * ap + par, g, par) for par in range(2) for g in (4, 0, 1, 2, 3)],
                  sequence_idft, feature_idft, 3)
        return carry

    wait(cp_piece[2])
    wait(cp_piece[3])
    jax.lax.fori_loop(0, RS // 2, inverse, 0)

    def last_pieces(ap, carry):
        for p in (4, 5):
            pl.when(ap == 4 * (p - 4))(functools.partial(wait, cp_piece[p]))
        for unit in (2 * ap, 2 * ap + 1):
            precompute(2 * GROUP + unit, w_23[unit])
        for j in (2 * ap, 2 * ap + 1):
            repack(4 + j // KT, j % KT, w_45, GROUP * (j // KT), j % KT)
        for b in range(0, LANES, 8):
            y = [_radix8_adj([u_load(2 * ap + par, i, b, 8) for i in range(RD)])
                 for par in range(2)]
            for j in range(RD):
                ua[RS + j, pl.ds(ap + 8 * b, 8, stride=8), :] = pltpu.pack_elementwise(
                    [y[0][j], y[1][j]], packed_dtype=BF16)
        return carry

    jax.lax.fori_loop(0, RS // 2, last_pieces, 0)

    L = M + seg
    scale = E ** -0.5
    mem_rows = pl.ds(seg, M)

    def segment(s):
        hbuf[pl.ds(0, seg), :] = bx[s].astype(F32)
        qi = jax.lax.broadcasted_iota(jnp.int32, (L, L), 0)
        ki = jax.lax.broadcasted_iota(jnp.int32, (L, L), 1)
        mask = (qi >= seg) | (ki >= seg) | (qi >= ki)
        qkv, probs, ctx = {}, {}, {}

        def project(h, m):
            p, i = 3 * (h // GROUP) + m, h % GROUP
            if p == 0:
                w = jnp.concatenate(
                    [w_0[kt % 2][i, pl.ds(kt // 2 * (LANES // 2), LANES // 2), :]
                     for kt in range(KT)], axis=0)
            else:
                w = w_1[i] if p == 1 else (w_23, w_45)[p // 2 - 1][GROUP * (p % 2) + i]
            w = pltpu.bitcast(w, BF16)
            unit = GROUP * p + i
            if not 1 <= unit < pre.shape[0]:
                return _dot(hbuf[...], w)
            x = jnp.concatenate([hbuf[pl.ds(0, seg - AHEAD), :], hbuf[mem_rows, :]], axis=0)
            r = _dot(x, w)
            done = pre[unit, pl.ds(pl.multiple_of(AHEAD * s, AHEAD), AHEAD), :]
            return jnp.concatenate([r[:seg - AHEAD], done, r[seg - AHEAD:]], axis=0)

        def scores(h):
            q, k, v = qkv.pop(h)
            sc = jnp.where(mask, _dot_nt(q, k) * scale, -1000000000.0)
            e = jnp.exp(sc - jnp.max(sc, axis=-1, keepdims=True))
            probs[h] = e, jnp.sum(e, axis=-1, keepdims=True), v

        def mix(h):
            e, total, v = probs.pop(h)
            o = _dot(e, v) * (1.0 / total)
            ctx[h] = jnp.concatenate([o[seg:], o[:seg]], axis=0)

        def output(h):
            rows = pl.ds(h * (E // 2), E // 2)
            w = jnp.concatenate([wo[j, rows, :] for j in range(RD)], axis=1)
            return _dot(ctx.pop(h), pltpu.bitcast(w, BF16))

        lag_scores, lag_mix, lag_output = 2, 5, 7
        acc = None
        for t in range(H + lag_output):
            if t < H:
                qkv[t] = [project(t, m) for m in range(3)]
            if 0 <= t - lag_scores < H:
                scores(t - lag_scores)
            if 0 <= t - lag_mix < H:
                mix(t - lag_mix)
            if 0 <= t - lag_output < H:
                y = output(t - lag_output)
                acc = y if acc is None else acc + y
        hbuf[mem_rows, :] = acc[:M]
        yb[pl.ds(pl.multiple_of(s * seg, seg), seg), :] = acc[M:].astype(BF16)

    def yb_copy(i):
        rows = pl.ds(pl.multiple_of(i * (UNROLL * seg), UNROLL * seg), UNROLL * seg)
        return pltpu.make_async_copy(yb.at[rows], out_hbm.at[rows, pl.ds(D, D)], yb_sem)

    wait(cp_bx0)
    wait(cp_wo)
    hbuf[mem_rows, :] = mem0[...].astype(F32)
    start(cp_bx1)
    start(cp_ya)

    def segments(i, carry):
        pl.when(i == 1)(functools.partial(wait, cp_bx1))

        @pl.when(i > 0)
        def _():
            yb_copy(i - 1).start()

        for u in range(UNROLL):
            segment(UNROLL * i + u)
        return carry

    jax.lax.fori_loop(0, n_seg // UNROLL, segments, 0)
    yb_copy(n_seg // UNROLL - 1).start()
    wait(cp_ya)
    pltpu.make_async_copy(yb, out_hbm.at[:, pl.ds(D, D)], yb_sem).wait()


@functools.partial(jax.jit, static_argnames=("B_seg_len",))
def pallas_concat_heads__spectral_gfnet__memory_aug_recurrent_mem_tr__prompt_kernel(
    A_x: jax.Array,
    A_w_r: jax.Array,
    A_w_i: jax.Array,
    B_x: jax.Array,
    B_mem0: jax.Array,
    B_Wq: jax.Array,
    B_Wk: jax.Array,
    B_Wv: jax.Array,
    B_Wo: jax.Array,
    B_seg_len: int,
):
    assert A_x.shape == (1, S, D) and B_x.shape == (1, S, D) and B_mem0.shape == (1, M, D)
    assert B_Wq.shape == (D, H, E) and B_Wo.shape == (H, E, D)
    seg = int(B_seg_len)
    n_seg = S // seg
    assert seg % 16 == 0 and n_seg * seg == S and n_seg % 8 == 0
    mats, tw = _tables()
    vmem = pltpu.VMEM
    out = pl.pallas_call(
        functools.partial(_kernel, seg=seg, n_seg=n_seg),
        out_shape=jax.ShapeDtypeStruct((S, 2 * D), BF16),
        in_specs=[pl.BlockSpec(memory_space=pl.ANY)] * 11,
        out_specs=pl.BlockSpec(memory_space=pl.ANY),
        scratch_shapes=[
            vmem((RS + RD, RD * LANES, LANES), U32),
            vmem((RS, KH + 1, LANES), BF16),
            vmem((RS, KH + 1, LANES), BF16),
            vmem((mats.shape[0] // 2, LANES), U32),
            vmem(tw.shape, F32),
            vmem((RS, 3, LANES, LANES), F32),
            vmem((2, RS, KROWS, LANES), F32),
            vmem((6, D, GROUP // 2, LANES), U32),
            vmem((GROUP, D // 4 + LANES // 2, LANES), U32),
            vmem((GROUP, D // 4, LANES), U32),
            vmem((GROUP, D // 2, LANES), U32),
            vmem((2 * GROUP, D // 2, LANES), U32),
            vmem((2 * GROUP, D // 2, LANES), U32),
            vmem((RD, H * E // 2, LANES), U32),
            vmem((n_seg, seg, D), BF16),
            vmem((M, D), BF16),
            vmem((M + seg, D), F32),
            vmem((S, D), BF16),
            vmem((n_seg, AHEAD, D), BF16),
            vmem((KT, AHEAD * n_seg // 2, LANES), U32),
            vmem((3 * GROUP, AHEAD * n_seg, LANES), F32),
            pltpu.SemaphoreType.DMA((26,)),
        ],
        compiler_params=pltpu.CompilerParams(vmem_limit_bytes=120 * 1024 * 1024),
        name="gfnet_rmt",
    )(A_x.reshape(S, D), A_w_r.T, A_w_i.T, B_x.reshape(n_seg, seg, D), B_mem0.reshape(M, D),
      B_Wq, B_Wk, B_Wv, B_Wo.reshape(H * E, D), mats, tw)
    return out.reshape(1, S, 2 * D)
```

```python
import functools

import jax
import jax.numpy as jnp
import numpy as np
from jax.experimental import pallas as pl
from jax.experimental.pallas import tpu as pltpu

F32 = jnp.float32
BF16 = jnp.bfloat16
U32 = jnp.uint32

S = 2048
D = 1024
H = 32
E = 128
M = 8
LANES = 128
RS = S // LANES
RD = D // LANES
KH = D // 2
KROWS = KH + 8
K_CLASSES = (0, 4, 1, 7, 2, 6, 5, 3)
_ROOT_NORM = 2.0 ** -10
TW_ROW = 2 * LANES
NYQ_ROW = TW_ROW + 2 * RS
CLASS_SIGN = (-1.0, 1.0)
KT = D // LANES
GROUP = H // 2
AHEAD = 8
AHEAD_PIECES = (0, 1, 3)
UNROLL = 4


@functools.lru_cache(maxsize=None)
def _tables():
    bf16 = jnp.dtype(BF16)
    h = np.sqrt(0.5)
    butterfly = np.array([
        [1, 1, 1, 1, 1, 1, 1, 1],
        [1, -1, 1, -1, 1, -1, 1, -1],
        [1, h, 0, -h, -1, -h, 0, h],
        [0, h, 1, h, 0, -h, -1, -h],
        [1, 0, -1, 0, 1, 0, -1, 0],
        [0, 1, 0, -1, 0, 1, 0, -1],
        [1, -h, 0, h, -1, h, 0, -h],
        [0, -h, 1, -h, 0, h, -1, h],
    ], dtype=np.float64)
    norm = (butterfly ** 2).sum(axis=1)
    d = np.arange(D)
    half = LANES // 2
    mats = []
    for g in range(4):
        k = np.concatenate([K_CLASSES[2 * g + i] + 8 * np.arange(KH // 8) for i in range(2)])
        ang = 2.0 * np.pi * ((k[:, None] * d[None, :]) % D) / D
        rows = np.concatenate([np.cos(ang), -np.sin(ang)]).reshape(2 * LANES, RD, LANES)
        proj = np.einsum("rjd,cj->rcd", rows, butterfly) / norm[None, :, None]
        p, q = proj[:LANES, 2 * g], proj[:LANES, 2 * g + 1]
        r, t = proj[LANES:, 2 * g], proj[LANES:, 2 * g + 1]
        if g == 0:
            mats += [np.concatenate([p[:half], r[:half]]), np.concatenate([q[half:], t[half:]])]
        else:
            sign = np.repeat(CLASS_SIGN, half)[:, None]
            assert np.allclose(t, sign * p) and np.allclose(q, -sign * r)
            mats += [p, r - sign * p, p + sign * r]
    mats = np.concatenate(mats) * _ROOT_NORM
    nyq = np.tile(1.0 - 2.0 * (np.arange(LANES) % 2), (8, 1)) * _ROOT_NORM
    b = np.arange(LANES)
    ang = 2.0 * np.pi * ((b[:, None] * b[None, :]) % LANES) / LANES
    twang = 2.0 * np.pi * (np.arange(RS)[:, None] * b[None, :]) / S
    tw = np.concatenate([np.cos(ang), -np.sin(ang), np.cos(twang), -np.sin(twang), nyq])
    return mats.astype(bf16), tw.astype(np.float32)


def _lo(v):
    return pltpu.bitcast(v << 16, F32)


def _hi(v):
    return pltpu.bitcast(v & np.uint32(0xFFFF0000), F32)


def _dot(a, b):
    return jnp.dot(a, b, preferred_element_type=F32)


def _dot_nt(a, b):
    return jax.lax.dot_general(a, b, (((1,), (1,)), ((), ())), preferred_element_type=F32)


_H8 = float(np.sqrt(0.5))


def _radix8_fwd(x):
    s04, d04 = x[0] + x[4], x[0] - x[4]
    s26, d26 = x[2] + x[6], x[2] - x[6]
    s15, d15 = x[1] + x[5], x[1] - x[5]
    s37, d37 = x[3] + x[7], x[3] - x[7]
    e0, e1 = s04 + s26, s15 + s37
    p, q = (d15 - d37) * _H8, (d15 + d37) * _H8
    return [e0 + e1, e0 - e1, d04 + p, d26 + q, s04 - s26, s15 - s37, d04 - p, d26 - q]


def _radix8_adj(p):
    e0, e1 = p[0] + p[1], p[0] - p[1]
    s04, s26 = e0 + p[4], e0 - p[4]
    s15, s37 = e1 + p[5], e1 - p[5]
    d04, d26 = p[2] + p[6], p[3] + p[7]
    m, n = (p[2] - p[6]) * _H8, (p[3] - p[7]) * _H8
    d15, d37 = m + n, n - m
    return [s04 + d04, s15 + d15, s26 + d26, s37 + d37,
            s04 - d04, s15 - d15, s26 - d26, s37 - d37]


def _cmul(a, b):
    return a[0] * b[0] - a[1] * b[1], a[0] * b[1] + a[1] * b[0]


def _dft4(z):
    ar, ai = z[0][0] + z[2][0], z[0][1] + z[2][1]
    br, bi = z[0][0] - z[2][0], z[0][1] - z[2][1]
    cr, ci = z[1][0] + z[3][0], z[1][1] + z[3][1]
    dr, di = z[1][0] - z[3][0], z[1][1] - z[3][1]
    return [(ar + cr, ai + ci), (br + di, bi - dr), (ar - cr, ai - ci), (br - di, bi + dr)]


def _rot16(z, n):
    re, im = z
    if n == 0:
        return z
    if n == 4:
        return im, -re
    if n == 2:
        return (re + im) * _H8, (im - re) * _H8
    if n == 6:
        return (im - re) * _H8, (re + im) * (-_H8)
    c, s = float(np.cos(np.pi * n / 8)), float(np.sin(np.pi * n / 8))
    return re * c + im * s, im * c - re * s


def _kernel(ax_hbm, wr_hbm, wi_hbm, bx_hbm, mem_hbm, wq_hbm, wk_hbm, wv_hbm, wo_hbm,
            mats_hbm, tw_hbm, out_hbm,
            ua, wr, wi, mats, tw, ftw, tbuf,
            raw, w_even, w_odd, w_1, w_23, w_45, wo,
            bx, mem0, hbuf, yb, xpre_raw, xpre, pre, zeros, sems, *, seg, n_seg):
    sem_ids = iter(range(sems.shape[0]))

    def copies(pairs):
        sem = sems.at[next(sem_ids)]
        return [pltpu.make_async_copy(src, dst, sem) for src, dst in pairs]

    def start(group, **kwargs):
        for c in group:
            c.start(**kwargs)

    def wait(group):
        for c in group:
            c.wait()

    def col(j):
        return pl.ds(j * LANES, LANES)

    def pipelined(items, first, second, lag):
        pending = []
        for item in items:
            pending.append((item, first(item)))
            if len(pending) > lag:
                second(*pending.pop(0))
        for p in pending:
            second(*p)

    def u_load(a, i, first=0, n=LANES):
        return pltpu.bitcast(ua[a, pl.ds(i * LANES + first, n), :], F32)

    def u_store(a, i, value, first=0):
        ua[a, pl.ds(i * LANES + first, value.shape[0]), :] = pltpu.bitcast(value, U32)

    def piece(p, rows):
        src = (wq_hbm, wk_hbm, wv_hbm)[p % 3].bitcast(U32)
        return src.at[rows, pl.ds(GROUP // 2 * (p // 3), GROUP // 2), :], raw.at[p, rows]

    quarter = S // 8
    cp_tw = copies([(tw_hbm, tw)])
    cp_mats = copies([(mats_hbm.bitcast(U32), mats)])
    cp_xpre = copies([(bx_hbm.at[:, pl.ds(seg - AHEAD, AHEAD), :], xpre_raw)])
    cp_tile = [copies([piece(0, pl.ds(kt * LANES, LANES))]) for kt in range(KT)]
    cp_ax = [copies([(ax_hbm.bitcast(U32).at[pl.ds(q * quarter, quarter), col(j)],
                      ua.at[RS + j, pl.ds(q * quarter, quarter)]) for j in range(RD)])
             for q in range(4)]
    cp_piece = {p: copies([piece(p, pl.ds(0, D))]) for p in range(1, 6)}
    cp_w = copies([(src.at[:, col(f)], dst.at[f])
                   for src, dst in ((wr_hbm, wr), (wi_hbm, wi)) for f in range(RS)])
    cp_bx0 = copies([(bx_hbm.at[pl.ds(0, UNROLL)], bx.at[pl.ds(0, UNROLL)]), (mem_hbm, mem0)])
    cp_bx1 = copies([(bx_hbm.at[pl.ds(UNROLL, n_seg - UNROLL)],
                      bx.at[pl.ds(UNROLL, n_seg - UNROLL)])])
    cp_wo = copies([(wo_hbm.bitcast(U32).at[:, col(j)], wo.at[j]) for j in range(RD)])
    cp_ya = copies([(ua.at[RS + j], out_hbm.bitcast(U32).at[:, col(j)]) for j in range(RD)])
    yb_sem = sems.at[next(sem_ids)]

    for group in (cp_tw, cp_xpre, cp_tile[0], cp_tile[1], cp_tile[2], cp_ax[0], cp_tile[3],
                  cp_tile[4], cp_ax[1], cp_tile[5], cp_tile[6], cp_ax[2], cp_tile[7], cp_mats,
                  cp_ax[3], cp_piece[1]):
        start(group)

    def repack(p, kt, dst, unit, tile):
        src = raw.at[p].reshape(D * GROUP // 2, LANES)
        rows = pl.ds(pl.multiple_of(tile * (LANES // 2), LANES // 2), LANES // 2)
        for hp in range(GROUP // 2):
            v = src[pl.ds(kt * (GROUP // 2 * LANES) + hp, LANES, stride=GROUP // 2), :]
            for par, half in enumerate((v, v >> 16)):
                dst[unit + 2 * hp + par, rows, :] = pltpu.bitcast(half.astype(jnp.uint16), U32)

    def precompute(unit, w):
        x = jnp.concatenate([xpre[kt] for kt in range(KT)], axis=1)
        pre[unit] = _dot(pltpu.bitcast(x, BF16), pltpu.bitcast(w, BF16))

    def clear(unit, carry):
        pre[unit] = jnp.zeros(pre.shape[1:], F32)
        return carry

    jax.lax.fori_loop(0, GROUP, clear, 0)
    for k in range(zeros.shape[0]):
        zeros[k] = 0

    wait(cp_tw)

    def twiddled_dft(a, carry):
        dft = tw[pl.ds(0, LANES), :], tw[pl.ds(LANES, LANES), :]
        re, im = _cmul(dft, (tw[pl.ds(TW_ROW + a, 1), :], tw[pl.ds(TW_ROW + RS + a, 1), :]))
        ftw[a, 0], ftw[a, 1], ftw[a, 2] = re, im - re, im + re
        return carry

    jax.lax.fori_loop(0, RS, twiddled_dft, 0)
    wait(cp_xpre)

    def gather_tokens(i, carry):
        v = pltpu.bitcast(xpre_raw[pl.ds(8 * i, 8)].reshape(8 * AHEAD, D), U32)
        rows = pl.ds(pl.multiple_of(4 * AHEAD * i, 4 * AHEAD), 4 * AHEAD)
        for kt in range(KT):
            xpre[kt, rows, :] = v[:, kt * LANES:(kt + 1) * LANES]
        return carry

    jax.lax.fori_loop(0, n_seg // 8, gather_tokens, 0)

    def butterflies(q):
        for ap in range(RS // 2):
            for b in range(0, LANES // 4, 8):
                b = pl.multiple_of(q * (LANES // 4) + b, 8)
                v = [ua[RS + j, pl.ds(ap + 8 * b, 8, stride=8), :] for j in range(RD)]
                for par, half in enumerate((_lo, _hi)):
                    for i, u in enumerate(_radix8_fwd([half(t) for t in v])):
                        u_store(2 * ap + par, i, u, b)

    w_0 = (w_even, w_odd)
    wait(cp_tile[0])
    repack(0, 0, w_even, 0, 0)

    def first_piece(i, carry):
        for par in range(2):
            kt = 2 * i + par
            for n in range(1 + par, KT, 2):
                pl.when(kt + 1 == n)(functools.partial(wait, cp_tile[n]))
            if par:
                for q in range(4):
                    pl.when(i == q)(functools.partial(wait, cp_ax[q]))
            x = pltpu.bitcast(xpre[kt], BF16)
            rows = pl.ds(pl.multiple_of(i * (LANES // 2), LANES // 2), LANES // 2)
            for unit in range(GROUP):
                pre[unit] += _dot(x, pltpu.bitcast(w_0[par][unit, rows, :], BF16))
            repack(0, jnp.minimum(kt + 1, KT - 1), w_0[1 - par], 0, i + par)
            if par:
                butterflies(i)
        return carry

    jax.lax.fori_loop(0, KT // 2, first_piece, 0)

    wait(cp_mats)

    def table(g, i):
        first = 0 if g == 0 else 3 * g - 1
        return pltpu.bitcast(mats[pl.ds((first + i) * (LANES // 2), LANES // 2), :], BF16)

    def forward(ap):
        half = LANES // 2

        def feature_dft(item):
            a, g = item
            if g == 4:
                return _dot_nt(tw[pl.ds(NYQ_ROW, 8), :], u_load(a, 0))
            u0, u1 = u_load(a, 2 * g), u_load(a, 2 * g + 1)
            if g == 0:
                y0, y1 = _dot_nt(table(0, 0), u0), _dot_nt(table(0, 1), u1)
                return (jnp.concatenate([y0[:half], y1[:half]], axis=0),
                        jnp.concatenate([y0[half:], y1[half:]], axis=0))
            both = _dot_nt(table(g, 0), u0 + u1)
            im = _dot_nt(table(g, 1), u0)
            re = both - _dot_nt(table(g, 2), u1)
            return re, jnp.concatenate([im[:half] - both[:half], im[half:] + both[half:]], axis=0)

        def sequence_dft(item, y):
            a, g = item
            if g == 4:
                rows = pl.ds(KH, 8)
                both = _dot(y, ftw[a, 0])
                re, im = both, both + _dot(y, ftw[a, 1])
            else:
                rows = pl.ds(g * LANES, LANES)
                both = _dot(y[0] + y[1], ftw[a, 0])
                re, im = both - _dot(y[1], ftw[a, 2]), both + _dot(y[0], ftw[a, 1])
            tbuf[0, a, rows, :], tbuf[1, a, rows, :] = re, im

        pipelined([(2 * ap + par, g) for par in range(2) for g in range(5)],
                  feature_dft, sequence_dft, 2)

    def forward_first(ap, carry):
        forward(ap)
        return carry

    def forward_second(i, carry):
        for kt in range(2):
            repack(1, 2 * i + kt, w_1, 0, 2 * i + kt)
        forward(RS // 4 + i)
        return carry

    jax.lax.fori_loop(0, RS // 4, forward_first, 0)
    wait(cp_piece[1])
    for group in (cp_w, *(cp_piece[p] for p in range(2, 6)), cp_bx0):
        start(group)
    start(cp_wo, priority=1)
    jax.lax.fori_loop(0, RS // 4, forward_second, 0)

    def load(slots, rows):
        return [(tbuf[0, a, rows, :], tbuf[1, a, rows, :]) for a in slots]

    def store(slots, rows, z):
        for a, v in zip(slots, z):
            tbuf[0, a, rows, :], tbuf[1, a, rows, :] = v

    def swap(z):
        return [(im, re) for re, im in z]

    def rotate(z, n):
        return [_rot16(v, n * k) for k, v in enumerate(z)]

    def columns(n):
        return range(n, RS, 4)

    def lines(n):
        return range(4 * n, 4 * n + 4)

    passes = (
        (columns, lambda z, n, filt: rotate(_dft4(z), n)),
        (lines, lambda z, n, filt: [_cmul(v, filt(n + 4 * k)) for k, v in enumerate(_dft4(z))]),
        (lines, lambda z, n, filt: rotate(_dft4(swap(z)), n)),
        (columns, lambda z, n, filt: swap(_dft4(z))),
    )

    def run_pass(index, row, filt, link):
        slots, step = passes[index]
        for half in range(2):
            rows = pl.ds(pl.multiple_of(row + zeros[(2 * link + half) % zeros.shape[0]], 8), 8)
            group = (2 * half, 2 * half + 1)
            z = [load(slots(n), rows) for n in group]
            for n, v in zip(group, z):
                store(slots(n), rows, step(v, n, filt))

    def filter_rows(cls, mb, f):
        block = pl.ds(pl.multiple_of(32 * mb, 32), 32)
        half, src = (_lo, _hi)[cls % 2], pl.ds(cls // 2, 8, stride=4)
        re, im = (half(ref.at[:, pl.ds(0, KH), :].bitcast(U32).at[f, block][src, :])
                  for ref in (wr, wi))
        if cls == 0:
            row = jax.lax.broadcasted_iota(jnp.int32, (8, LANES), 0)
            weight = jnp.where(row + mb == 0, 0.5, 1.0)
            re, im = re * weight, im * weight
        return re, im

    def filter_nyquist(f):
        return tuple(jnp.broadcast_to(ref[f, pl.ds(KH, 1), :].astype(F32), (8, LANES))
                     for ref in (wr, wi))

    for index in range(4):
        if index == 1:
            wait(cp_w)

        def middle(i, carry, index=index):
            for unit in (4 * index + 2 * i, 4 * index + 2 * i + 1):
                precompute(GROUP + unit, w_1[unit])
            for n in range(4):
                mb = 4 * i + n
                for cls in range(8):
                    run_pass(index, 64 * K_CLASSES.index(cls) + 8 * mb,
                             functools.partial(filter_rows, cls, mb), 8 * n + cls)
            return carry

        jax.lax.fori_loop(0, 2, middle, 0)
        run_pass(index, KH, filter_nyquist, 0)

    def inverse(ap, carry):
        for p in (2, 3):
            repack(p, ap, w_23, GROUP * (p - 2), ap)

        def sequence_idft(item):
            a, g, _ = item
            if g == 4:
                re, im = (jnp.concatenate([tbuf[i, a, pl.ds(KH, 8), :]] * (LANES // 8), axis=0)
                          for i in range(2))
                return _dot_nt(ftw[a, 0], re + im) + _dot_nt(ftw[a, 1], im)
            rows = pl.ds(g * LANES, LANES)
            re, im = tbuf[0, a, rows, :], tbuf[1, a, rows, :]
            both = _dot_nt(ftw[a, 0], re + im)
            return both + _dot_nt(ftw[a, 1], im), both - _dot_nt(ftw[a, 2], re)

        nyquist = {}
        low = jax.lax.broadcasted_iota(jnp.int32, (LANES, LANES), 1) < LANES // 2

        def feature_idft(item, v):
            a, g, par = item
            if g == 4:
                nyquist[par] = v * (0.5 * tw[pl.ds(NYQ_ROW, 1), :])
            elif g == 0:
                re, im = v
                v0 = jnp.where(low, re, pltpu.roll(im, LANES // 2, 1))
                v1 = jnp.where(low, pltpu.roll(re, LANES // 2, 1), im)
                u_store(a, 0, _dot(v0, table(0, 0)) + nyquist.pop(par))
                u_store(a, 1, _dot(v1, table(0, 1)))
            else:
                re, im = v
                both = _dot(jnp.where(low, re - im, re + im), table(g, 0))
                u_store(a, 2 * g, both + _dot(im, table(g, 1)))
                u_store(a, 2 * g + 1, both - _dot(re, table(g, 2)))

        pipelined([(2 * ap + par, g, par) for par in range(2) for g in (4, 0, 1, 2, 3)],
                  sequence_idft, feature_idft, 3)
        return carry

    wait(cp_piece[2])
    wait(cp_piece[3])
    jax.lax.fori_loop(0, RS // 2, inverse, 0)

    def last_pieces(ap, carry):
        for p in (4, 5):
            pl.when(ap == 4 * (p - 4))(functools.partial(wait, cp_piece[p]))
        for unit in (2 * ap, 2 * ap + 1):
            precompute(2 * GROUP + unit, w_23[GROUP + unit])
        for j in (2 * ap, 2 * ap + 1):
            repack(4 + j // KT, j % KT, w_45, GROUP * (j // KT), j % KT)
        for b in range(0, LANES, 8):
            y = [_radix8_adj([u_load(2 * ap + par, i, b, 8) for i in range(RD)])
                 for par in range(2)]
            for j in range(RD):
                ua[RS + j, pl.ds(ap + 8 * b, 8, stride=8), :] = pltpu.pack_elementwise(
                    [y[0][j], y[1][j]], packed_dtype=BF16)
        return carry

    jax.lax.fori_loop(0, RS // 2, last_pieces, 0)

    L = M + seg
    scale = E ** -0.5
    mem_rows = pl.ds(seg, M)

    def segment(s):
        hbuf[pl.ds(0, seg), :] = bx[s].astype(F32)
        qi = jax.lax.broadcasted_iota(jnp.int32, (L, L), 0)
        ki = jax.lax.broadcasted_iota(jnp.int32, (L, L), 1)
        mask = (qi >= seg) | (ki >= seg) | (qi >= ki)
        qkv, probs, ctx = {}, {}, {}

        def project(h, m):
            p, i = 3 * (h // GROUP) + m, h % GROUP
            if p == 0:
                w = jnp.concatenate(
                    [w_0[kt % 2][i, pl.ds(kt // 2 * (LANES // 2), LANES // 2), :]
                     for kt in range(KT)], axis=0)
            else:
                w = w_1[i] if p == 1 else (w_23, w_45)[p // 2 - 1][GROUP * (p % 2) + i]
            w = pltpu.bitcast(w, BF16)
            if p not in AHEAD_PIECES or (h, m) == (0, 0):
                return _dot(hbuf[...], w)
            unit = GROUP * AHEAD_PIECES.index(p) + i
            x = jnp.concatenate([hbuf[pl.ds(0, seg - AHEAD), :], hbuf[mem_rows, :]], axis=0)
            r = _dot(x, w)
            done = pre[unit, pl.ds(pl.multiple_of(AHEAD * s, AHEAD), AHEAD), :]
            return jnp.concatenate([r[:seg - AHEAD], done, r[seg - AHEAD:]], axis=0)

        def scores(h):
            q, k, v = qkv.pop(h)
            sc = jnp.where(mask, _dot_nt(q, k) * scale, -1000000000.0)
            e = jnp.exp(sc - jnp.max(sc, axis=-1, keepdims=True))
            probs[h] = e, jnp.sum(e, axis=-1, keepdims=True), v

        def mix(h):
            e, total, v = probs.pop(h)
            o = _dot(e, v) * (1.0 / total)
            ctx[h] = jnp.concatenate([o[seg:], o[:seg]], axis=0)

        def output(h):
            rows = pl.ds(h * (E // 2), E // 2)
            w = jnp.concatenate([wo[j, rows, :] for j in range(RD)], axis=1)
            return _dot(ctx.pop(h), pltpu.bitcast(w, BF16))

        lag_scores, lag_mix, lag_output = 2, 6, 8
        acc = None
        for t in range(H + lag_output):
            if t < H:
                qkv[t] = [project(t, 0)]
            if 0 <= t - lag_scores < H:
                scores(t - lag_scores)
            if t < H:
                qkv[t].append(project(t, 1))
            if 0 <= t - lag_mix < H:
                mix(t - lag_mix)
            if t < H:
                qkv[t].append(project(t, 2))
            if 0 <= t - lag_output < H:
                y = output(t - lag_output)
                acc = y if acc is None else acc + y
        hbuf[mem_rows, :] = acc[:M]
        yb[pl.ds(pl.multiple_of(s * seg, seg), seg), :] = acc[M:].astype(BF16)

    def yb_copy(i):
        rows = pl.ds(pl.multiple_of(i * (UNROLL * seg), UNROLL * seg), UNROLL * seg)
        return pltpu.make_async_copy(yb.at[rows], out_hbm.at[rows, pl.ds(D, D)], yb_sem)

    wait(cp_bx0)
    wait(cp_wo)
    hbuf[mem_rows, :] = mem0[...].astype(F32)
    start(cp_bx1)
    start(cp_ya)

    def segments(i, carry):
        pl.when(i == 1)(functools.partial(wait, cp_bx1))

        @pl.when(i > 0)
        def _():
            yb_copy(i - 1).start()

        for u in range(UNROLL):
            segment(UNROLL * i + u)
        return carry

    jax.lax.fori_loop(0, n_seg // UNROLL, segments, 0)
    yb_copy(n_seg // UNROLL - 1).start()
    wait(cp_ya)
    pltpu.make_async_copy(yb, out_hbm.at[:, pl.ds(D, D)], yb_sem).wait()


@functools.partial(jax.jit, static_argnames=("B_seg_len",))
def pallas_concat_heads__spectral_gfnet__memory_aug_recurrent_mem_tr__prompt_kernel(
    A_x: jax.Array,
    A_w_r: jax.Array,
    A_w_i: jax.Array,
    B_x: jax.Array,
    B_mem0: jax.Array,
    B_Wq: jax.Array,
    B_Wk: jax.Array,
    B_Wv: jax.Array,
    B_Wo: jax.Array,
    B_seg_len: int,
):
    assert A_x.shape == (1, S, D) and B_x.shape == (1, S, D) and B_mem0.shape == (1, M, D)
    assert B_Wq.shape == (D, H, E) and B_Wo.shape == (H, E, D)
    seg = int(B_seg_len)
    n_seg = S // seg
    assert seg % 16 == 0 and n_seg * seg == S and n_seg % 8 == 0
    mats, tw = _tables()
    vmem = pltpu.VMEM
    out = pl.pallas_call(
        functools.partial(_kernel, seg=seg, n_seg=n_seg),
        out_shape=jax.ShapeDtypeStruct((S, 2 * D), BF16),
        in_specs=[pl.BlockSpec(memory_space=pl.ANY)] * 11,
        out_specs=pl.BlockSpec(memory_space=pl.ANY),
        scratch_shapes=[
            vmem((RS + RD, RD * LANES, LANES), U32),
            vmem((RS, KH + 1, LANES), BF16),
            vmem((RS, KH + 1, LANES), BF16),
            vmem((mats.shape[0] // 2, LANES), U32),
            vmem(tw.shape, F32),
            vmem((RS, 3, LANES, LANES), F32),
            vmem((2, RS, KROWS, LANES), F32),
            vmem((6, D, GROUP // 2, LANES), U32),
            vmem((GROUP, D // 4 + LANES // 2, LANES), U32),
            vmem((GROUP, D // 4, LANES), U32),
            vmem((GROUP, D // 2, LANES), U32),
            vmem((2 * GROUP, D // 2, LANES), U32),
            vmem((2 * GROUP, D // 2, LANES), U32),
            vmem((RD, H * E // 2, LANES), U32),
            vmem((n_seg, seg, D), BF16),
            vmem((M, D), BF16),
            vmem((M + seg, D), F32),
            vmem((S, D), BF16),
            vmem((n_seg, AHEAD, D), BF16),
            vmem((KT, AHEAD * n_seg // 2, LANES), U32),
            vmem((3 * GROUP, AHEAD * n_seg, LANES), F32),
            pltpu.SMEM((32,), jnp.int32),
            pltpu.SemaphoreType.DMA((26,)),
        ],
        compiler_params=pltpu.CompilerParams(vmem_limit_bytes=120 * 1024 * 1024),
        name="gfnet_rmt",
    )(A_x.reshape(S, D), A_w_r.T, A_w_i.T, B_x.reshape(n_seg, seg, D), B_mem0.reshape(M, D),
      B_Wq, B_Wk, B_Wv, B_Wo.reshape(H * E, D), mats, tw)
    return out.reshape(1, S, 2 * D)
```

```python
import functools

import jax
import jax.numpy as jnp
import numpy as np
from jax.experimental import pallas as pl
from jax.experimental.pallas import tpu as pltpu

F32 = jnp.float32
BF16 = jnp.bfloat16
U32 = jnp.uint32

S = 2048
D = 1024
H = 32
E = 128
M = 8
LANES = 128
RS = S // LANES
RD = D // LANES
KH = D // 2
KROWS = KH + 8
K_CLASSES = (0, 4, 1, 7, 2, 6, 5, 3)
_ROOT_NORM = 2.0 ** -10
TW_ROW = 2 * LANES
NYQ_ROW = TW_ROW + 2 * RS
CLASS_SIGN = (-1.0, 1.0)
KT = D // LANES
GROUP = H // 2
AHEAD = 8
AHEAD_PIECES = (0, 1, 3)
UNROLL = 4


@functools.lru_cache(maxsize=None)
def _tables():
    bf16 = jnp.dtype(BF16)
    h = np.sqrt(0.5)
    butterfly = np.array([
        [1, 1, 1, 1, 1, 1, 1, 1],
        [1, -1, 1, -1, 1, -1, 1, -1],
        [1, h, 0, -h, -1, -h, 0, h],
        [0, h, 1, h, 0, -h, -1, -h],
        [1, 0, -1, 0, 1, 0, -1, 0],
        [0, 1, 0, -1, 0, 1, 0, -1],
        [1, -h, 0, h, -1, h, 0, -h],
        [0, -h, 1, -h, 0, h, -1, h],
    ], dtype=np.float64)
    norm = (butterfly ** 2).sum(axis=1)
    d = np.arange(D)
    half = LANES // 2
    mats = []
    for g in range(4):
        k = np.concatenate([K_CLASSES[2 * g + i] + 8 * np.arange(KH // 8) for i in range(2)])
        ang = 2.0 * np.pi * ((k[:, None] * d[None, :]) % D) / D
        rows = np.concatenate([np.cos(ang), -np.sin(ang)]).reshape(2 * LANES, RD, LANES)
        proj = np.einsum("rjd,cj->rcd", rows, butterfly) / norm[None, :, None]
        p, q = proj[:LANES, 2 * g], proj[:LANES, 2 * g + 1]
        r, t = proj[LANES:, 2 * g], proj[LANES:, 2 * g + 1]
        if g == 0:
            mats += [np.concatenate([p[:half], r[:half]]), np.concatenate([q[half:], t[half:]])]
        else:
            sign = np.repeat(CLASS_SIGN, half)[:, None]
            assert np.allclose(t, sign * p) and np.allclose(q, -sign * r)
            mats += [p, r - sign * p, p + sign * r]
    mats = np.concatenate(mats) * _ROOT_NORM
    nyq = np.tile(1.0 - 2.0 * (np.arange(LANES) % 2), (8, 1)) * _ROOT_NORM
    b = np.arange(LANES)
    ang = 2.0 * np.pi * ((b[:, None] * b[None, :]) % LANES) / LANES
    twang = 2.0 * np.pi * (np.arange(RS)[:, None] * b[None, :]) / S
    tw = np.concatenate([np.cos(ang), -np.sin(ang), np.cos(twang), -np.sin(twang), nyq])
    return mats.astype(bf16), tw.astype(np.float32)


def _lo(v):
    return pltpu.bitcast(v << 16, F32)


def _hi(v):
    return pltpu.bitcast(v & np.uint32(0xFFFF0000), F32)


def _pack(lo, hi):
    lo, hi = (pltpu.bitcast(v.astype(BF16).astype(F32), U32) for v in (lo, hi))
    return (lo >> 16) | hi


def _dot(a, b):
    return jnp.dot(a, b, preferred_element_type=F32)


def _dot_nt(a, b):
    return jax.lax.dot_general(a, b, (((1,), (1,)), ((), ())), preferred_element_type=F32)


_H8 = float(np.sqrt(0.5))


def _radix8_fwd(x):
    s04, d04 = x[0] + x[4], x[0] - x[4]
    s26, d26 = x[2] + x[6], x[2] - x[6]
    s15, d15 = x[1] + x[5], x[1] - x[5]
    s37, d37 = x[3] + x[7], x[3] - x[7]
    e0, e1 = s04 + s26, s15 + s37
    p, q = (d15 - d37) * _H8, (d15 + d37) * _H8
    return [e0 + e1, e0 - e1, d04 + p, d26 + q, s04 - s26, s15 - s37, d04 - p, d26 - q]


def _radix8_adj(p):
    e0, e1 = p[0] + p[1], p[0] - p[1]
    s04, s26 = e0 + p[4], e0 - p[4]
    s15, s37 = e1 + p[5], e1 - p[5]
    d04, d26 = p[2] + p[6], p[3] + p[7]
    m, n = (p[2] - p[6]) * _H8, (p[3] - p[7]) * _H8
    d15, d37 = m + n, n - m
    return [s04 + d04, s15 + d15, s26 + d26, s37 + d37,
            s04 - d04, s15 - d15, s26 - d26, s37 - d37]


def _cmul(a, b):
    return a[0] * b[0] - a[1] * b[1], a[0] * b[1] + a[1] * b[0]


def _dft4(z):
    ar, ai = z[0][0] + z[2][0], z[0][1] + z[2][1]
    br, bi = z[0][0] - z[2][0], z[0][1] - z[2][1]
    cr, ci = z[1][0] + z[3][0], z[1][1] + z[3][1]
    dr, di = z[1][0] - z[3][0], z[1][1] - z[3][1]
    return [(ar + cr, ai + ci), (br + di, bi - dr), (ar - cr, ai - ci), (br - di, bi + dr)]


def _rot16(z, n):
    re, im = z
    if n == 0:
        return z
    if n == 4:
        return im, -re
    if n == 2:
        return (re + im) * _H8, (im - re) * _H8
    if n == 6:
        return (im - re) * _H8, (re + im) * (-_H8)
    c, s = float(np.cos(np.pi * n / 8)), float(np.sin(np.pi * n / 8))
    return re * c + im * s, im * c - re * s


def _kernel(ax_hbm, wr_hbm, wi_hbm, bx_hbm, mem_hbm, wq_hbm, wk_hbm, wv_hbm, wo_hbm,
            mats_hbm, tw_hbm, out_hbm,
            ua, wr, wi, mats, tw, ftw, tbuf,
            raw, w_even, w_odd, w_1, w_23, w_45, wo,
            bx, mem0, hbuf, yb, xpre_raw, xpre, pre, zeros, sems, *, seg, n_seg):
    sem_ids = iter(range(sems.shape[0]))

    def copies(pairs):
        sem = sems.at[next(sem_ids)]
        return [pltpu.make_async_copy(src, dst, sem) for src, dst in pairs]

    def start(group, **kwargs):
        for c in group:
            c.start(**kwargs)

    def wait(group):
        for c in group:
            c.wait()

    def col(j):
        return pl.ds(j * LANES, LANES)

    def pipelined(items, first, second, lag):
        pending = []
        for item in items:
            pending.append((item, first(item)))
            if len(pending) > lag:
                second(*pending.pop(0))
        for p in pending:
            second(*p)

    def u_load(a, i, first=0, n=LANES):
        return pltpu.bitcast(ua[a, pl.ds(i * LANES + first, n), :], F32)

    def u_store(a, i, value, first=0):
        ua[a, pl.ds(i * LANES + first, value.shape[0]), :] = pltpu.bitcast(value, U32)

    def piece(p, rows):
        src = (wq_hbm, wk_hbm, wv_hbm)[p % 3].bitcast(U32)
        return src.at[rows, pl.ds(GROUP // 2 * (p // 3), GROUP // 2), :], raw.at[p, rows]

    quarter = S // 8
    cp_tw = copies([(tw_hbm, tw)])
    cp_mats = copies([(mats_hbm.bitcast(U32), mats)])
    cp_tile = [copies([piece(0, col(kt)),
                       (bx_hbm.at[:, pl.ds(seg - AHEAD, AHEAD), col(kt)], xpre_raw.at[kt])])
               for kt in range(KT)]
    cp_ax = [copies([(ax_hbm.bitcast(U32).at[pl.ds(q * quarter, quarter), col(j)],
                      ua.at[RS + j, pl.ds(q * quarter, quarter)]) for j in range(RD)])
             for q in range(4)]
    cp_piece = {p: copies([piece(p, pl.ds(0, D))]) for p in range(1, 6)}
    cp_w = copies([(src.at[:, col(f)], dst.at[f])
                   for src, dst in ((wr_hbm, wr), (wi_hbm, wi)) for f in range(RS)])
    cp_bx0 = copies([(bx_hbm.at[pl.ds(0, UNROLL)], bx.at[pl.ds(0, UNROLL)]), (mem_hbm, mem0)])
    cp_bx1 = copies([(bx_hbm.at[pl.ds(UNROLL, n_seg - UNROLL)],
                      bx.at[pl.ds(UNROLL, n_seg - UNROLL)])])
    cp_wo = copies([(wo_hbm.bitcast(U32).at[:, col(j)], wo.at[j]) for j in range(RD)])
    cp_ya = copies([(ua.at[RS + j], out_hbm.bitcast(U32).at[:, col(j)]) for j in range(RD)])
    yb_sem = sems.at[next(sem_ids)]

    for group in (cp_tw, cp_tile[0], cp_tile[1], cp_tile[2], cp_ax[0], cp_tile[3], cp_tile[4],
                  cp_ax[1], cp_tile[5], cp_tile[6], cp_ax[2], cp_tile[7], cp_mats, cp_ax[3],
                  cp_piece[1]):
        start(group)

    def repack(p, kt, dst, unit, tile):
        src = raw.at[p].reshape(D * GROUP // 2, LANES)
        rows = pl.ds(pl.multiple_of(tile * (LANES // 2), LANES // 2), LANES // 2)
        for hp in range(GROUP // 2):
            v = src[pl.ds(kt * (GROUP // 2 * LANES) + hp, LANES, stride=GROUP // 2), :]
            for par, half in enumerate((v, v >> 16)):
                dst[unit + 2 * hp + par, rows, :] = pltpu.bitcast(half.astype(jnp.uint16), U32)

    def precompute(unit, w):
        x = jnp.concatenate([xpre[kt] for kt in range(KT)], axis=1)
        pre[unit] = _dot(pltpu.bitcast(x, BF16), pltpu.bitcast(w, BF16))

    def clear(unit, carry):
        pre[unit] = jnp.zeros(pre.shape[1:], F32)
        return carry

    jax.lax.fori_loop(0, GROUP, clear, 0)
    for k in range(zeros.shape[0]):
        zeros[k] = 0

    wait(cp_tw)

    def twiddled_dft(a, carry):
        dft = tw[pl.ds(0, LANES), :], tw[pl.ds(LANES, LANES), :]
        re, im = _cmul(dft, (tw[pl.ds(TW_ROW + a, 1), :], tw[pl.ds(TW_ROW + RS + a, 1), :]))
        ftw[a, 0], ftw[a, 1], ftw[a, 2] = re, im - re, im + re
        return carry

    jax.lax.fori_loop(0, RS, twiddled_dft, 0)

    def prepare_tile(kt, dst, tile):
        repack(0, kt, dst, 0, tile)
        xpre[kt] = pltpu.bitcast(xpre_raw[kt].reshape(n_seg * AHEAD, LANES), U32)

    def butterflies(q):
        for ap in range(RS // 2):
            for b in range(0, LANES // 4, 8):
                b = pl.multiple_of(q * (LANES // 4) + b, 8)
                v = [ua[RS + j, pl.ds(ap + 8 * b, 8, stride=8), :] for j in range(RD)]
                for par, half in enumerate((_lo, _hi)):
                    for i, u in enumerate(_radix8_fwd([half(t) for t in v])):
                        u_store(2 * ap + par, i, u, b)

    w_0 = (w_even, w_odd)
    wait(cp_tile[0])
    prepare_tile(0, w_even, 0)

    def first_piece(i, carry):
        for par in range(2):
            kt = 2 * i + par
            for n in range(1 + par, KT, 2):
                pl.when(kt + 1 == n)(functools.partial(wait, cp_tile[n]))
            if par:
                for q in range(4):
                    pl.when(i == q)(functools.partial(wait, cp_ax[q]))
            x = pltpu.bitcast(xpre[kt], BF16)
            rows = pl.ds(pl.multiple_of(i * (LANES // 2), LANES // 2), LANES // 2)
            for unit in range(GROUP):
                pre[unit] += _dot(x, pltpu.bitcast(w_0[par][unit, rows, :], BF16))
            prepare_tile(jnp.minimum(kt + 1, KT - 1), w_0[1 - par], i + par)
            if par:
                butterflies(i)
        return carry

    jax.lax.fori_loop(0, KT // 2, first_piece, 0)

    wait(cp_mats)

    def table(g, i):
        first = 0 if g == 0 else 3 * g - 1
        return pltpu.bitcast(mats[pl.ds((first + i) * (LANES // 2), LANES // 2), :], BF16)

    def forward(ap):
        half = LANES // 2

        def feature_dft(item):
            a, g = item
            if g == 4:
                return _dot_nt(tw[pl.ds(NYQ_ROW, 8), :], u_load(a, 0))
            u0, u1 = u_load(a, 2 * g), u_load(a, 2 * g + 1)
            if g == 0:
                y0, y1 = _dot_nt(table(0, 0), u0), _dot_nt(table(0, 1), u1)
                return (jnp.concatenate([y0[:half], y1[:half]], axis=0),
                        jnp.concatenate([y0[half:], y1[half:]], axis=0))
            both = _dot_nt(table(g, 0), u0 + u1)
            im = _dot_nt(table(g, 1), u0)
            re = both - _dot_nt(table(g, 2), u1)
            return re, jnp.concatenate([im[:half] - both[:half], im[half:] + both[half:]], axis=0)

        def sequence_dft(item, y):
            a, g = item
            if g == 4:
                rows = pl.ds(KH, 8)
                both = _dot(y, ftw[a, 0])
                re, im = both, both + _dot(y, ftw[a, 1])
            else:
                rows = pl.ds(g * LANES, LANES)
                both = _dot(y[0] + y[1], ftw[a, 0])
                re, im = both - _dot(y[1], ftw[a, 2]), both + _dot(y[0], ftw[a, 1])
            tbuf[0, a, rows, :], tbuf[1, a, rows, :] = re, im

        pipelined([(2 * ap + par, g) for par in range(2) for g in range(5)],
                  feature_dft, sequence_dft, 2)

    def forward_first(ap, carry):
        forward(ap)
        return carry

    def forward_second(i, carry):
        for kt in range(2):
            repack(1, 2 * i + kt, w_1, 0, 2 * i + kt)
        forward(RS // 4 + i)
        return carry

    jax.lax.fori_loop(0, RS // 4, forward_first, 0)
    wait(cp_piece[1])
    for group in (cp_w, *(cp_piece[p] for p in range(2, 6)), cp_bx0):
        start(group)
    start(cp_wo, priority=1)
    jax.lax.fori_loop(0, RS // 4, forward_second, 0)

    def load(slots, rows):
        return [(tbuf[0, a, rows, :], tbuf[1, a, rows, :]) for a in slots]

    def store(slots, rows, z):
        for a, v in zip(slots, z):
            tbuf[0, a, rows, :], tbuf[1, a, rows, :] = v

    def swap(z):
        return [(im, re) for re, im in z]

    def rotate(z, n):
        return [_rot16(v, n * k) for k, v in enumerate(z)]

    def columns(n):
        return range(n, RS, 4)

    def lines(n):
        return range(4 * n, 4 * n + 4)

    passes = (
        (columns, lambda z, n, filt: rotate(_dft4(z), n)),
        (lines, lambda z, n, filt: [_cmul(v, filt(n + 4 * k)) for k, v in enumerate(_dft4(z))]),
        (lines, lambda z, n, filt: rotate(_dft4(swap(z)), n)),
        (columns, lambda z, n, filt: swap(_dft4(z))),
    )

    def run_pass(index, row, filt, link):
        slots, step = passes[index]
        for half in range(2):
            rows = pl.ds(pl.multiple_of(row + zeros[(2 * link + half) % zeros.shape[0]], 8), 8)
            group = (2 * half, 2 * half + 1)
            z = [load(slots(n), rows) for n in group]
            for n, v in zip(group, z):
                store(slots(n), rows, step(v, n, filt))

    def filter_rows(cls, mb, f):
        block = pl.ds(pl.multiple_of(32 * mb, 32), 32)
        half, src = (_lo, _hi)[cls % 2], pl.ds(cls // 2, 8, stride=4)
        re, im = (half(ref.at[:, pl.ds(0, KH), :].bitcast(U32).at[f, block][src, :])
                  for ref in (wr, wi))
        if cls == 0:
            row = jax.lax.broadcasted_iota(jnp.int32, (8, LANES), 0)
            weight = jnp.where(row + mb == 0, 0.5, 1.0)
            re, im = re * weight, im * weight
        return re, im

    def filter_nyquist(f):
        return tuple(jnp.broadcast_to(ref[f, pl.ds(KH, 1), :].astype(F32), (8, LANES))
                     for ref in (wr, wi))

    for index in range(4):
        if index == 1:
            wait(cp_w)

        def middle(i, carry, index=index):
            for unit in (4 * index + 2 * i, 4 * index + 2 * i + 1):
                precompute(GROUP + unit, w_1[unit])
            for n in range(4):
                mb = 4 * i + n
                for cls in range(8):
                    run_pass(index, 64 * K_CLASSES.index(cls) + 8 * mb,
                             functools.partial(filter_rows, cls, mb), 8 * n + cls)
            return carry

        jax.lax.fori_loop(0, 2, middle, 0)
        run_pass(index, KH, filter_nyquist, 0)

    def inverse(ap, carry):
        for p in (2, 3):
            repack(p, ap, w_23, GROUP * (p - 2), ap)

        def sequence_idft(item):
            a, g, _ = item
            if g == 4:
                re, im = (jnp.concatenate([tbuf[i, a, pl.ds(KH, 8), :]] * (LANES // 8), axis=0)
                          for i in range(2))
                return _dot_nt(ftw[a, 0], re + im) + _dot_nt(ftw[a, 1], im)
            rows = pl.ds(g * LANES, LANES)
            re, im = tbuf[0, a, rows, :], tbuf[1, a, rows, :]
            both = _dot_nt(ftw[a, 0], re + im)
            return both + _dot_nt(ftw[a, 1], im), both - _dot_nt(ftw[a, 2], re)

        nyquist = {}
        low = jax.lax.broadcasted_iota(jnp.int32, (LANES, LANES), 1) < LANES // 2

        def feature_idft(item, v):
            a, g, par = item
            if g == 4:
                nyquist[par] = v * (0.5 * tw[pl.ds(NYQ_ROW, 1), :])
            elif g == 0:
                re, im = v
                v0 = jnp.where(low, re, pltpu.roll(im, LANES // 2, 1))
                v1 = jnp.where(low, pltpu.roll(re, LANES // 2, 1), im)
                u_store(a, 0, _dot(v0, table(0, 0)) + nyquist.pop(par))
                u_store(a, 1, _dot(v1, table(0, 1)))
            else:
                re, im = v
                both = _dot(jnp.where(low, re - im, re + im), table(g, 0))
                u_store(a, 2 * g, both + _dot(im, table(g, 1)))
                u_store(a, 2 * g + 1, both - _dot(re, table(g, 2)))

        pipelined([(2 * ap + par, g, par) for par in range(2) for g in (4, 0, 1, 2, 3)],
                  sequence_idft, feature_idft, 3)
        return carry

    wait(cp_piece[2])
    wait(cp_piece[3])
    jax.lax.fori_loop(0, RS // 2, inverse, 0)

    def last_pieces(ap, carry):
        for p in (4, 5):
            pl.when(ap == 4 * (p - 4))(functools.partial(wait, cp_piece[p]))
        for unit in (2 * ap, 2 * ap + 1):
            precompute(2 * GROUP + unit, w_23[GROUP + unit])
        for j in (2 * ap, 2 * ap + 1):
            repack(4 + j // KT, j % KT, w_45, GROUP * (j // KT), j % KT)
        for b in range(0, LANES, 8):
            y = [_radix8_adj([u_load(2 * ap + par, i, b, 8) for i in range(RD)])
                 for par in range(2)]
            for j in range(RD):
                ua[RS + j, pl.ds(ap + 8 * b, 8, stride=8), :] = _pack(y[0][j], y[1][j])
        return carry

    jax.lax.fori_loop(0, RS // 2, last_pieces, 0)

    L = M + seg
    scale = E ** -0.5
    mem_rows = pl.ds(seg, M)

    def segment(s):
        hbuf[pl.ds(0, seg), :] = bx[s].astype(F32)
        qi = jax.lax.broadcasted_iota(jnp.int32, (L, L), 0)
        ki = jax.lax.broadcasted_iota(jnp.int32, (L, L), 1)
        mask = (qi >= seg) | (ki >= seg) | (qi >= ki)
        qkv, probs, ctx = {}, {}, {}

        def project(h, m):
            p, i = 3 * (h // GROUP) + m, h % GROUP
            if p == 0:
                w = jnp.concatenate(
                    [w_0[kt % 2][i, pl.ds(kt // 2 * (LANES // 2), LANES // 2), :]
                     for kt in range(KT)], axis=0)
            else:
                w = w_1[i] if p == 1 else (w_23, w_45)[p // 2 - 1][GROUP * (p % 2) + i]
            w = pltpu.bitcast(w, BF16)
            if p not in AHEAD_PIECES or (h, m) == (0, 0):
                return _dot(hbuf[...], w)
            unit = GROUP * AHEAD_PIECES.index(p) + i
            x = jnp.concatenate([hbuf[pl.ds(0, seg - AHEAD), :], hbuf[mem_rows, :]], axis=0)
            r = _dot(x, w)
            done = pre[unit, pl.ds(pl.multiple_of(AHEAD * s, AHEAD), AHEAD), :]
            return jnp.concatenate([r[:seg - AHEAD], done, r[seg - AHEAD:]], axis=0)

        def scores(h):
            q, k, v = qkv.pop(h)
            sc = jnp.where(mask, _dot_nt(q, k) * scale, -1000000000.0)
            e = jnp.exp(sc - jnp.max(sc, axis=-1, keepdims=True))
            probs[h] = e, jnp.sum(e, axis=-1, keepdims=True), v

        def mix(h):
            e, total, v = probs.pop(h)
            o = _dot(e, v) * (1.0 / total)
            ctx[h] = jnp.concatenate([o[seg:], o[:seg]], axis=0)

        def output(h):
            rows = pl.ds(h * (E // 2), E // 2)
            w = jnp.concatenate([wo[j, rows, :] for j in range(RD)], axis=1)
            return _dot(ctx.pop(h), pltpu.bitcast(w, BF16))

        lag_scores, lag_mix, lag_output = 2, 6, 8
        acc = None
        for t in range(H + lag_output):
            if t < H:
                qkv[t] = [project(t, 0)]
            if 0 <= t - lag_scores < H:
                scores(t - lag_scores)
            if t < H:
                qkv[t].append(project(t, 1))
            if 0 <= t - lag_mix < H:
                mix(t - lag_mix)
            if t < H:
                qkv[t].append(project(t, 2))
            if 0 <= t - lag_output < H:
                y = output(t - lag_output)
                acc = y if acc is None else acc + y
        hbuf[mem_rows, :] = acc[:M]
        yb[pl.ds(pl.multiple_of(s * seg, seg), seg), :] = acc[M:].astype(BF16)

    def yb_copy(i):
        rows = pl.ds(pl.multiple_of(i * (UNROLL * seg), UNROLL * seg), UNROLL * seg)
        return pltpu.make_async_copy(yb.at[rows], out_hbm.at[rows, pl.ds(D, D)], yb_sem)

    wait(cp_bx0)
    wait(cp_wo)
    hbuf[mem_rows, :] = mem0[...].astype(F32)
    start(cp_bx1)
    start(cp_ya)

    def segments(i, carry):
        pl.when(i == 1)(functools.partial(wait, cp_bx1))

        @pl.when(i > 0)
        def _():
            yb_copy(i - 1).start()

        for u in range(UNROLL):
            segment(UNROLL * i + u)
        return carry

    jax.lax.fori_loop(0, n_seg // UNROLL, segments, 0)
    yb_copy(n_seg // UNROLL - 1).start()
    wait(cp_ya)
    pltpu.make_async_copy(yb, out_hbm.at[:, pl.ds(D, D)], yb_sem).wait()


@functools.partial(jax.jit, static_argnames=("B_seg_len",))
def pallas_concat_heads__spectral_gfnet__memory_aug_recurrent_mem_tr__prompt_kernel(
    A_x: jax.Array,
    A_w_r: jax.Array,
    A_w_i: jax.Array,
    B_x: jax.Array,
    B_mem0: jax.Array,
    B_Wq: jax.Array,
    B_Wk: jax.Array,
    B_Wv: jax.Array,
    B_Wo: jax.Array,
    B_seg_len: int,
):
    assert A_x.shape == (1, S, D) and B_x.shape == (1, S, D) and B_mem0.shape == (1, M, D)
    assert B_Wq.shape == (D, H, E) and B_Wo.shape == (H, E, D)
    seg = int(B_seg_len)
    n_seg = S // seg
    assert seg % 16 == 0 and n_seg * seg == S and n_seg % 8 == 0
    mats, tw = _tables()
    vmem = pltpu.VMEM
    out = pl.pallas_call(
        functools.partial(_kernel, seg=seg, n_seg=n_seg),
        out_shape=jax.ShapeDtypeStruct((S, 2 * D), BF16),
        in_specs=[pl.BlockSpec(memory_space=pl.ANY)] * 11,
        out_specs=pl.BlockSpec(memory_space=pl.ANY),
        scratch_shapes=[
            vmem((RS + RD, RD * LANES, LANES), U32),
            vmem((RS, KH + 1, LANES), BF16),
            vmem((RS, KH + 1, LANES), BF16),
            vmem((mats.shape[0] // 2, LANES), U32),
            vmem(tw.shape, F32),
            vmem((RS, 3, LANES, LANES), F32),
            vmem((2, RS, KROWS, LANES), F32),
            vmem((6, D, GROUP // 2, LANES), U32),
            vmem((GROUP, D // 4 + LANES // 2, LANES), U32),
            vmem((GROUP, D // 4, LANES), U32),
            vmem((GROUP, D // 2, LANES), U32),
            vmem((2 * GROUP, D // 2, LANES), U32),
            vmem((2 * GROUP, D // 2, LANES), U32),
            vmem((RD, H * E // 2, LANES), U32),
            vmem((n_seg, seg, D), BF16),
            vmem((M, D), BF16),
            vmem((M + seg, D), F32),
            vmem((S, D), BF16),
            vmem((KT, n_seg, AHEAD, LANES), BF16),
            vmem((KT, AHEAD * n_seg // 2, LANES), U32),
            vmem((3 * GROUP, AHEAD * n_seg, LANES), F32),
            pltpu.SMEM((32,), jnp.int32),
            pltpu.SemaphoreType.DMA((26,)),
        ],
        compiler_params=pltpu.CompilerParams(vmem_limit_bytes=120 * 1024 * 1024),
        name="gfnet_rmt",
    )(A_x.reshape(S, D), A_w_r.T, A_w_i.T, B_x.reshape(n_seg, seg, D), B_mem0.reshape(M, D),
      B_Wq, B_Wk, B_Wv, B_Wo.reshape(H * E, D), mats, tw)
    return out.reshape(1, S, 2 * D)
```

```python
import functools

import jax
import jax.numpy as jnp
import numpy as np
from jax.experimental import pallas as pl
from jax.experimental.pallas import tpu as pltpu

F32 = jnp.float32
BF16 = jnp.bfloat16
U32 = jnp.uint32

S = 2048
D = 1024
H = 32
E = 128
M = 8
LANES = 128
RS = S // LANES
RD = D // LANES
KH = D // 2
KROWS = KH + 8
K_CLASSES = (0, 4, 1, 7, 2, 6, 5, 3)
_ROOT_NORM = 2.0 ** -10
TW_ROW = 2 * LANES
NYQ_ROW = TW_ROW + 2 * RS
CLASS_SIGN = (-1.0, 1.0)
KT = D // LANES
GROUP = H // 2
PIECES = ((2, 0), (0, 0), (1, 0), (2, 1), (0, 1), (1, 1))
UNROLL = 4


@functools.lru_cache(maxsize=None)
def _tables():
    bf16 = jnp.dtype(BF16)
    h = np.sqrt(0.5)
    butterfly = np.array([
        [1, 1, 1, 1, 1, 1, 1, 1],
        [1, -1, 1, -1, 1, -1, 1, -1],
        [1, h, 0, -h, -1, -h, 0, h],
        [0, h, 1, h, 0, -h, -1, -h],
        [1, 0, -1, 0, 1, 0, -1, 0],
        [0, 1, 0, -1, 0, 1, 0, -1],
        [1, -h, 0, h, -1, h, 0, -h],
        [0, -h, 1, -h, 0, h, -1, h],
    ], dtype=np.float64)
    norm = (butterfly ** 2).sum(axis=1)
    d = np.arange(D)
    half = LANES // 2
    mats = []
    for g in range(4):
        k = np.concatenate([K_CLASSES[2 * g + i] + 8 * np.arange(KH // 8) for i in range(2)])
        ang = 2.0 * np.pi * ((k[:, None] * d[None, :]) % D) / D
        rows = np.concatenate([np.cos(ang), -np.sin(ang)]).reshape(2 * LANES, RD, LANES)
        proj = np.einsum("rjd,cj->rcd", rows, butterfly) / norm[None, :, None]
        p, q = proj[:LANES, 2 * g], proj[:LANES, 2 * g + 1]
        r, t = proj[LANES:, 2 * g], proj[LANES:, 2 * g + 1]
        if g == 0:
            mats += [np.concatenate([p[:half], r[:half]]), np.concatenate([q[half:], t[half:]])]
        else:
            sign = np.repeat(CLASS_SIGN, half)[:, None]
            assert np.allclose(t, sign * p) and np.allclose(q, -sign * r)
            mats += [p, r - sign * p, p + sign * r]
    mats = np.concatenate(mats) * _ROOT_NORM
    nyq = np.tile(1.0 - 2.0 * (np.arange(LANES) % 2), (8, 1)) * _ROOT_NORM
    b = np.arange(LANES)
    ang = 2.0 * np.pi * ((b[:, None] * b[None, :]) % LANES) / LANES
    twang = 2.0 * np.pi * (np.arange(RS)[:, None] * b[None, :]) / S
    tw = np.concatenate([np.cos(ang), -np.sin(ang), np.cos(twang), -np.sin(twang), nyq])
    return mats.astype(bf16), tw.astype(np.float32)


def _lo(v):
    return pltpu.bitcast(v << 16, F32)


def _hi(v):
    return pltpu.bitcast(v & np.uint32(0xFFFF0000), F32)


def _pack(lo, hi):
    lo, hi = (pltpu.bitcast(v.astype(BF16).astype(F32), U32) for v in (lo, hi))
    return (lo >> 16) | hi


def _dot(a, b):
    return jnp.dot(a, b, preferred_element_type=F32)


def _dot_nt(a, b):
    return jax.lax.dot_general(a, b, (((1,), (1,)), ((), ())), preferred_element_type=F32)


_H8 = float(np.sqrt(0.5))


def _radix8_fwd(x):
    s04, d04 = x[0] + x[4], x[0] - x[4]
    s26, d26 = x[2] + x[6], x[2] - x[6]
    s15, d15 = x[1] + x[5], x[1] - x[5]
    s37, d37 = x[3] + x[7], x[3] - x[7]
    e0, e1 = s04 + s26, s15 + s37
    p, q = (d15 - d37) * _H8, (d15 + d37) * _H8
    return [e0 + e1, e0 - e1, d04 + p, d26 + q, s04 - s26, s15 - s37, d04 - p, d26 - q]


def _radix8_adj(p):
    e0, e1 = p[0] + p[1], p[0] - p[1]
    s04, s26 = e0 + p[4], e0 - p[4]
    s15, s37 = e1 + p[5], e1 - p[5]
    d04, d26 = p[2] + p[6], p[3] + p[7]
    m, n = (p[2] - p[6]) * _H8, (p[3] - p[7]) * _H8
    d15, d37 = m + n, n - m
    return [s04 + d04, s15 + d15, s26 + d26, s37 + d37,
            s04 - d04, s15 - d15, s26 - d26, s37 - d37]


def _cmul(a, b):
    return a[0] * b[0] - a[1] * b[1], a[0] * b[1] + a[1] * b[0]


def _dft4(z):
    ar, ai = z[0][0] + z[2][0], z[0][1] + z[2][1]
    br, bi = z[0][0] - z[2][0], z[0][1] - z[2][1]
    cr, ci = z[1][0] + z[3][0], z[1][1] + z[3][1]
    dr, di = z[1][0] - z[3][0], z[1][1] - z[3][1]
    return [(ar + cr, ai + ci), (br + di, bi - dr), (ar - cr, ai - ci), (br - di, bi + dr)]


def _rot16(z, n):
    re, im = z
    if n == 0:
        return z
    if n == 4:
        return im, -re
    if n == 2:
        return (re + im) * _H8, (im - re) * _H8
    if n == 6:
        return (im - re) * _H8, (re + im) * (-_H8)
    c, s = float(np.cos(np.pi * n / 8)), float(np.sin(np.pi * n / 8))
    return re * c + im * s, im * c - re * s


def _kernel(ax_hbm, wr_hbm, wi_hbm, bx_hbm, mem_hbm, wq_hbm, wk_hbm, wv_hbm, wo_hbm,
            mats_hbm, tw_hbm, out_hbm,
            ua, wr, wi, mats, tw, ftw, tbuf,
            raw, w_v0, w_qk0, pool_a, pool_b, wo,
            bx, mem0, hbuf, hsum, yb, tokens, xs, pre_v0, zeros, sems, *, seg, n_seg):
    sem_ids = iter(range(sems.shape[0]))
    w_v1, w_q1 = pool_a.at[pl.ds(0, GROUP)], pool_a.at[pl.ds(GROUP, GROUP)]
    pre_qk0 = pool_a.at[pl.ds(2 * GROUP, 2 * GROUP)]
    w_k1, pre_v1 = pool_b.at[pl.ds(0, GROUP)], pool_b.at[pl.ds(GROUP, GROUP)]

    def copies(pairs):
        sem = sems.at[next(sem_ids)]
        return [pltpu.make_async_copy(src, dst, sem) for src, dst in pairs]

    def start(group, **kwargs):
        for c in group:
            c.start(**kwargs)

    def wait(group):
        for c in group:
            c.wait()

    def col(j):
        return pl.ds(j * LANES, LANES)

    def pipelined(items, first, second, lag):
        pending = []
        for item in items:
            pending.append((item, first(item)))
            if len(pending) > lag:
                second(*pending.pop(0))
        for p in pending:
            second(*p)

    def u_load(a, i, first=0, n=LANES):
        return pltpu.bitcast(ua[a, pl.ds(i * LANES + first, n), :], F32)

    def u_store(a, i, value, first=0):
        ua[a, pl.ds(i * LANES + first, value.shape[0]), :] = pltpu.bitcast(value, U32)

    def piece(p):
        m, g = PIECES[p]
        src = (wq_hbm, wk_hbm, wv_hbm)[m].bitcast(U32)
        return src.at[:, pl.ds(GROUP // 2 * g, GROUP // 2), :], raw.at[p]

    quarter = S // 8
    cp_tables = copies([(tw_hbm, tw), (mats_hbm.bitcast(U32), mats)])
    cp_ax = [copies([(ax_hbm.bitcast(U32).at[pl.ds(q * quarter, quarter), col(j)],
                      ua.at[RS + j, pl.ds(q * quarter, quarter)]) for j in range(RD)])
             for q in range(4)]
    cp_piece = [copies([piece(p)]) for p in range(6)]
    cp_tokens = copies([(bx_hbm.at[:, pl.ds(seg - 16, 16), :], tokens)])
    cp_w = copies([(src.at[:, col(f)], dst.at[f])
                   for src, dst in ((wr_hbm, wr), (wi_hbm, wi)) for f in range(RS)])
    cp_bx0 = copies([(bx_hbm.at[pl.ds(0, UNROLL)], bx.at[pl.ds(0, UNROLL)]), (mem_hbm, mem0)])
    cp_bx1 = copies([(bx_hbm.at[pl.ds(UNROLL, n_seg - UNROLL)],
                      bx.at[pl.ds(UNROLL, n_seg - UNROLL)])])
    cp_wo = copies([(wo_hbm.bitcast(U32).at[:, col(j)], wo.at[j]) for j in range(RD)])
    cp_ya = copies([(ua.at[RS + j], out_hbm.bitcast(U32).at[:, col(j)]) for j in range(RD)])
    yb_sem = sems.at[next(sem_ids)]

    for group in (cp_tables, *cp_ax, cp_piece[0], cp_tokens):
        start(group)
    for k in range(zeros.shape[0]):
        zeros[k] = 0

    def words(p, kt, hp):
        src = raw.at[p].reshape(D * GROUP // 2, LANES)
        return src[pl.ds(kt * (GROUP // 2 * LANES) + hp, LANES, stride=GROUP // 2), :]

    def put(dst, head, kt, v):
        rows = pl.ds(pl.multiple_of(kt * (LANES // 2), LANES // 2), LANES // 2)
        dst[head, rows, :] = pltpu.bitcast(v, U32)

    def repack(p, kt, dst, pairs=range(GROUP // 2)):
        for hp in pairs:
            v = words(p, kt, hp)
            for par in range(2):
                put(dst, 2 * hp + par, kt, (v >> (16 * par)).astype(jnp.uint16))

    def repack_right(p, j, pairs, dst, is_right):
        for hp in pairs:
            v = [words(p, j, hp), words(p, j + KT // 2, hp)]
            for par, half in enumerate((_lo, _hi)):
                put(dst, 2 * hp + par, j + KT // 2, (v[1] >> (16 * par)).astype(jnp.uint16))
                if is_right[par]:
                    put(dst, 2 * hp + par, j, (half(v[0]) - half(v[1])).astype(BF16))
                else:
                    put(dst, 2 * hp + par, j, (v[0] >> (16 * par)).astype(jnp.uint16))

    def token_sums(j, carry):
        n = n_seg // 4
        v = tokens[pl.ds(j * n, n)].astype(F32)
        top, bottom = v[:, :8].reshape(8 * n, D), v[:, 8:].reshape(8 * n, D)
        rows = pl.ds(pl.multiple_of(j * (4 * n), 4 * n), 4 * n)
        s1 = bottom[:, :KH] + bottom[:, KH:]
        for i, x in enumerate((bottom[:, KH:], s1, s1 - top[:, :KH])):
            xs[i, rows, :] = pltpu.bitcast(x.astype(BF16), U32)
        return carry

    def precompute(left, right, dst, at, beside=()):
        b11, b21, t3, b22 = (pltpu.bitcast(v, BF16).astype(F32) for v in (
            left[:KH // 2], left[KH // 2:], right[:KH // 2], right[KH // 2:]))
        t2 = b11 - t3
        beside = list(beside)
        for i, w in ((2, t2), (1, b22 - t2), (0, t2 - b21)):
            p = _dot(pltpu.bitcast(xs[i], BF16), w)
            if beside:
                beside.pop(0)()
            if i == 2:
                dst[at(0)] = dst[at(1)] = pltpu.bitcast(p, U32)
            elif i == 1:
                dst[at(0)] = pltpu.bitcast(pltpu.bitcast(dst[at(0)], F32) + p, U32)
            else:
                dst[at(1)] = pltpu.bitcast(pltpu.bitcast(dst[at(1)], F32) - p, U32)

    wait(cp_tables)

    def twiddled_dft(a, carry):
        dft = tw[pl.ds(0, LANES), :], tw[pl.ds(LANES, LANES), :]
        re, im = _cmul(dft, (tw[pl.ds(TW_ROW + a, 1), :], tw[pl.ds(TW_ROW + RS + a, 1), :]))
        ftw[a, 0], ftw[a, 1], ftw[a, 2] = re, im - re, im + re
        return carry

    jax.lax.fori_loop(0, RS, twiddled_dft, 0)
    for q in range(4):
        wait(cp_ax[q])

        def butterflies(ap, carry, q=q):
            blocks = range(q * LANES // 4, (q + 1) * LANES // 4, 8)
            x = [[ua[RS + j, pl.ds(ap + 8 * b, 8, stride=8), :] for j in range(RD)]
                 for b in blocks]
            for b, v in zip(blocks, x):
                for par, half in enumerate((_lo, _hi)):
                    for i, u in enumerate(_radix8_fwd([half(t) for t in v])):
                        u_store(2 * ap + par, i, u, b)
            return carry

        jax.lax.fori_loop(0, RS // 2, butterflies, 0)

    def table(g, i):
        first = 0 if g == 0 else 3 * g - 1
        return pltpu.bitcast(mats[pl.ds((first + i) * (LANES // 2), LANES // 2), :], BF16)

    def forward(ap):
        half = LANES // 2

        def feature_dft(item):
            a, g = item
            if g == 4:
                return _dot_nt(tw[pl.ds(NYQ_ROW, 8), :], u_load(a, 0))
            u0, u1 = u_load(a, 2 * g), u_load(a, 2 * g + 1)
            if g == 0:
                y0, y1 = _dot_nt(table(0, 0), u0), _dot_nt(table(0, 1), u1)
                return (jnp.concatenate([y0[:half], y1[:half]], axis=0),
                        jnp.concatenate([y0[half:], y1[half:]], axis=0))
            both = _dot_nt(table(g, 0), u0 + u1)
            im = _dot_nt(table(g, 1), u0)
            re = both - _dot_nt(table(g, 2), u1)
            return re, jnp.concatenate([im[:half] - both[:half], im[half:] + both[half:]], axis=0)

        def sequence_dft(item, y):
            a, g = item
            if g == 4:
                rows = pl.ds(KH, 8)
                both = _dot(y, ftw[a, 0])
                re, im = both, both + _dot(y, ftw[a, 1])
            else:
                rows = pl.ds(g * LANES, LANES)
                both = _dot(y[0] + y[1], ftw[a, 0])
                re, im = both - _dot(y[1], ftw[a, 2]), both + _dot(y[0], ftw[a, 1])
            tbuf[0, a, rows, :], tbuf[1, a, rows, :] = re, im

        pipelined([(2 * ap + par, g) for par in range(2) for g in range(5)],
                  feature_dft, sequence_dft, 2)

    def forward_first(ap, carry):
        forward(ap)
        return carry

    def forward_second(i, carry):
        repack_right(0, i, range(GROUP // 2), w_v0, (False, True))
        forward(RS // 4 + i)
        return carry

    jax.lax.fori_loop(0, RS // 4, forward_first, 0)
    wait(cp_piece[0])
    for group in (cp_w, *cp_piece[1:], cp_bx0):
        start(group)
    start(cp_wo, priority=1)
    jax.lax.fori_loop(0, RS // 4, forward_second, 0)
    wait(cp_tokens)
    jax.lax.fori_loop(0, 4, token_sums, 0)

    def load(slots, rows):
        return [(tbuf[0, a, rows, :], tbuf[1, a, rows, :]) for a in slots]

    def store(slots, rows, z):
        for a, v in zip(slots, z):
            tbuf[0, a, rows, :], tbuf[1, a, rows, :] = v

    def swap(z):
        return [(im, re) for re, im in z]

    def rotate(z, n):
        return [_rot16(v, n * k) for k, v in enumerate(z)]

    def columns(n):
        return range(n, RS, 4)

    def lines(n):
        return range(4 * n, 4 * n + 4)

    passes = (
        (columns, lambda z, n, filt: rotate(_dft4(z), n)),
        (lines, lambda z, n, filt: [_cmul(v, filt(n + 4 * k)) for k, v in enumerate(_dft4(z))]),
        (lines, lambda z, n, filt: rotate(_dft4(swap(z)), n)),
        (columns, lambda z, n, filt: swap(_dft4(z))),
    )

    def run_pass(index, row, filt, link):
        slots, step = passes[index]
        for half in range(2):
            rows = pl.ds(pl.multiple_of(row + zeros[(2 * link + half) % zeros.shape[0]], 8), 8)
            group = (2 * half, 2 * half + 1)
            z = [load(slots(n), rows) for n in group]
            for n, v in zip(group, z):
                store(slots(n), rows, step(v, n, filt))

    def filter_rows(cls, mb, f):
        block = pl.ds(pl.multiple_of(32 * mb, 32), 32)
        half, src = (_lo, _hi)[cls % 2], pl.ds(cls // 2, 8, stride=4)
        re, im = (half(ref.at[:, pl.ds(0, KH), :].bitcast(U32).at[f, block][src, :])
                  for ref in (wr, wi))
        if cls == 0:
            row = jax.lax.broadcasted_iota(jnp.int32, (8, LANES), 0)
            weight = jnp.where(row + mb == 0, 0.5, 1.0)
            re, im = re * weight, im * weight
        return re, im

    def filter_nyquist(f):
        return tuple(jnp.broadcast_to(ref[f, pl.ds(KH, 1), :].astype(F32), (8, LANES))
                     for ref in (wr, wi))

    for index in range(4):
        if index == 1:
            wait(cp_w)

        def middle(i, carry, index=index):
            pair = 2 * index + i
            precompute(w_v0[2 * pair], w_v0[2 * pair + 1], pre_v0, lambda n: 2 * pair + n)
            for n in range(4):
                mb = 4 * i + n
                for cls in range(8):
                    run_pass(index, 64 * K_CLASSES.index(cls) + 8 * mb,
                             functools.partial(filter_rows, cls, mb), 8 * n + cls)
            return carry

        jax.lax.fori_loop(0, 2, middle, 0)
        run_pass(index, KH, filter_nyquist, 0)

    def inverse(ap, carry):
        repack(1, ap, w_qk0.at[0])
        repack_right(2, ap // 2, [4 * (ap % 2) + hp for hp in range(4)], w_qk0.at[1], (True, True))

        def sequence_idft(item):
            a, g, _ = item
            if g == 4:
                re, im = (jnp.concatenate([tbuf[i, a, pl.ds(KH, 8), :]] * (LANES // 8), axis=0)
                          for i in range(2))
                return _dot_nt(ftw[a, 0], re + im) + _dot_nt(ftw[a, 1], im)
            rows = pl.ds(g * LANES, LANES)
            re, im = tbuf[0, a, rows, :], tbuf[1, a, rows, :]
            both = _dot_nt(ftw[a, 0], re + im)
            return both + _dot_nt(ftw[a, 1], im), both - _dot_nt(ftw[a, 2], re)

        nyquist = {}
        low = jax.lax.broadcasted_iota(jnp.int32, (LANES, LANES), 1) < LANES // 2

        def feature_idft(item, v):
            a, g, par = item
            if g == 4:
                nyquist[par] = v * (0.5 * tw[pl.ds(NYQ_ROW, 1), :])
            elif g == 0:
                re, im = v
                v0 = jnp.where(low, re, pltpu.roll(im, LANES // 2, 1))
                v1 = jnp.where(low, pltpu.roll(re, LANES // 2, 1), im)
                u_store(a, 0, _dot(v0, table(0, 0)) + nyquist.pop(par))
                u_store(a, 1, _dot(v1, table(0, 1)))
            else:
                re, im = v
                both = _dot(jnp.where(low, re - im, re + im), table(g, 0))
                u_store(a, 2 * g, both + _dot(im, table(g, 1)))
                u_store(a, 2 * g + 1, both - _dot(re, table(g, 2)))

        pipelined([(2 * ap + par, g, par) for par in range(2) for g in (4, 0, 1, 2, 3)],
                  sequence_idft, feature_idft, 3)
        return carry

    wait(cp_piece[1])
    wait(cp_piece[2])
    jax.lax.fori_loop(0, RS // 2, inverse, 0)

    def adjoint(ap):
        for b in range(0, LANES, 8):
            y = [_radix8_adj([u_load(2 * ap + par, n, b, 8) for n in range(RD)])
                 for par in range(2)]
            for j in range(RD):
                ua[RS + j, pl.ds(ap + 8 * b, 8, stride=8), :] = _pack(y[0][j], y[1][j])

    def finish(ap, carry):
        def v_part(hp):
            return functools.partial(repack_right, 3, ap // 2, [4 * (ap % 2) + i for i in hp],
                                     w_v1, (False, True))

        def q_part(hp):
            return functools.partial(repack, 4, ap, w_q1, hp)

        work = ([v_part((0, 1)), v_part((2,)), v_part((3,))],
                [q_part((0, 1, 2)), q_part((3, 4, 5)), q_part((6, 7))])
        adjoint(ap)
        for n in range(2):
            h = 2 * ap + n
            precompute(w_qk0[0, h], w_qk0[1, h], pre_qk0, lambda i: 2 * h + i, work[n])
        return carry

    wait(cp_piece[3])
    wait(cp_piece[4])
    jax.lax.fori_loop(0, RS // 2, finish, 0)

    def last_piece(i, carry):
        for n in range(2):
            pair = 2 * i + n
            work = [functools.partial(repack_right, 5, i, [4 * n + j for j in hp], w_k1,
                                      (True, True)) for hp in ((0, 1), (2,), (3,))]
            precompute(w_v1[2 * pair], w_v1[2 * pair + 1], pre_v1, lambda j: 2 * pair + j, work)
        return carry

    wait(cp_piece[5])
    jax.lax.fori_loop(0, 4, last_piece, 0)

    def late(h):
        return raw.at[h // 8].reshape(D * GROUP // 2, LANES)

    def late_rows(h, i, first, n):
        return pl.ds(pl.multiple_of((2 * (h % 8) + i) * (8 * n_seg) + first, 8), n)

    def last_pairs(i, carry):
        for h in (2 * i, 2 * i + 1):
            precompute(w_q1[h], w_k1[h], late(h), lambda n: late_rows(h, n, 0, 8 * n_seg))
        return carry

    jax.lax.fori_loop(0, GROUP // 2, last_pairs, 0)

    L = M + seg
    scale = E ** -0.5
    mem_rows = pl.ds(seg, M)

    def segment(s):
        hbuf[pl.ds(0, seg), :] = bx[s].astype(F32)
        qi = jax.lax.broadcasted_iota(jnp.int32, (L, L), 0)
        ki = jax.lax.broadcasted_iota(jnp.int32, (L, L), 1)
        mask = (qi >= seg) | (ki >= seg) | (qi >= ki)
        queries, keys, values, probs, ctx = {}, {}, {}, {}, {}

        n = seg - 16
        first, second = pl.ds(0, KH), pl.ds(KH, KH)
        plain, upper, top, bottom = pl.ds(0, n), pl.ds(0, n + 8), pl.ds(n, 8), pl.ds(n + 8, 8)
        total = hbuf[pl.ds(0, seg), first] + hbuf[pl.ds(0, seg), second]
        hsum[plain, :] = total[:n]
        hsum[top, :] = total[n:n + 8] - total[n + 8:]
        hsum[bottom, :] = hbuf[bottom, first] - hbuf[top, first]

        def weights(h, m):
            g, i = divmod(h, GROUP)
            ref = ((w_qk0.at[0], w_qk0.at[1], w_v0), (w_q1, w_k1, w_v1))[g][m]
            return pltpu.bitcast(ref[i], BF16)

        def ahead(h, m, i):
            g, j = divmod(h, GROUP)
            rows = pl.ds(pl.multiple_of(8 * s, 8), 8)
            if m == 2:
                v = (pre_v0, pre_v1)[g][j + i, rows, :]
            elif g == 0:
                v = pre_qk0[2 * j + i, rows, :]
            else:
                v = late(j)[late_rows(j, i, 8 * s, 8), :]
            return pltpu.bitcast(v, F32)

        def left(h, m):
            w = weights(h, m)
            return [_dot(jnp.concatenate([hbuf[upper, cols], hbuf[mem_rows, cols]], axis=0), v)
                    for cols, v in ((first, w[:KH]), (second, w[KH:]))]

        def right(h, m):
            w = weights(h, m)
            x = jnp.concatenate(
                [hbuf[plain, first], hsum[bottom, :], hbuf[mem_rows, first]], axis=0)
            y = jnp.concatenate([hsum[upper, :], hsum[mem_rows, :]], axis=0)
            return _dot(x, w[:KH]), _dot(y, w[KH:])

        def combine(h, m, l, r):
            c1, c2 = l[0] + l[1], r[0] + r[1]
            p1, p7, p3 = l[0][n:n + 8], r[0][n:n + 8], r[1][n:n + 8]
            u = p1 + ahead(h, m, 0)
            return (jnp.concatenate([c1[:n + 8], p1 + p7 + ahead(h, m, 1), c1[n + 8:]], axis=0),
                    jnp.concatenate([c2[:n], u + p3, u + p7, c2[n + 8:]], axis=0))

        def scores(h):
            sc = jnp.where(mask, _dot_nt(queries.pop(h), keys.pop(h)) * scale, -1000000000.0)
            e = jnp.exp(sc - jnp.max(sc, axis=-1, keepdims=True))
            probs[h] = e, jnp.sum(e, axis=-1, keepdims=True)

        def mix(h):
            e, norm = probs.pop(h)
            o = _dot(e, values.pop(h)) * (1.0 / norm)
            ctx[h] = jnp.concatenate([o[seg:], o[:seg]], axis=0)

        def output(h):
            rows = pl.ds(h * (E // 2), E // 2)
            w = jnp.concatenate([wo[j, rows, :] for j in range(RD)], axis=1)
            return _dot(ctx.pop(h), pltpu.bitcast(w, BF16))

        lag_scores, lag_mix, lag_output = 2, 6, 8
        acc = None
        for t in range(H + lag_output):
            if 0 <= t - lag_scores < H:
                scores(t - lag_scores)
            if t < H:
                q_parts = left(t, 0)
            if 0 <= t - lag_mix < H:
                mix(t - lag_mix)
            if t < H:
                queries[t], keys[t] = combine(t, 0, q_parts, right(t, 1))
                if t % 2 == 0:
                    v_parts = left(t, 2)
                else:
                    values[t - 1], values[t] = combine(t - 1, 2, v_parts, right(t, 2))
            if 0 <= t - lag_output < H:
                y = output(t - lag_output)
                acc = y if acc is None else acc + y
        hbuf[mem_rows, :] = acc[:M]
        hsum[mem_rows, :] = acc[:M, :KH] + acc[:M, KH:]
        yb[pl.ds(pl.multiple_of(s * seg, seg), seg), :] = acc[M:].astype(BF16)

    def yb_copy(i):
        rows = pl.ds(pl.multiple_of(i * (UNROLL * seg), UNROLL * seg), UNROLL * seg)
        return pltpu.make_async_copy(yb.at[rows], out_hbm.at[rows, pl.ds(D, D)], yb_sem)

    wait(cp_bx0)
    wait(cp_wo)
    hbuf[mem_rows, :] = mem0[...].astype(F32)
    hsum[mem_rows, :] = hbuf[mem_rows, pl.ds(0, KH)] + hbuf[mem_rows, pl.ds(KH, KH)]
    start(cp_bx1)
    start(cp_ya)

    def segments(i, carry):
        pl.when(i == 1)(functools.partial(wait, cp_bx1))

        @pl.when(i > 0)
        def _():
            yb_copy(i - 1).start()

        for u in range(UNROLL):
            segment(UNROLL * i + u)
        return carry

    jax.lax.fori_loop(0, n_seg // UNROLL, segments, 0)
    yb_copy(n_seg // UNROLL - 1).start()
    wait(cp_ya)
    pltpu.make_async_copy(yb, out_hbm.at[:, pl.ds(D, D)], yb_sem).wait()


@functools.partial(jax.jit, static_argnames=("B_seg_len",))
def pallas_concat_heads__spectral_gfnet__memory_aug_recurrent_mem_tr__prompt_kernel(
    A_x: jax.Array,
    A_w_r: jax.Array,
    A_w_i: jax.Array,
    B_x: jax.Array,
    B_mem0: jax.Array,
    B_Wq: jax.Array,
    B_Wk: jax.Array,
    B_Wv: jax.Array,
    B_Wo: jax.Array,
    B_seg_len: int,
):
    assert A_x.shape == (1, S, D) and B_x.shape == (1, S, D) and B_mem0.shape == (1, M, D)
    assert B_Wq.shape == (D, H, E) and B_Wo.shape == (H, E, D)
    seg = int(B_seg_len)
    n_seg = S // seg
    assert n_seg * seg == S and 8 * n_seg == D // 2
    mats, tw = _tables()
    vmem = pltpu.VMEM
    out = pl.pallas_call(
        functools.partial(_kernel, seg=seg, n_seg=n_seg),
        out_shape=jax.ShapeDtypeStruct((S, 2 * D), BF16),
        in_specs=[pl.BlockSpec(memory_space=pl.ANY)] * 11,
        out_specs=pl.BlockSpec(memory_space=pl.ANY),
        scratch_shapes=[
            vmem((RS + RD, RD * LANES, LANES), U32),
            vmem((RS, KH + 1, LANES), BF16),
            vmem((RS, KH + 1, LANES), BF16),
            vmem((mats.shape[0] // 2, LANES), U32),
            vmem(tw.shape, F32),
            vmem((RS, 3, LANES, LANES), F32),
            vmem((2, RS, KROWS, LANES), F32),
            vmem((6, D, GROUP // 2, LANES), U32),
            vmem((GROUP, D // 2, LANES), U32),
            vmem((2, GROUP, D // 2, LANES), U32),
            vmem((4 * GROUP, D // 2, LANES), U32),
            vmem((2 * GROUP, D // 2, LANES), U32),
            vmem((RD, H * E // 2, LANES), U32),
            vmem((n_seg, seg, D), BF16),
            vmem((M, D), BF16),
            vmem((M + seg, D), F32),
            vmem((M + seg, KH), F32),
            vmem((S, D), BF16),
            vmem((n_seg, 16, D), BF16),
            vmem((3, 4 * n_seg, KH), U32),
            vmem((GROUP, 8 * n_seg, LANES), U32),
            pltpu.SMEM((32,), jnp.int32),
            pltpu.SemaphoreType.DMA((26,)),
        ],
        compiler_params=pltpu.CompilerParams(vmem_limit_bytes=120 * 1024 * 1024),
        name="gfnet_rmt",
    )(A_x.reshape(S, D), A_w_r.T, A_w_i.T, B_x.reshape(n_seg, seg, D), B_mem0.reshape(M, D),
      B_Wq, B_Wk, B_Wv, B_Wo.reshape(H * E, D), mats, tw)
    return out.reshape(1, S, 2 * D)
```

```python
import functools

import jax
import jax.numpy as jnp
import numpy as np
from jax.experimental import pallas as pl
from jax.experimental.pallas import tpu as pltpu

F32 = jnp.float32
BF16 = jnp.bfloat16
U32 = jnp.uint32

S = 2048
D = 1024
H = 32
E = 128
M = 8
LANES = 128
RS = S // LANES
RD = D // LANES
KH = D // 2
KROWS = KH + 8
K_CLASSES = (0, 4, 1, 7, 2, 6, 5, 3)
_ROOT_NORM = 2.0 ** -10
TW_ROW = 2 * LANES
NYQ_ROW = TW_ROW + 2 * RS
CLASS_SIGN = (-1.0, 1.0)
KT = D // LANES
GROUP = H // 2
PIECES = ((2, 0), (0, 0), (1, 0), (2, 1), (0, 1), (1, 1))
UNROLL = 4


@functools.lru_cache(maxsize=None)
def _tables():
    bf16 = jnp.dtype(BF16)
    h = np.sqrt(0.5)
    butterfly = np.array([
        [1, 1, 1, 1, 1, 1, 1, 1],
        [1, -1, 1, -1, 1, -1, 1, -1],
        [1, h, 0, -h, -1, -h, 0, h],
        [0, h, 1, h, 0, -h, -1, -h],
        [1, 0, -1, 0, 1, 0, -1, 0],
        [0, 1, 0, -1, 0, 1, 0, -1],
        [1, -h, 0, h, -1, h, 0, -h],
        [0, -h, 1, -h, 0, h, -1, h],
    ], dtype=np.float64)
    norm = (butterfly ** 2).sum(axis=1)
    d = np.arange(D)
    half = LANES // 2
    mats = []
    for g in range(4):
        k = np.concatenate([K_CLASSES[2 * g + i] + 8 * np.arange(KH // 8) for i in range(2)])
        ang = 2.0 * np.pi * ((k[:, None] * d[None, :]) % D) / D
        rows = np.concatenate([np.cos(ang), -np.sin(ang)]).reshape(2 * LANES, RD, LANES)
        proj = np.einsum("rjd,cj->rcd", rows, butterfly) / norm[None, :, None]
        p, q = proj[:LANES, 2 * g], proj[:LANES, 2 * g + 1]
        r, t = proj[LANES:, 2 * g], proj[LANES:, 2 * g + 1]
        if g == 0:
            mats += [np.concatenate([p[:half], r[:half]]), np.concatenate([q[half:], t[half:]])]
        else:
            sign = np.repeat(CLASS_SIGN, half)[:, None]
            assert np.allclose(t, sign * p) and np.allclose(q, -sign * r)
            mats += [p, r - sign * p, p + sign * r]
    mats = np.concatenate(mats) * _ROOT_NORM
    nyq = np.tile(1.0 - 2.0 * (np.arange(LANES) % 2), (8, 1)) * _ROOT_NORM
    b = np.arange(LANES)
    ang = 2.0 * np.pi * ((b[:, None] * b[None, :]) % LANES) / LANES
    twang = 2.0 * np.pi * (np.arange(RS)[:, None] * b[None, :]) / S
    tw = np.concatenate([np.cos(ang), -np.sin(ang), np.cos(twang), -np.sin(twang), nyq])
    return mats.astype(bf16), tw.astype(np.float32)


def _lo(v):
    return pltpu.bitcast(v << 16, F32)


def _hi(v):
    return pltpu.bitcast(v & np.uint32(0xFFFF0000), F32)


def _pack(lo, hi):
    lo, hi = (pltpu.bitcast(v.astype(BF16).astype(F32), U32) for v in (lo, hi))
    return (lo >> 16) | hi


def _dot(a, b):
    return jnp.dot(a, b, preferred_element_type=F32)


def _dot_nt(a, b):
    return jax.lax.dot_general(a, b, (((1,), (1,)), ((), ())), preferred_element_type=F32)


_H8 = float(np.sqrt(0.5))


def _radix8_fwd(x):
    s04, d04 = x[0] + x[4], x[0] - x[4]
    s26, d26 = x[2] + x[6], x[2] - x[6]
    s15, d15 = x[1] + x[5], x[1] - x[5]
    s37, d37 = x[3] + x[7], x[3] - x[7]
    e0, e1 = s04 + s26, s15 + s37
    p, q = (d15 - d37) * _H8, (d15 + d37) * _H8
    return [e0 + e1, e0 - e1, d04 + p, d26 + q, s04 - s26, s15 - s37, d04 - p, d26 - q]


def _radix8_adj(p):
    e0, e1 = p[0] + p[1], p[0] - p[1]
    s04, s26 = e0 + p[4], e0 - p[4]
    s15, s37 = e1 + p[5], e1 - p[5]
    d04, d26 = p[2] + p[6], p[3] + p[7]
    m, n = (p[2] - p[6]) * _H8, (p[3] - p[7]) * _H8
    d15, d37 = m + n, n - m
    return [s04 + d04, s15 + d15, s26 + d26, s37 + d37,
            s04 - d04, s15 - d15, s26 - d26, s37 - d37]


def _cmul(a, b):
    return a[0] * b[0] - a[1] * b[1], a[0] * b[1] + a[1] * b[0]


def _dft4(z):
    ar, ai = z[0][0] + z[2][0], z[0][1] + z[2][1]
    br, bi = z[0][0] - z[2][0], z[0][1] - z[2][1]
    cr, ci = z[1][0] + z[3][0], z[1][1] + z[3][1]
    dr, di = z[1][0] - z[3][0], z[1][1] - z[3][1]
    return [(ar + cr, ai + ci), (br + di, bi - dr), (ar - cr, ai - ci), (br - di, bi + dr)]


def _rot16(z, n):
    re, im = z
    if n == 0:
        return z
    if n == 4:
        return im, -re
    if n == 2:
        return (re + im) * _H8, (im - re) * _H8
    if n == 6:
        return (im - re) * _H8, (re + im) * (-_H8)
    c, s = float(np.cos(np.pi * n / 8)), float(np.sin(np.pi * n / 8))
    return re * c + im * s, im * c - re * s


def _kernel(ax_hbm, wr_hbm, wi_hbm, bx_hbm, mem_hbm, wq_hbm, wk_hbm, wv_hbm, wo_hbm,
            mats_hbm, tw_hbm, out_hbm,
            ua, wr, wi, mats, tw, ftw, tbuf,
            raw, w_v0, w_qk0, pool_a, pool_b, wo,
            bx, mem0, hbuf, hsum, yb, tokens, xs, pre_v0, zeros, sems, *, seg, n_seg):
    sem_ids = iter(range(sems.shape[0]))
    w_v1, w_q1 = pool_a.at[pl.ds(0, GROUP)], pool_a.at[pl.ds(GROUP, GROUP)]
    pre_qk0 = pool_a.at[pl.ds(2 * GROUP, 2 * GROUP)]
    w_k1, pre_v1 = pool_b.at[pl.ds(0, GROUP)], pool_b.at[pl.ds(GROUP, GROUP)]

    def copies(pairs):
        sem = sems.at[next(sem_ids)]
        return [pltpu.make_async_copy(src, dst, sem) for src, dst in pairs]

    def start(group, **kwargs):
        for c in group:
            c.start(**kwargs)

    def wait(group):
        for c in group:
            c.wait()

    def col(j):
        return pl.ds(j * LANES, LANES)

    def pipelined(items, first, second, lag):
        pending = []
        for item in items:
            pending.append((item, first(item)))
            if len(pending) > lag:
                second(*pending.pop(0))
        for p in pending:
            second(*p)

    def u_load(a, i, first=0, n=LANES):
        return pltpu.bitcast(ua[a, pl.ds(i * LANES + first, n), :], F32)

    def u_store(a, i, value, first=0):
        ua[a, pl.ds(i * LANES + first, value.shape[0]), :] = pltpu.bitcast(value, U32)

    def piece(p):
        m, g = PIECES[p]
        src = (wq_hbm, wk_hbm, wv_hbm)[m].bitcast(U32)
        return src.at[:, pl.ds(GROUP // 2 * g, GROUP // 2), :], raw.at[p]

    quarter = S // 8
    cp_tables = copies([(tw_hbm, tw), (mats_hbm.bitcast(U32), mats)])
    cp_ax = [copies([(ax_hbm.bitcast(U32).at[pl.ds(q * quarter, quarter), col(j)],
                      ua.at[RS + j, pl.ds(q * quarter, quarter)]) for j in range(RD)])
             for q in range(4)]
    cp_piece = [copies([piece(p)]) for p in range(6)]
    cp_tokens = copies([(bx_hbm.at[:, pl.ds(seg - 16, 16), :], tokens)])
    cp_w = copies([(src.at[:, col(f)], dst.at[f])
                   for src, dst in ((wr_hbm, wr), (wi_hbm, wi)) for f in range(RS)])
    cp_bx0 = copies([(bx_hbm.at[pl.ds(0, UNROLL)], bx.at[pl.ds(0, UNROLL)]), (mem_hbm, mem0)])
    cp_bx1 = copies([(bx_hbm.at[pl.ds(UNROLL, n_seg - UNROLL)],
                      bx.at[pl.ds(UNROLL, n_seg - UNROLL)])])
    cp_wo = copies([(wo_hbm.bitcast(U32).at[:, col(j)], wo.at[j]) for j in range(RD)])
    cp_ya = copies([(ua.at[RS + j], out_hbm.bitcast(U32).at[:, col(j)]) for j in range(RD)])
    yb_sem = sems.at[next(sem_ids)]

    for group in (cp_tables, *cp_ax, cp_piece[0], cp_tokens):
        start(group)
    for k in range(zeros.shape[0]):
        zeros[k] = 0

    def words(p, kt, hp):
        src = raw.at[p].reshape(D * GROUP // 2, LANES)
        return src[pl.ds(kt * (GROUP // 2 * LANES) + hp, LANES, stride=GROUP // 2), :]

    def put(dst, head, kt, v):
        rows = pl.ds(pl.multiple_of(kt * (LANES // 2), LANES // 2), LANES // 2)
        dst[head, rows, :] = pltpu.bitcast(v, U32)

    def repack(p, kt, dst, pairs=range(GROUP // 2)):
        for hp in pairs:
            v = words(p, kt, hp)
            for par in range(2):
                put(dst, 2 * hp + par, kt, (v >> (16 * par)).astype(jnp.uint16))

    def repack_right(p, j, pairs, dst, is_right):
        for hp in pairs:
            v = [words(p, j, hp), words(p, j + KT // 2, hp)]
            for par, half in enumerate((_lo, _hi)):
                put(dst, 2 * hp + par, j + KT // 2, (v[1] >> (16 * par)).astype(jnp.uint16))
                if is_right[par]:
                    put(dst, 2 * hp + par, j, (half(v[0]) - half(v[1])).astype(BF16))
                else:
                    put(dst, 2 * hp + par, j, (v[0] >> (16 * par)).astype(jnp.uint16))

    def token_sums(j, carry):
        n = n_seg // 4
        v = tokens[pl.ds(j * n, n)].astype(F32)
        top, bottom = v[:, :8].reshape(8 * n, D), v[:, 8:].reshape(8 * n, D)
        rows = pl.ds(pl.multiple_of(j * (4 * n), 4 * n), 4 * n)
        s1 = bottom[:, :KH] + bottom[:, KH:]
        for i, x in enumerate((bottom[:, KH:], s1, s1 - top[:, :KH])):
            xs[i, rows, :] = pltpu.bitcast(x.astype(BF16), U32)
        return carry

    def precompute(left, right, dst, at, beside=()):
        b11, b21, t3, b22 = (pltpu.bitcast(v, BF16).astype(F32) for v in (
            left[:KH // 2], left[KH // 2:], right[:KH // 2], right[KH // 2:]))
        t2 = b11 - t3
        beside = list(beside)
        for i, w in ((2, t2), (1, b22 - t2), (0, t2 - b21)):
            p = _dot(pltpu.bitcast(xs[i], BF16), w)
            if beside:
                beside.pop(0)()
            if i == 2:
                dst[at(0)] = dst[at(1)] = pltpu.bitcast(p, U32)
            elif i == 1:
                dst[at(0)] = pltpu.bitcast(pltpu.bitcast(dst[at(0)], F32) + p, U32)
            else:
                dst[at(1)] = pltpu.bitcast(pltpu.bitcast(dst[at(1)], F32) - p, U32)

    wait(cp_tables)

    def twiddled_dft(a, carry):
        dft = tw[pl.ds(0, LANES), :], tw[pl.ds(LANES, LANES), :]
        re, im = _cmul(dft, (tw[pl.ds(TW_ROW + a, 1), :], tw[pl.ds(TW_ROW + RS + a, 1), :]))
        ftw[a, 0], ftw[a, 1], ftw[a, 2] = re, im - re, im + re
        return carry

    jax.lax.fori_loop(0, RS, twiddled_dft, 0)
    for q in range(4):
        wait(cp_ax[q])

        def butterflies(ap, carry, q=q):
            blocks = range(q * LANES // 4, (q + 1) * LANES // 4, 8)
            x = [[ua[RS + j, pl.ds(ap + 8 * b, 8, stride=8), :] for j in range(RD)]
                 for b in blocks]
            for b, v in zip(blocks, x):
                for par, half in enumerate((_lo, _hi)):
                    for i, u in enumerate(_radix8_fwd([half(t) for t in v])):
                        u_store(2 * ap + par, i, u, b)
            return carry

        jax.lax.fori_loop(0, RS // 2, butterflies, 0)

    def table(g, i):
        first = 0 if g == 0 else 3 * g - 1
        return pltpu.bitcast(mats[pl.ds((first + i) * (LANES // 2), LANES // 2), :], BF16)

    def forward(ap):
        half = LANES // 2

        def feature_dft(item):
            a, g = item
            if g == 4:
                return _dot_nt(tw[pl.ds(NYQ_ROW, 8), :], u_load(a, 0))
            u0, u1 = u_load(a, 2 * g), u_load(a, 2 * g + 1)
            if g == 0:
                y0, y1 = _dot_nt(table(0, 0), u0), _dot_nt(table(0, 1), u1)
                return (jnp.concatenate([y0[:half], y1[:half]], axis=0),
                        jnp.concatenate([y0[half:], y1[half:]], axis=0))
            both = _dot_nt(table(g, 0), u0 + u1)
            im = _dot_nt(table(g, 1), u0)
            re = both - _dot_nt(table(g, 2), u1)
            return re, jnp.concatenate([im[:half] - both[:half], im[half:] + both[half:]], axis=0)

        def sequence_dft(item, y):
            a, g = item
            if g == 4:
                rows = pl.ds(KH, 8)
                both = _dot(y, ftw[a, 0])
                re, im = both, both + _dot(y, ftw[a, 1])
            else:
                rows = pl.ds(g * LANES, LANES)
                both = _dot(y[0] + y[1], ftw[a, 0])
                re, im = both - _dot(y[1], ftw[a, 2]), both + _dot(y[0], ftw[a, 1])
            tbuf[0, a, rows, :], tbuf[1, a, rows, :] = re, im

        pipelined([(2 * ap + par, g) for par in range(2) for g in range(5)],
                  feature_dft, sequence_dft, 2)

    def forward_first(ap, carry):
        forward(ap)
        return carry

    def forward_second(i, carry):
        repack_right(0, i, range(GROUP // 2), w_v0, (False, True))
        forward(RS // 4 + i)
        return carry

    jax.lax.fori_loop(0, RS // 4, forward_first, 0)
    wait(cp_piece[0])
    for group in (cp_w, *cp_piece[1:], cp_bx0):
        start(group)
    start(cp_wo, priority=1)
    jax.lax.fori_loop(0, RS // 4, forward_second, 0)
    wait(cp_tokens)
    jax.lax.fori_loop(0, 4, token_sums, 0)

    def load(slots, rows):
        return [(tbuf[0, a, rows, :], tbuf[1, a, rows, :]) for a in slots]

    def store(slots, rows, z):
        for a, v in zip(slots, z):
            tbuf[0, a, rows, :], tbuf[1, a, rows, :] = v

    def swap(z):
        return [(im, re) for re, im in z]

    def rotate(z, n):
        return [_rot16(v, n * k) for k, v in enumerate(z)]

    def apply(z, n, filt, which):
        return [_cmul(v, filt(n + 4 * k)) if k in which else v for k, v in enumerate(z)]

    def columns(n):
        return range(n, RS, 4)

    def lines(n):
        return range(4 * n, 4 * n + 4)

    passes = (
        (columns, lambda z, n, filt: rotate(_dft4(z), n), 8),
        (lines, lambda z, n, filt: apply(_dft4(z), n, filt, (0, 1, 2)), 2),
        (lines, lambda z, n, filt: rotate(_dft4(swap(apply(z, n, filt, (3,)))), n), 4),
        (columns, lambda z, n, filt: swap(_dft4(z)), 16),
    )

    def run_pass(index, row, filt, position):
        slots, step, size = passes[index]
        for first in range(0, 4, size):
            rows = pl.ds(pl.multiple_of(
                row + zeros[(4 * position + first) // size % zeros.shape[0]], 8), 8)
            group = range(first, min(first + size, 4))
            z = [load(slots(n), rows) for n in group]
            for n, v in zip(group, z):
                store(slots(n), rows, step(v, n, filt))

    def filter_rows(cls, mb, f):
        block = pl.ds(pl.multiple_of(32 * mb, 32), 32)
        half, src = (_lo, _hi)[cls % 2], pl.ds(cls // 2, 8, stride=4)
        re, im = (half(ref.at[:, pl.ds(0, KH), :].bitcast(U32).at[f, block][src, :])
                  for ref in (wr, wi))
        if cls == 0:
            row = jax.lax.broadcasted_iota(jnp.int32, (8, LANES), 0)
            weight = jnp.where(row + mb == 0, 0.5, 1.0)
            re, im = re * weight, im * weight
        return re, im

    def filter_nyquist(f):
        return tuple(jnp.broadcast_to(ref[f, pl.ds(KH, 1), :].astype(F32), (8, LANES))
                     for ref in (wr, wi))

    for index in range(4):
        if index == 1:
            wait(cp_w)

        def middle(i, carry, index=index):
            pair = 2 * index + i
            precompute(w_v0[2 * pair], w_v0[2 * pair + 1], pre_v0, lambda n: 2 * pair + n)
            for n in range(4):
                mb = 4 * i + n
                for cls in range(8):
                    run_pass(index, 64 * K_CLASSES.index(cls) + 8 * mb,
                             functools.partial(filter_rows, cls, mb), 8 * n + cls)
            return carry

        jax.lax.fori_loop(0, 2, middle, 0)
        run_pass(index, KH, filter_nyquist, 0)

    def inverse(ap):
        def sequence_idft(item):
            a, g, _ = item
            if g == 4:
                re, im = (jnp.concatenate([tbuf[i, a, pl.ds(KH, 8), :]] * (LANES // 8), axis=0)
                          for i in range(2))
                return _dot_nt(ftw[a, 0], re + im) + _dot_nt(ftw[a, 1], im)
            rows = pl.ds(g * LANES, LANES)
            re, im = tbuf[0, a, rows, :], tbuf[1, a, rows, :]
            both = _dot_nt(ftw[a, 0], re + im)
            return both + _dot_nt(ftw[a, 1], im), both - _dot_nt(ftw[a, 2], re)

        nyquist = {}
        low = jax.lax.broadcasted_iota(jnp.int32, (LANES, LANES), 1) < LANES // 2

        def feature_idft(item, v):
            a, g, par = item
            if g == 4:
                nyquist[par] = v * (0.5 * tw[pl.ds(NYQ_ROW, 1), :])
            elif g == 0:
                re, im = v
                v0 = jnp.where(low, re, pltpu.roll(im, LANES // 2, 1))
                v1 = jnp.where(low, pltpu.roll(re, LANES // 2, 1), im)
                u_store(a, 0, _dot(v0, table(0, 0)) + nyquist.pop(par))
                u_store(a, 1, _dot(v1, table(0, 1)))
            else:
                re, im = v
                both = _dot(jnp.where(low, re - im, re + im), table(g, 0))
                u_store(a, 2 * g, both + _dot(im, table(g, 1)))
                u_store(a, 2 * g + 1, both - _dot(re, table(g, 2)))

        pipelined([(2 * ap + par, g, par) for par in range(2) for g in (4, 0, 1, 2, 3)],
                  sequence_idft, feature_idft, 3)

    def inverse_first(i, carry):
        for kt in (2 * i, 2 * i + 1):
            repack(1, kt, w_qk0.at[0])
        inverse(i)
        return carry

    def inverse_second(i, carry):
        repack_right(2, i, range(GROUP // 2), w_qk0.at[1], (True, True))
        inverse(RS // 4 + i)
        return carry

    wait(cp_piece[1])
    jax.lax.fori_loop(0, RS // 4, inverse_first, 0)
    wait(cp_piece[2])
    jax.lax.fori_loop(0, RS // 4, inverse_second, 0)

    def adjoint(ap):
        for b in range(0, LANES, 8):
            y = [_radix8_adj([u_load(2 * ap + par, n, b, 8) for n in range(RD)])
                 for par in range(2)]
            for j in range(RD):
                ua[RS + j, pl.ds(ap + 8 * b, 8, stride=8), :] = _pack(y[0][j], y[1][j])

    def finish(ap, carry):
        def v_part(hp):
            return functools.partial(repack_right, 3, ap // 2, [4 * (ap % 2) + i for i in hp],
                                     w_v1, (False, True))

        def q_part(hp):
            return functools.partial(repack, 4, ap, w_q1, hp)

        work = ([v_part((0, 1)), v_part((2,)), v_part((3,))],
                [q_part((0, 1, 2)), q_part((3, 4, 5)), q_part((6, 7))])
        adjoint(ap)
        for n in range(2):
            h = 2 * ap + n
            precompute(w_qk0[0, h], w_qk0[1, h], pre_qk0, lambda i: 2 * h + i, work[n])
        return carry

    wait(cp_piece[3])
    wait(cp_piece[4])
    jax.lax.fori_loop(0, RS // 2, finish, 0)

    def last_piece(i, carry):
        for n in range(2):
            pair = 2 * i + n
            work = [functools.partial(repack_right, 5, i, [4 * n + j for j in hp], w_k1,
                                      (True, True)) for hp in ((0, 1), (2,), (3,))]
            precompute(w_v1[2 * pair], w_v1[2 * pair + 1], pre_v1, lambda j: 2 * pair + j, work)
        return carry

    wait(cp_piece[5])
    jax.lax.fori_loop(0, 4, last_piece, 0)

    def late(h):
        return raw.at[h // 8].reshape(D * GROUP // 2, LANES)

    def late_rows(h, i, first, n):
        return pl.ds(pl.multiple_of((2 * (h % 8) + i) * (8 * n_seg) + first, 8), n)

    def last_pairs(i, carry):
        for h in (2 * i, 2 * i + 1):
            precompute(w_q1[h], w_k1[h], late(h), lambda n: late_rows(h, n, 0, 8 * n_seg))
        return carry

    jax.lax.fori_loop(0, GROUP // 2, last_pairs, 0)

    L = M + seg
    scale = E ** -0.5
    mem_rows = pl.ds(seg, M)

    def segment(s):
        hbuf[pl.ds(0, seg), :] = bx[s].astype(F32)
        qi = jax.lax.broadcasted_iota(jnp.int32, (L, L), 0)
        ki = jax.lax.broadcasted_iota(jnp.int32, (L, L), 1)
        mask = (qi >= seg) | (ki >= seg) | (qi >= ki)
        queries, keys, values, probs, ctx = {}, {}, {}, {}, {}

        n = seg - 16
        first, second = pl.ds(0, KH), pl.ds(KH, KH)
        plain, upper, top, bottom = pl.ds(0, n), pl.ds(0, n + 8), pl.ds(n, 8), pl.ds(n + 8, 8)
        total = hbuf[pl.ds(0, seg), first] + hbuf[pl.ds(0, seg), second]
        hsum[plain, :] = total[:n]
        hsum[top, :] = total[n:n + 8] - total[n + 8:]
        hsum[bottom, :] = hbuf[bottom, first] - hbuf[top, first]

        def weights(h, m):
            g, i = divmod(h, GROUP)
            ref = ((w_qk0.at[0], w_qk0.at[1], w_v0), (w_q1, w_k1, w_v1))[g][m]
            return pltpu.bitcast(ref[i], BF16)

        def ahead(h, m, i):
            g, j = divmod(h, GROUP)
            rows = pl.ds(pl.multiple_of(8 * s, 8), 8)
            if m == 2:
                v = (pre_v0, pre_v1)[g][j + i, rows, :]
            elif g == 0:
                v = pre_qk0[2 * j + i, rows, :]
            else:
                v = late(j)[late_rows(j, i, 8 * s, 8), :]
            return pltpu.bitcast(v, F32)

        def left(h, m):
            w = weights(h, m)
            return [_dot(jnp.concatenate([hbuf[upper, cols], hbuf[mem_rows, cols]], axis=0), v)
                    for cols, v in ((first, w[:KH]), (second, w[KH:]))]

        def right(h, m):
            w = weights(h, m)
            x = jnp.concatenate(
                [hbuf[plain, first], hsum[bottom, :], hbuf[mem_rows, first]], axis=0)
            y = jnp.concatenate([hsum[upper, :], hsum[mem_rows, :]], axis=0)
            return _dot(x, w[:KH]), _dot(y, w[KH:])

        def combine(h, m, l, r):
            c1, c2 = l[0] + l[1], r[0] + r[1]
            p1, p7, p3 = l[0][n:n + 8], r[0][n:n + 8], r[1][n:n + 8]
            u = p1 + ahead(h, m, 0)
            return (jnp.concatenate([c1[:n + 8], p1 + p7 + ahead(h, m, 1), c1[n + 8:]], axis=0),
                    jnp.concatenate([c2[:n], u + p3, u + p7, c2[n + 8:]], axis=0))

        def scores(h):
            sc = jnp.where(mask, _dot_nt(queries.pop(h), keys.pop(h)) * scale, -1000000000.0)
            e = jnp.exp(sc - jnp.max(sc, axis=-1, keepdims=True))
            probs[h] = e, jnp.sum(e, axis=-1, keepdims=True)

        def mix(h):
            e, norm = probs.pop(h)
            o = _dot(e, values.pop(h)) * (1.0 / norm)
            ctx[h] = jnp.concatenate([o[seg:], o[:seg]], axis=0)

        def output(h):
            rows = pl.ds(h * (E // 2), E // 2)
            w = jnp.concatenate([wo[j, rows, :] for j in range(RD)], axis=1)
            return _dot(ctx.pop(h), pltpu.bitcast(w, BF16))

        lag_scores, lag_mix, lag_output = 2, 6, 8
        acc = None
        for t in range(H + lag_output):
            if 0 <= t - lag_scores < H:
                scores(t - lag_scores)
            if t < H:
                q_parts = left(t, 0)
            if 0 <= t - lag_mix < H:
                mix(t - lag_mix)
            if t < H:
                queries[t], keys[t] = combine(t, 0, q_parts, right(t, 1))
                if t % 2 == 0:
                    v_parts = left(t, 2)
                else:
                    values[t - 1], values[t] = combine(t - 1, 2, v_parts, right(t, 2))
            if 0 <= t - lag_output < H:
                y = output(t - lag_output)
                acc = y if acc is None else acc + y
        hbuf[mem_rows, :] = acc[:M]
        hsum[mem_rows, :] = acc[:M, :KH] + acc[:M, KH:]
        yb[pl.ds(pl.multiple_of(s * seg, seg), seg), :] = acc[M:].astype(BF16)

    def yb_copy(i):
        rows = pl.ds(pl.multiple_of(i * (UNROLL * seg), UNROLL * seg), UNROLL * seg)
        return pltpu.make_async_copy(yb.at[rows], out_hbm.at[rows, pl.ds(D, D)], yb_sem)

    wait(cp_bx0)
    wait(cp_wo)
    hbuf[mem_rows, :] = mem0[...].astype(F32)
    hsum[mem_rows, :] = hbuf[mem_rows, pl.ds(0, KH)] + hbuf[mem_rows, pl.ds(KH, KH)]
    start(cp_bx1)
    start(cp_ya)

    def segments(i, carry):
        pl.when(i == 1)(functools.partial(wait, cp_bx1))

        @pl.when(i > 0)
        def _():
            yb_copy(i - 1).start()

        for u in range(UNROLL):
            segment(UNROLL * i + u)
        return carry

    jax.lax.fori_loop(0, n_seg // UNROLL, segments, 0)
    yb_copy(n_seg // UNROLL - 1).start()
    wait(cp_ya)
    pltpu.make_async_copy(yb, out_hbm.at[:, pl.ds(D, D)], yb_sem).wait()


@functools.partial(jax.jit, static_argnames=("B_seg_len",))
def pallas_concat_heads__spectral_gfnet__memory_aug_recurrent_mem_tr__prompt_kernel(
    A_x: jax.Array,
    A_w_r: jax.Array,
    A_w_i: jax.Array,
    B_x: jax.Array,
    B_mem0: jax.Array,
    B_Wq: jax.Array,
    B_Wk: jax.Array,
    B_Wv: jax.Array,
    B_Wo: jax.Array,
    B_seg_len: int,
):
    assert A_x.shape == (1, S, D) and B_x.shape == (1, S, D) and B_mem0.shape == (1, M, D)
    assert B_Wq.shape == (D, H, E) and B_Wo.shape == (H, E, D)
    seg = int(B_seg_len)
    n_seg = S // seg
    assert n_seg * seg == S and 8 * n_seg == D // 2
    mats, tw = _tables()
    vmem = pltpu.VMEM
    out = pl.pallas_call(
        functools.partial(_kernel, seg=seg, n_seg=n_seg),
        out_shape=jax.ShapeDtypeStruct((S, 2 * D), BF16),
        in_specs=[pl.BlockSpec(memory_space=pl.ANY)] * 11,
        out_specs=pl.BlockSpec(memory_space=pl.ANY),
        scratch_shapes=[
            vmem((RS + RD, RD * LANES, LANES), U32),
            vmem((RS, KH + 1, LANES), BF16),
            vmem((RS, KH + 1, LANES), BF16),
            vmem((mats.shape[0] // 2, LANES), U32),
            vmem(tw.shape, F32),
            vmem((RS, 3, LANES, LANES), F32),
            vmem((2, RS, KROWS, LANES), F32),
            vmem((6, D, GROUP // 2, LANES), U32),
            vmem((GROUP, D // 2, LANES), U32),
            vmem((2, GROUP, D // 2, LANES), U32),
            vmem((4 * GROUP, D // 2, LANES), U32),
            vmem((2 * GROUP, D // 2, LANES), U32),
            vmem((RD, H * E // 2, LANES), U32),
            vmem((n_seg, seg, D), BF16),
            vmem((M, D), BF16),
            vmem((M + seg, D), F32),
            vmem((M + seg, KH), F32),
            vmem((S, D), BF16),
            vmem((n_seg, 16, D), BF16),
            vmem((3, 4 * n_seg, KH), U32),
            vmem((GROUP, 8 * n_seg, LANES), U32),
            pltpu.SMEM((32,), jnp.int32),
            pltpu.SemaphoreType.DMA((26,)),
        ],
        compiler_params=pltpu.CompilerParams(vmem_limit_bytes=120 * 1024 * 1024),
        name="gfnet_rmt",
    )(A_x.reshape(S, D), A_w_r.T, A_w_i.T, B_x.reshape(n_seg, seg, D), B_mem0.reshape(M, D),
      B_Wq, B_Wk, B_Wv, B_Wo.reshape(H * E, D), mats, tw)
    return out.reshape(1, S, 2 * D)
```

```python
import functools

import jax
import jax.numpy as jnp
import numpy as np
from jax.experimental import pallas as pl
from jax.experimental.pallas import tpu as pltpu

F32 = jnp.float32
BF16 = jnp.bfloat16
U32 = jnp.uint32

S = 2048
D = 1024
H = 32
E = 128
M = 8
LANES = 128
RS = S // LANES
RD = D // LANES
KH = D // 2
KROWS = KH + 8
K_CLASSES = (0, 4, 1, 7, 2, 6, 5, 3)
_ROOT_NORM = 2.0 ** -10
TW_ROW = 2 * LANES
NYQ_ROW = TW_ROW + 2 * RS
CLASS_SIGN = (-1.0, 1.0)
KT = D // LANES
GROUP = H // 2
PIECES = ((2, 0), (0, 0), (1, 0), (2, 1), (0, 1), (1, 1))
UNROLL = 4


@functools.lru_cache(maxsize=None)
def _tables():
    bf16 = jnp.dtype(BF16)
    h = np.sqrt(0.5)
    butterfly = np.array([
        [1, 1, 1, 1, 1, 1, 1, 1],
        [1, -1, 1, -1, 1, -1, 1, -1],
        [1, h, 0, -h, -1, -h, 0, h],
        [0, h, 1, h, 0, -h, -1, -h],
        [1, 0, -1, 0, 1, 0, -1, 0],
        [0, 1, 0, -1, 0, 1, 0, -1],
        [1, -h, 0, h, -1, h, 0, -h],
        [0, -h, 1, -h, 0, h, -1, h],
    ], dtype=np.float64)
    norm = (butterfly ** 2).sum(axis=1)
    d = np.arange(D)
    half = LANES // 2
    mats = []
    for g in range(4):
        k = np.concatenate([K_CLASSES[2 * g + i] + 8 * np.arange(KH // 8) for i in range(2)])
        ang = 2.0 * np.pi * ((k[:, None] * d[None, :]) % D) / D
        rows = np.concatenate([np.cos(ang), -np.sin(ang)]).reshape(2 * LANES, RD, LANES)
        proj = np.einsum("rjd,cj->rcd", rows, butterfly) / norm[None, :, None]
        p, q = proj[:LANES, 2 * g], proj[:LANES, 2 * g + 1]
        r, t = proj[LANES:, 2 * g], proj[LANES:, 2 * g + 1]
        if g == 0:
            mats += [np.concatenate([p[:half], r[:half]]), np.concatenate([q[half:], t[half:]])]
        else:
            sign = np.repeat(CLASS_SIGN, half)[:, None]
            assert np.allclose(t, sign * p) and np.allclose(q, -sign * r)
            mats += [p, r - sign * p, p + sign * r]
    mats = np.concatenate(mats) * _ROOT_NORM
    nyq = np.tile(1.0 - 2.0 * (np.arange(LANES) % 2), (8, 1)) * _ROOT_NORM
    b = np.arange(LANES)
    ang = 2.0 * np.pi * ((b[:, None] * b[None, :]) % LANES) / LANES
    twang = 2.0 * np.pi * (np.arange(RS)[:, None] * b[None, :]) / S
    tw = np.concatenate([np.cos(ang), -np.sin(ang), np.cos(twang), -np.sin(twang), nyq])
    return mats.astype(bf16), tw.astype(np.float32)


def _lo(v):
    return pltpu.bitcast(v << 16, F32)


def _hi(v):
    return pltpu.bitcast(v & np.uint32(0xFFFF0000), F32)


def _pack(lo, hi):
    lo, hi = (pltpu.bitcast(v.astype(BF16).astype(F32), U32) for v in (lo, hi))
    return (lo >> 16) | hi


def _dot(a, b):
    return jnp.dot(a, b, preferred_element_type=F32)


def _dot_nt(a, b):
    return jax.lax.dot_general(a, b, (((1,), (1,)), ((), ())), preferred_element_type=F32)


_H8 = float(np.sqrt(0.5))


def _radix8_fwd(x):
    s04, d04 = x[0] + x[4], x[0] - x[4]
    s26, d26 = x[2] + x[6], x[2] - x[6]
    s15, d15 = x[1] + x[5], x[1] - x[5]
    s37, d37 = x[3] + x[7], x[3] - x[7]
    e0, e1 = s04 + s26, s15 + s37
    p, q = (d15 - d37) * _H8, (d15 + d37) * _H8
    return [e0 + e1, e0 - e1, d04 + p, d26 + q, s04 - s26, s15 - s37, d04 - p, d26 - q]


def _radix8_adj(p):
    e0, e1 = p[0] + p[1], p[0] - p[1]
    s04, s26 = e0 + p[4], e0 - p[4]
    s15, s37 = e1 + p[5], e1 - p[5]
    d04, d26 = p[2] + p[6], p[3] + p[7]
    m, n = (p[2] - p[6]) * _H8, (p[3] - p[7]) * _H8
    d15, d37 = m + n, n - m
    return [s04 + d04, s15 + d15, s26 + d26, s37 + d37,
            s04 - d04, s15 - d15, s26 - d26, s37 - d37]


def _cmul(a, b):
    return a[0] * b[0] - a[1] * b[1], a[0] * b[1] + a[1] * b[0]


def _dft4(z):
    ar, ai = z[0][0] + z[2][0], z[0][1] + z[2][1]
    br, bi = z[0][0] - z[2][0], z[0][1] - z[2][1]
    cr, ci = z[1][0] + z[3][0], z[1][1] + z[3][1]
    dr, di = z[1][0] - z[3][0], z[1][1] - z[3][1]
    return [(ar + cr, ai + ci), (br + di, bi - dr), (ar - cr, ai - ci), (br - di, bi + dr)]


def _rot16(z, n):
    re, im = z
    if n == 0:
        return z
    if n == 4:
        return im, -re
    if n == 2:
        return (re + im) * _H8, (im - re) * _H8
    if n == 6:
        return (im - re) * _H8, (re + im) * (-_H8)
    c, s = float(np.cos(np.pi * n / 8)), float(np.sin(np.pi * n / 8))
    return re * c + im * s, im * c - re * s


def _kernel(ax_hbm, wr_hbm, wi_hbm, bx_hbm, mem_hbm, wq_hbm, wk_hbm, wv_hbm, wo_hbm,
            mats_hbm, tw_hbm, out_hbm,
            ua, wr, wi, mats, tw, ftw, tbuf,
            raw, w_v0, w_qk0, pool_a, pool_b, wo,
            bx, mem0, hbuf, hsum, yb, tokens, xs, pre_v0, zeros, sems, *, seg, n_seg):
    sem_ids = iter(range(sems.shape[0]))
    w_v1, w_q1 = pool_a.at[pl.ds(0, GROUP)], pool_a.at[pl.ds(GROUP, GROUP)]
    pre_qk0 = pool_a.at[pl.ds(2 * GROUP, 2 * GROUP)]
    w_k1, pre_v1 = pool_b.at[pl.ds(0, GROUP)], pool_b.at[pl.ds(GROUP, GROUP)]

    def copies(pairs):
        sem = sems.at[next(sem_ids)]
        return [pltpu.make_async_copy(src, dst, sem) for src, dst in pairs]

    def start(group, **kwargs):
        for c in group:
            c.start(**kwargs)

    def wait(group):
        for c in group:
            c.wait()

    def col(j):
        return pl.ds(j * LANES, LANES)

    def pipelined(items, first, second, lag):
        pending = []
        for item in items:
            pending.append((item, first(item)))
            if len(pending) > lag:
                second(*pending.pop(0))
        for p in pending:
            second(*p)

    def u_load(a, i, first=0, n=LANES):
        return pltpu.bitcast(ua[a, pl.ds(i * LANES + first, n), :], F32)

    def u_store(a, i, value, first=0):
        ua[a, pl.ds(i * LANES + first, value.shape[0]), :] = pltpu.bitcast(value, U32)

    def piece(p):
        m, g = PIECES[p]
        src = (wq_hbm, wk_hbm, wv_hbm)[m].bitcast(U32)
        return src.at[:, pl.ds(GROUP // 2 * g, GROUP // 2), :], raw.at[p]

    quarter = S // 8
    cp_tables = copies([(tw_hbm, tw), (mats_hbm.bitcast(U32), mats)])
    cp_ax = [copies([(ax_hbm.bitcast(U32).at[pl.ds(q * quarter, quarter), col(j)],
                      ua.at[RS + j, pl.ds(q * quarter, quarter)]) for j in range(RD)])
             for q in range(4)]
    cp_piece = [copies([piece(p)]) for p in range(6)]
    cp_tokens = copies([(bx_hbm.at[:, pl.ds(seg - 16, 16), :], tokens)])
    cp_w = copies([(src.at[:, col(f)], dst.at[f])
                   for src, dst in ((wr_hbm, wr), (wi_hbm, wi)) for f in range(RS)])
    cp_bx0 = copies([(bx_hbm.at[pl.ds(0, UNROLL)], bx.at[pl.ds(0, UNROLL)]), (mem_hbm, mem0)])
    cp_bx1 = copies([(bx_hbm.at[pl.ds(UNROLL, n_seg - UNROLL)],
                      bx.at[pl.ds(UNROLL, n_seg - UNROLL)])])
    cp_wo = copies([(wo_hbm.bitcast(U32).at[:, col(j)], wo.at[j]) for j in range(RD)])
    cp_ya = copies([(ua.at[RS + j], out_hbm.bitcast(U32).at[:, col(j)]) for j in range(RD)])
    yb_sem = sems.at[next(sem_ids)]

    for group in (cp_tables, *cp_ax, cp_piece[0], cp_tokens):
        start(group)
    for k in range(zeros.shape[0]):
        zeros[k] = 0

    def words(p, kt, hp):
        src = raw.at[p].reshape(D * GROUP // 2, LANES)
        return src[pl.ds(kt * (GROUP // 2 * LANES) + hp, LANES, stride=GROUP // 2), :]

    def put(dst, head, kt, v):
        rows = pl.ds(pl.multiple_of(kt * (LANES // 2), LANES // 2), LANES // 2)
        dst[head, rows, :] = pltpu.bitcast(v, U32)

    def repack(p, kt, dst, pairs=range(GROUP // 2)):
        for hp in pairs:
            v = words(p, kt, hp)
            for par in range(2):
                put(dst, 2 * hp + par, kt, (v >> (16 * par)).astype(jnp.uint16))

    def repack_right(p, j, pairs, dst, is_right):
        for hp in pairs:
            v = [words(p, j, hp), words(p, j + KT // 2, hp)]
            for par, half in enumerate((_lo, _hi)):
                put(dst, 2 * hp + par, j + KT // 2, (v[1] >> (16 * par)).astype(jnp.uint16))
                if is_right[par]:
                    put(dst, 2 * hp + par, j, (half(v[0]) - half(v[1])).astype(BF16))
                else:
                    put(dst, 2 * hp + par, j, (v[0] >> (16 * par)).astype(jnp.uint16))

    def token_sums(j, carry):
        n = n_seg // 4
        v = tokens[pl.ds(j * n, n)].astype(F32)
        top, bottom = v[:, :8].reshape(8 * n, D), v[:, 8:].reshape(8 * n, D)
        rows = pl.ds(pl.multiple_of(j * (4 * n), 4 * n), 4 * n)
        s1 = bottom[:, :KH] + bottom[:, KH:]
        for i, x in enumerate((bottom[:, KH:], s1, s1 - top[:, :KH])):
            xs[i, rows, :] = pltpu.bitcast(x.astype(BF16), U32)
        return carry

    def precompute(left, right, dst, at, beside=()):
        b11, b21, t3, b22 = (pltpu.bitcast(v, BF16).astype(F32) for v in (
            left[:KH // 2], left[KH // 2:], right[:KH // 2], right[KH // 2:]))
        t2 = b11 - t3
        beside = list(beside)
        for i, w in ((2, t2), (1, b22 - t2), (0, t2 - b21)):
            p = _dot(pltpu.bitcast(xs[i], BF16), w)
            if beside:
                beside.pop(0)()
            if i == 2:
                dst[at(0)] = dst[at(1)] = pltpu.bitcast(p, U32)
            elif i == 1:
                dst[at(0)] = pltpu.bitcast(pltpu.bitcast(dst[at(0)], F32) + p, U32)
            else:
                dst[at(1)] = pltpu.bitcast(pltpu.bitcast(dst[at(1)], F32) - p, U32)

    wait(cp_tables)

    def twiddled_dft(a, carry):
        dft = tw[pl.ds(0, LANES), :], tw[pl.ds(LANES, LANES), :]
        re, im = _cmul(dft, (tw[pl.ds(TW_ROW + a, 1), :], tw[pl.ds(TW_ROW + RS + a, 1), :]))
        ftw[a, 0], ftw[a, 1], ftw[a, 2] = re, im - re, im + re
        return carry

    jax.lax.fori_loop(0, RS, twiddled_dft, 0)
    for q in range(4):
        wait(cp_ax[q])

        def butterflies(ap, carry, q=q):
            blocks = range(q * LANES // 4, (q + 1) * LANES // 4, 8)
            x = [[ua[RS + j, pl.ds(ap + 8 * b, 8, stride=8), :] for j in range(RD)]
                 for b in blocks]
            for b, v in zip(blocks, x):
                for par, half in enumerate((_lo, _hi)):
                    for i, u in enumerate(_radix8_fwd([half(t) for t in v])):
                        u_store(2 * ap + par, i, u, b)
            return carry

        jax.lax.fori_loop(0, RS // 2, butterflies, 0)

    def table(g, i):
        first = 0 if g == 0 else 3 * g - 1
        return pltpu.bitcast(mats[pl.ds((first + i) * (LANES // 2), LANES // 2), :], BF16)

    def forward(ap):
        half = LANES // 2

        def feature_dft(item):
            a, g = item
            if g == 4:
                return _dot_nt(tw[pl.ds(NYQ_ROW, 8), :], u_load(a, 0))
            u0, u1 = u_load(a, 2 * g), u_load(a, 2 * g + 1)
            if g == 0:
                y0, y1 = _dot_nt(table(0, 0), u0), _dot_nt(table(0, 1), u1)
                return (jnp.concatenate([y0[:half], y1[:half]], axis=0),
                        jnp.concatenate([y0[half:], y1[half:]], axis=0))
            both = _dot_nt(table(g, 0), u0 + u1)
            im = _dot_nt(table(g, 1), u0)
            re = both - _dot_nt(table(g, 2), u1)
            return re, jnp.concatenate([im[:half] - both[:half], im[half:] + both[half:]], axis=0)

        def sequence_dft(item, y):
            a, g = item
            if g == 4:
                rows = pl.ds(KH, 8)
                both = _dot(y, ftw[a, 0])
                re, im = both, both + _dot(y, ftw[a, 1])
            else:
                rows = pl.ds(g * LANES, LANES)
                both = _dot(y[0] + y[1], ftw[a, 0])
                re, im = both - _dot(y[1], ftw[a, 2]), both + _dot(y[0], ftw[a, 1])
            tbuf[0, a, rows, :], tbuf[1, a, rows, :] = re, im

        pipelined([(2 * ap + par, g) for par in range(2) for g in range(5)],
                  feature_dft, sequence_dft, 2)

    def forward_first(ap, carry):
        forward(ap)
        return carry

    def forward_second(i, carry):
        repack_right(0, i, range(GROUP // 2), w_v0, (False, True))
        forward(RS // 4 + i)
        return carry

    jax.lax.fori_loop(0, RS // 4, forward_first, 0)
    wait(cp_piece[0])
    for group in (cp_w, *cp_piece[1:], cp_bx0):
        start(group)
    start(cp_wo, priority=1)
    jax.lax.fori_loop(0, RS // 4, forward_second, 0)
    wait(cp_tokens)
    jax.lax.fori_loop(0, 4, token_sums, 0)

    def load(slots, rows):
        return [(tbuf[0, a, rows, :], tbuf[1, a, rows, :]) for a in slots]

    def store(slots, rows, z):
        for a, v in zip(slots, z):
            tbuf[0, a, rows, :], tbuf[1, a, rows, :] = v

    def swap(z):
        return [(im, re) for re, im in z]

    def rotate(z, n):
        return [_rot16(v, n * k) for k, v in enumerate(z)]

    def apply(z, n, filt, which):
        return [_cmul(v, filt(n + 4 * k)) if k in which else v for k, v in enumerate(z)]

    def columns(n):
        return range(n, RS, 4)

    def lines(n):
        return range(4 * n, 4 * n + 4)

    passes = (
        (columns, lambda z, n, filt: rotate(_dft4(z), n), 8),
        (lines, lambda z, n, filt: apply(_dft4(z), n, filt, (0, 1, 2)), 2),
        (lines, lambda z, n, filt: rotate(_dft4(swap(apply(z, n, filt, (3,)))), n), 4),
        (columns, lambda z, n, filt: swap(_dft4(z)), 16),
    )

    def run_pass(index, row, filt, position):
        slots, step, size = passes[index]
        for first in range(0, 4, size):
            rows = pl.ds(pl.multiple_of(
                row + zeros[(4 * position + first) // size % zeros.shape[0]], 8), 8)
            group = range(first, min(first + size, 4))
            z = [load(slots(n), rows) for n in group]
            for n, v in zip(group, z):
                store(slots(n), rows, step(v, n, filt))

    def filter_rows(cls, mb, f):
        block = pl.ds(pl.multiple_of(32 * mb, 32), 32)
        half, src = (_lo, _hi)[cls % 2], pl.ds(cls // 2, 8, stride=4)
        re, im = (half(ref.at[:, pl.ds(0, KH), :].bitcast(U32).at[f, block][src, :])
                  for ref in (wr, wi))
        if cls == 0:
            row = jax.lax.broadcasted_iota(jnp.int32, (8, LANES), 0)
            weight = jnp.where(row + mb == 0, 0.5, 1.0)
            re, im = re * weight, im * weight
        return re, im

    def filter_nyquist(f):
        return tuple(jnp.broadcast_to(ref[f, pl.ds(KH, 1), :].astype(F32), (8, LANES))
                     for ref in (wr, wi))

    for index in range(4):
        if index == 1:
            wait(cp_w)

        def middle(i, carry, index=index):
            pair = 2 * index + i
            precompute(w_v0[2 * pair], w_v0[2 * pair + 1], pre_v0, lambda n: 2 * pair + n)
            for n in range(4):
                mb = 4 * i + n
                for cls in range(8):
                    run_pass(index, 64 * K_CLASSES.index(cls) + 8 * mb,
                             functools.partial(filter_rows, cls, mb), 8 * n + cls)
            return carry

        jax.lax.fori_loop(0, 2, middle, 0)
        run_pass(index, KH, filter_nyquist, 0)

    def inverse(ap):
        def sequence_idft(item):
            a, g, _ = item
            if g == 4:
                re, im = (jnp.concatenate([tbuf[i, a, pl.ds(KH, 8), :]] * (LANES // 8), axis=0)
                          for i in range(2))
                return _dot_nt(ftw[a, 0], re + im) + _dot_nt(ftw[a, 1], im)
            rows = pl.ds(g * LANES, LANES)
            re, im = tbuf[0, a, rows, :], tbuf[1, a, rows, :]
            both = _dot_nt(ftw[a, 0], re + im)
            return both + _dot_nt(ftw[a, 1], im), both - _dot_nt(ftw[a, 2], re)

        nyquist = {}
        low = jax.lax.broadcasted_iota(jnp.int32, (LANES, LANES), 1) < LANES // 2

        def feature_idft(item, v):
            a, g, par = item
            if g == 4:
                nyquist[par] = v * (0.5 * tw[pl.ds(NYQ_ROW, 1), :])
            elif g == 0:
                re, im = v
                v0 = jnp.where(low, re, pltpu.roll(im, LANES // 2, 1))
                v1 = jnp.where(low, pltpu.roll(re, LANES // 2, 1), im)
                u_store(a, 0, _dot(v0, table(0, 0)) + nyquist.pop(par))
                u_store(a, 1, _dot(v1, table(0, 1)))
            else:
                re, im = v
                both = _dot(jnp.where(low, re - im, re + im), table(g, 0))
                u_store(a, 2 * g, both + _dot(im, table(g, 1)))
                u_store(a, 2 * g + 1, both - _dot(re, table(g, 2)))

        pipelined([(2 * ap + par, g, par) for par in range(2) for g in (4, 0, 1, 2, 3)],
                  sequence_idft, feature_idft, 3)

    def inverse_first(i, carry):
        for kt in (2 * i, 2 * i + 1):
            repack(1, kt, w_qk0.at[0])
        inverse(i)
        return carry

    def inverse_second(i, carry):
        repack_right(2, i, range(GROUP // 2), w_qk0.at[1], (True, True))
        inverse(RS // 4 + i)
        return carry

    wait(cp_piece[1])
    jax.lax.fori_loop(0, RS // 4, inverse_first, 0)
    wait(cp_piece[2])
    jax.lax.fori_loop(0, RS // 4, inverse_second, 0)

    def adjoint(ap):
        for b in range(0, LANES, 8):
            y = [_radix8_adj([u_load(2 * ap + par, n, b, 8) for n in range(RD)])
                 for par in range(2)]
            for j in range(RD):
                ua[RS + j, pl.ds(ap + 8 * b, 8, stride=8), :] = _pack(y[0][j], y[1][j])

    def middle_pieces(kt, carry):
        def v_part(hp):
            return functools.partial(repack_right, 3, kt // 2, [4 * (kt % 2) + i for i in hp],
                                     w_v1, (False, True))

        def q_part(hp):
            return functools.partial(repack, 4, kt, w_q1, hp)

        work = ([v_part((0, 1)), v_part((2,)), v_part((3,))],
                [q_part((0, 1, 2)), q_part((3, 4, 5)), q_part((6, 7))])
        for n in range(2):
            h = 2 * kt + n
            precompute(w_qk0[0, h], w_qk0[1, h], pre_qk0, lambda i: 2 * h + i, work[n])
        return carry

    wait(cp_piece[3])
    wait(cp_piece[4])
    jax.lax.fori_loop(0, KT, middle_pieces, 0)

    def last_piece(i, carry):
        for n in range(2):
            pair = 2 * i + n
            work = [functools.partial(repack_right, 5, i, [4 * n + j for j in hp], w_k1,
                                      (True, True)) for hp in ((0, 1), (2,), (3,))]
            precompute(w_v1[2 * pair], w_v1[2 * pair + 1], pre_v1, lambda j: 2 * pair + j, work)
        return carry

    wait(cp_piece[5])
    jax.lax.fori_loop(0, 4, last_piece, 0)

    def late(h):
        return raw.at[h // 8].reshape(D * GROUP // 2, LANES)

    def late_rows(h, i, first, n):
        return pl.ds(pl.multiple_of((2 * (h % 8) + i) * (8 * n_seg) + first, 8), n)

    def last_pairs(i, carry):
        adjoint(i)
        for h in (2 * i, 2 * i + 1):
            precompute(w_q1[h], w_k1[h], late(h), lambda n: late_rows(h, n, 0, 8 * n_seg))
        return carry

    jax.lax.fori_loop(0, GROUP // 2, last_pairs, 0)

    L = M + seg
    scale = E ** -0.5
    mem_rows = pl.ds(seg, M)

    def segment(s):
        hbuf[pl.ds(0, seg), :] = bx[s].astype(F32)
        qi = jax.lax.broadcasted_iota(jnp.int32, (L, L), 0)
        ki = jax.lax.broadcasted_iota(jnp.int32, (L, L), 1)
        mask = (qi >= seg) | (ki >= seg) | (qi >= ki)
        queries, keys, values, probs, ctx = {}, {}, {}, {}, {}

        n = seg - 16
        first, second = pl.ds(0, KH), pl.ds(KH, KH)
        plain, upper, top, bottom = pl.ds(0, n), pl.ds(0, n + 8), pl.ds(n, 8), pl.ds(n + 8, 8)
        total = hbuf[pl.ds(0, seg), first] + hbuf[pl.ds(0, seg), second]
        hsum[plain, :] = total[:n]
        hsum[top, :] = total[n:n + 8] - total[n + 8:]
        hsum[bottom, :] = hbuf[bottom, first] - hbuf[top, first]

        def weights(h, m):
            g, i = divmod(h, GROUP)
            ref = ((w_qk0.at[0], w_qk0.at[1], w_v0), (w_q1, w_k1, w_v1))[g][m]
            return pltpu.bitcast(ref[i], BF16)

        def ahead(h, m, i):
            g, j = divmod(h, GROUP)
            rows = pl.ds(pl.multiple_of(8 * s, 8), 8)
            if m == 2:
                v = (pre_v0, pre_v1)[g][j + i, rows, :]
            elif g == 0:
                v = pre_qk0[2 * j + i, rows, :]
            else:
                v = late(j)[late_rows(j, i, 8 * s, 8), :]
            return pltpu.bitcast(v, F32)

        def left(h, m):
            w = weights(h, m)
            return [_dot(jnp.concatenate([hbuf[upper, cols], hbuf[mem_rows, cols]], axis=0), v)
                    for cols, v in ((first, w[:KH]), (second, w[KH:]))]

        def right(h, m):
            w = weights(h, m)
            x = jnp.concatenate(
                [hbuf[plain, first], hsum[bottom, :], hbuf[mem_rows, first]], axis=0)
            y = jnp.concatenate([hsum[upper, :], hsum[mem_rows, :]], axis=0)
            return _dot(x, w[:KH]), _dot(y, w[KH:])

        def combine(h, m, l, r):
            c1, c2 = l[0] + l[1], r[0] + r[1]
            p1, p7, p3 = l[0][n:n + 8], r[0][n:n + 8], r[1][n:n + 8]
            u = p1 + ahead(h, m, 0)
            return (jnp.concatenate([c1[:n + 8], p1 + p7 + ahead(h, m, 1), c1[n + 8:]], axis=0),
                    jnp.concatenate([c2[:n], u + p3, u + p7, c2[n + 8:]], axis=0))

        def scores(h):
            sc = jnp.where(mask, _dot_nt(queries.pop(h), keys.pop(h)) * scale, -1000000000.0)
            e = jnp.exp(sc - jnp.max(sc, axis=-1, keepdims=True))
            probs[h] = e, jnp.sum(e, axis=-1, keepdims=True)

        def mix(h):
            e, norm = probs.pop(h)
            o = _dot(e, values.pop(h)) * (1.0 / norm)
            ctx[h] = jnp.concatenate([o[seg:], o[:seg]], axis=0)

        def output(h):
            rows = pl.ds(h * (E // 2), E // 2)
            w = jnp.concatenate([wo[j, rows, :] for j in range(RD)], axis=1)
            return _dot(ctx.pop(h), pltpu.bitcast(w, BF16))

        lag_scores, lag_mix, lag_output = 2, 6, 8
        acc = None
        for t in range(H + lag_output):
            if 0 <= t - lag_scores < H:
                scores(t - lag_scores)
            if t < H:
                q_parts = left(t, 0)
            if 0 <= t - lag_mix < H:
                mix(t - lag_mix)
            if t < H:
                queries[t], keys[t] = combine(t, 0, q_parts, right(t, 1))
                if t % 2 == 0:
                    v_parts = left(t, 2)
                else:
                    values[t - 1], values[t] = combine(t - 1, 2, v_parts, right(t, 2))
            if 0 <= t - lag_output < H:
                y = output(t - lag_output)
                acc = y if acc is None else acc + y
        hbuf[mem_rows, :] = acc[:M]
        hsum[mem_rows, :] = acc[:M, :KH] + acc[:M, KH:]
        yb[pl.ds(pl.multiple_of(s * seg, seg), seg), :] = acc[M:].astype(BF16)

    def yb_copy(i):
        rows = pl.ds(pl.multiple_of(i * (UNROLL * seg), UNROLL * seg), UNROLL * seg)
        return pltpu.make_async_copy(yb.at[rows], out_hbm.at[rows, pl.ds(D, D)], yb_sem)

    wait(cp_bx0)
    wait(cp_wo)
    hbuf[mem_rows, :] = mem0[...].astype(F32)
    hsum[mem_rows, :] = hbuf[mem_rows, pl.ds(0, KH)] + hbuf[mem_rows, pl.ds(KH, KH)]
    start(cp_bx1)
    start(cp_ya)

    def segments(i, carry):
        pl.when(i == 1)(functools.partial(wait, cp_bx1))

        @pl.when(i > 0)
        def _():
            yb_copy(i - 1).start()

        for u in range(UNROLL):
            segment(UNROLL * i + u)
        return carry

    jax.lax.fori_loop(0, n_seg // UNROLL, segments, 0)
    yb_copy(n_seg // UNROLL - 1).start()
    wait(cp_ya)
    pltpu.make_async_copy(yb, out_hbm.at[:, pl.ds(D, D)], yb_sem).wait()


@functools.partial(jax.jit, static_argnames=("B_seg_len",))
def pallas_concat_heads__spectral_gfnet__memory_aug_recurrent_mem_tr__prompt_kernel(
    A_x: jax.Array,
    A_w_r: jax.Array,
    A_w_i: jax.Array,
    B_x: jax.Array,
    B_mem0: jax.Array,
    B_Wq: jax.Array,
    B_Wk: jax.Array,
    B_Wv: jax.Array,
    B_Wo: jax.Array,
    B_seg_len: int,
):
    assert A_x.shape == (1, S, D) and B_x.shape == (1, S, D) and B_mem0.shape == (1, M, D)
    assert B_Wq.shape == (D, H, E) and B_Wo.shape == (H, E, D)
    seg = int(B_seg_len)
    n_seg = S // seg
    assert n_seg * seg == S and 8 * n_seg == D // 2
    mats, tw = _tables()
    vmem = pltpu.VMEM
    out = pl.pallas_call(
        functools.partial(_kernel, seg=seg, n_seg=n_seg),
        out_shape=jax.ShapeDtypeStruct((S, 2 * D), BF16),
        in_specs=[pl.BlockSpec(memory_space=pl.ANY)] * 11,
        out_specs=pl.BlockSpec(memory_space=pl.ANY),
        scratch_shapes=[
            vmem((RS + RD, RD * LANES, LANES), U32),
            vmem((RS, KH + 1, LANES), BF16),
            vmem((RS, KH + 1, LANES), BF16),
            vmem((mats.shape[0] // 2, LANES), U32),
            vmem(tw.shape, F32),
            vmem((RS, 3, LANES, LANES), F32),
            vmem((2, RS, KROWS, LANES), F32),
            vmem((6, D, GROUP // 2, LANES), U32),
            vmem((GROUP, D // 2, LANES), U32),
            vmem((2, GROUP, D // 2, LANES), U32),
            vmem((4 * GROUP, D // 2, LANES), U32),
            vmem((2 * GROUP, D // 2, LANES), U32),
            vmem((RD, H * E // 2, LANES), U32),
            vmem((n_seg, seg, D), BF16),
            vmem((M, D), BF16),
            vmem((M + seg, D), F32),
            vmem((M + seg, KH), F32),
            vmem((S, D), BF16),
            vmem((n_seg, 16, D), BF16),
            vmem((3, 4 * n_seg, KH), U32),
            vmem((GROUP, 8 * n_seg, LANES), U32),
            pltpu.SMEM((32,), jnp.int32),
            pltpu.SemaphoreType.DMA((26,)),
        ],
        compiler_params=pltpu.CompilerParams(vmem_limit_bytes=120 * 1024 * 1024),
        name="gfnet_rmt",
    )(A_x.reshape(S, D), A_w_r.T, A_w_i.T, B_x.reshape(n_seg, seg, D), B_mem0.reshape(M, D),
      B_Wq, B_Wk, B_Wv, B_Wo.reshape(H * E, D), mats, tw)
    return out.reshape(1, S, 2 * D)
```

```python
import functools

import jax
import jax.numpy as jnp
import numpy as np
from jax.experimental import pallas as pl
from jax.experimental.pallas import tpu as pltpu

F32 = jnp.float32
BF16 = jnp.bfloat16
U32 = jnp.uint32

S = 2048
D = 1024
H = 32
E = 128
M = 8
LANES = 128
RS = S // LANES
RD = D // LANES
KH = D // 2
KROWS = KH + 8
K_CLASSES = (0, 4, 1, 7, 2, 6, 5, 3)
_ROOT_NORM = 2.0 ** -10
TW_ROW = 2 * LANES
NYQ_ROW = TW_ROW + 2 * RS
CLASS_SIGN = (-1.0, 1.0)
KT = D // LANES
GROUP = H // 2
PIECES = ((2, 0), (0, 0), (1, 0), (2, 1), (0, 1), (1, 1))
UNROLL = 4


@functools.lru_cache(maxsize=None)
def _tables():
    bf16 = jnp.dtype(BF16)
    h = np.sqrt(0.5)
    butterfly = np.array([
        [1, 1, 1, 1, 1, 1, 1, 1],
        [1, -1, 1, -1, 1, -1, 1, -1],
        [1, h, 0, -h, -1, -h, 0, h],
        [0, h, 1, h, 0, -h, -1, -h],
        [1, 0, -1, 0, 1, 0, -1, 0],
        [0, 1, 0, -1, 0, 1, 0, -1],
        [1, -h, 0, h, -1, h, 0, -h],
        [0, -h, 1, -h, 0, h, -1, h],
    ], dtype=np.float64)
    norm = (butterfly ** 2).sum(axis=1)
    d = np.arange(D)
    half = LANES // 2
    mats = []
    for g in range(4):
        k = np.concatenate([K_CLASSES[2 * g + i] + 8 * np.arange(KH // 8) for i in range(2)])
        ang = 2.0 * np.pi * ((k[:, None] * d[None, :]) % D) / D
        rows = np.concatenate([np.cos(ang), -np.sin(ang)]).reshape(2 * LANES, RD, LANES)
        proj = np.einsum("rjd,cj->rcd", rows, butterfly) / norm[None, :, None]
        p, q = proj[:LANES, 2 * g], proj[:LANES, 2 * g + 1]
        r, t = proj[LANES:, 2 * g], proj[LANES:, 2 * g + 1]
        if g == 0:
            mats += [np.concatenate([p[:half], r[:half]]), np.concatenate([q[half:], t[half:]])]
        else:
            sign = np.repeat(CLASS_SIGN, half)[:, None]
            assert np.allclose(t, sign * p) and np.allclose(q, -sign * r)
            mats += [p, r - sign * p, p + sign * r]
    mats = np.concatenate(mats) * _ROOT_NORM
    nyq = np.tile(1.0 - 2.0 * (np.arange(LANES) % 2), (8, 1)) * _ROOT_NORM
    b = np.arange(LANES)
    ang = 2.0 * np.pi * ((b[:, None] * b[None, :]) % LANES) / LANES
    twang = 2.0 * np.pi * (np.arange(RS)[:, None] * b[None, :]) / S
    tw = np.concatenate([np.cos(ang), -np.sin(ang), np.cos(twang), -np.sin(twang), nyq])
    return mats.astype(bf16), tw.astype(np.float32)


def _lo(v):
    return pltpu.bitcast(v << 16, F32)


def _hi(v):
    return pltpu.bitcast(v & np.uint32(0xFFFF0000), F32)


def _pack(lo, hi):
    lo, hi = (pltpu.bitcast(v.astype(BF16).astype(F32), U32) for v in (lo, hi))
    return (lo >> 16) | hi


def _dot(a, b):
    return jnp.dot(a, b, preferred_element_type=F32)


def _dot_nt(a, b):
    return jax.lax.dot_general(a, b, (((1,), (1,)), ((), ())), preferred_element_type=F32)


_H8 = float(np.sqrt(0.5))


def _radix8_fwd(x):
    s04, d04 = x[0] + x[4], x[0] - x[4]
    s26, d26 = x[2] + x[6], x[2] - x[6]
    s15, d15 = x[1] + x[5], x[1] - x[5]
    s37, d37 = x[3] + x[7], x[3] - x[7]
    e0, e1 = s04 + s26, s15 + s37
    p, q = (d15 - d37) * _H8, (d15 + d37) * _H8
    return [e0 + e1, e0 - e1, d04 + p, d26 + q, s04 - s26, s15 - s37, d04 - p, d26 - q]


def _radix8_adj(p):
    e0, e1 = p[0] + p[1], p[0] - p[1]
    s04, s26 = e0 + p[4], e0 - p[4]
    s15, s37 = e1 + p[5], e1 - p[5]
    d04, d26 = p[2] + p[6], p[3] + p[7]
    m, n = (p[2] - p[6]) * _H8, (p[3] - p[7]) * _H8
    d15, d37 = m + n, n - m
    return [s04 + d04, s15 + d15, s26 + d26, s37 + d37,
            s04 - d04, s15 - d15, s26 - d26, s37 - d37]


def _cmul(a, b):
    return a[0] * b[0] - a[1] * b[1], a[0] * b[1] + a[1] * b[0]


def _dft4(z):
    ar, ai = z[0][0] + z[2][0], z[0][1] + z[2][1]
    br, bi = z[0][0] - z[2][0], z[0][1] - z[2][1]
    cr, ci = z[1][0] + z[3][0], z[1][1] + z[3][1]
    dr, di = z[1][0] - z[3][0], z[1][1] - z[3][1]
    return [(ar + cr, ai + ci), (br + di, bi - dr), (ar - cr, ai - ci), (br - di, bi + dr)]


def _rot16(z, n):
    re, im = z
    if n == 0:
        return z
    if n == 4:
        return im, -re
    if n == 2:
        return (re + im) * _H8, (im - re) * _H8
    if n == 6:
        return (im - re) * _H8, (re + im) * (-_H8)
    c, s = float(np.cos(np.pi * n / 8)), float(np.sin(np.pi * n / 8))
    return re * c + im * s, im * c - re * s


def _kernel(ax_hbm, wr_hbm, wi_hbm, bx_hbm, mem_hbm, wq_hbm, wk_hbm, wv_hbm, wo_hbm,
            mats_hbm, tw_hbm, out_hbm,
            ua, wr, wi, mats, tw, ftw, tbuf,
            raw, pool_a, pool_b, wo,
            bx, mem0, hbuf, hsum, yb, tokens, xs, pre_v0, zeros, sems, *, seg, n_seg):
    sem_ids = iter(range(sems.shape[0]))
    w_v0 = tbuf.at[2, :, pl.ds(0, D // 2)]
    w_q0, w_k0 = (ua.at[pl.ds(RS + RD, GROUP), pl.ds(i * (D // 2), D // 2)] for i in range(2))
    w_v1, pre_qk0 = pool_a.at[pl.ds(0, GROUP)], pool_a.at[pl.ds(GROUP, 2 * GROUP)]
    w_q1, w_k1, pre_v1 = (pool_b.at[pl.ds(i * GROUP, GROUP)] for i in range(3))

    def copies(pairs):
        sem = sems.at[next(sem_ids)]
        return [pltpu.make_async_copy(src, dst, sem) for src, dst in pairs]

    def start(group, **kwargs):
        for c in group:
            c.start(**kwargs)

    def wait(group):
        for c in group:
            c.wait()

    def col(j):
        return pl.ds(j * LANES, LANES)

    def pipelined(items, first, second, lag):
        pending = []
        for item in items:
            pending.append((item, first(item)))
            if len(pending) > lag:
                second(*pending.pop(0))
        for p in pending:
            second(*p)

    def u_load(a, i, first=0, n=LANES):
        return pltpu.bitcast(ua[a, pl.ds(i * LANES + first, n), :], F32)

    def u_store(a, i, value, first=0):
        ua[a, pl.ds(i * LANES + first, value.shape[0]), :] = pltpu.bitcast(value, U32)

    def t_load(a, rows):
        return tuple(pltpu.bitcast(tbuf[i, a, rows, :], F32) for i in range(2))

    def t_store(a, rows, z):
        for i in range(2):
            tbuf[i, a, rows, :] = pltpu.bitcast(z[i], U32)

    def piece(p):
        m, g = PIECES[p]
        src = (wq_hbm, wk_hbm, wv_hbm)[m].bitcast(U32)
        return src.at[:, pl.ds(GROUP // 2 * g, GROUP // 2), :], raw.at[p]

    quarter = S // 8
    cp_tables = copies([(tw_hbm, tw), (mats_hbm.bitcast(U32), mats)])
    cp_ax = [copies([(ax_hbm.bitcast(U32).at[pl.ds(q * quarter, quarter), col(j)],
                      ua.at[RS + j, pl.ds(q * quarter, quarter)]) for j in range(RD)])
             for q in range(4)]
    cp_piece = [copies([piece(p)]) for p in range(6)]
    cp_tokens = copies([(bx_hbm.at[:, pl.ds(seg - 16, 16), :], tokens)])
    cp_w = copies([(src.at[:, col(f)], dst.at[f])
                   for src, dst in ((wr_hbm, wr), (wi_hbm, wi)) for f in range(RS)])
    cp_bx0 = copies([(bx_hbm.at[pl.ds(0, UNROLL)], bx.at[pl.ds(0, UNROLL)]), (mem_hbm, mem0)])
    cp_bx1 = copies([(bx_hbm.at[pl.ds(UNROLL, n_seg - UNROLL)],
                      bx.at[pl.ds(UNROLL, n_seg - UNROLL)])])
    cp_wo = copies([(wo_hbm.bitcast(U32).at[:, col(j)], wo.at[j]) for j in range(RD)])
    cp_ya = copies([(ua.at[RS + j], out_hbm.bitcast(U32).at[:, col(j)]) for j in range(RD)])
    yb_sem = sems.at[next(sem_ids)]

    for group in (cp_tables, *cp_ax, cp_piece[0], cp_tokens):
        start(group)
    for k in range(zeros.shape[0]):
        zeros[k] = 0

    def words(p, kt, hp):
        src = raw.at[p].reshape(D * GROUP // 2, LANES)
        return src[pl.ds(kt * (GROUP // 2 * LANES) + hp, LANES, stride=GROUP // 2), :]

    def put(dst, head, kt, v):
        rows = pl.ds(pl.multiple_of(kt * (LANES // 2), LANES // 2), LANES // 2)
        dst[head, rows, :] = pltpu.bitcast(v, U32)

    def repack(p, kt, dst, pairs=range(GROUP // 2)):
        for hp in pairs:
            v = words(p, kt, hp)
            for par in range(2):
                put(dst, 2 * hp + par, kt, (v >> (16 * par)).astype(jnp.uint16))

    def repack_right(p, j, pairs, dst, is_right):
        for hp in pairs:
            v = [words(p, j, hp), words(p, j + KT // 2, hp)]
            for par, half in enumerate((_lo, _hi)):
                put(dst, 2 * hp + par, j + KT // 2, (v[1] >> (16 * par)).astype(jnp.uint16))
                if is_right[par]:
                    put(dst, 2 * hp + par, j, (half(v[0]) - half(v[1])).astype(BF16))
                else:
                    put(dst, 2 * hp + par, j, (v[0] >> (16 * par)).astype(jnp.uint16))

    def token_sums(j, carry):
        n = n_seg // 4
        v = tokens[pl.ds(j * n, n)].astype(F32)
        top, bottom = v[:, :8].reshape(8 * n, D), v[:, 8:].reshape(8 * n, D)
        rows = pl.ds(pl.multiple_of(j * (4 * n), 4 * n), 4 * n)
        s1 = bottom[:, :KH] + bottom[:, KH:]
        for i, x in enumerate((bottom[:, KH:], s1, s1 - top[:, :KH])):
            xs[i, rows, :] = pltpu.bitcast(x.astype(BF16), U32)
        return carry

    def precompute(left, right, dst, at, beside=()):
        b11, b21, t3, b22 = (pltpu.bitcast(v, BF16).astype(F32) for v in (
            left[:KH // 2], left[KH // 2:], right[:KH // 2], right[KH // 2:]))
        t2 = b11 - t3
        beside = list(beside)
        for i, w in ((2, t2), (1, b22 - t2), (0, t2 - b21)):
            p = _dot(pltpu.bitcast(xs[i], BF16), w)
            if beside:
                beside.pop(0)()
            if i == 2:
                dst[at(0)] = dst[at(1)] = pltpu.bitcast(p, U32)
            elif i == 1:
                dst[at(0)] = pltpu.bitcast(pltpu.bitcast(dst[at(0)], F32) + p, U32)
            else:
                dst[at(1)] = pltpu.bitcast(pltpu.bitcast(dst[at(1)], F32) - p, U32)

    wait(cp_tables)

    def twiddled_dft(a, carry):
        dft = tw[pl.ds(0, LANES), :], tw[pl.ds(LANES, LANES), :]
        re, im = _cmul(dft, (tw[pl.ds(TW_ROW + a, 1), :], tw[pl.ds(TW_ROW + RS + a, 1), :]))
        ftw[a, 0], ftw[a, 1], ftw[a, 2] = re, im - re, im + re
        return carry

    jax.lax.fori_loop(0, RS, twiddled_dft, 0)
    for q in range(4):
        wait(cp_ax[q])

        def butterflies(ap, carry, q=q):
            blocks = range(q * LANES // 4, (q + 1) * LANES // 4, 8)
            x = [[ua[RS + j, pl.ds(ap + 8 * b, 8, stride=8), :] for j in range(RD)]
                 for b in blocks]
            for b, v in zip(blocks, x):
                for par, half in enumerate((_lo, _hi)):
                    for i, u in enumerate(_radix8_fwd([half(t) for t in v])):
                        u_store(2 * ap + par, i, u, b)
            return carry

        jax.lax.fori_loop(0, RS // 2, butterflies, 0)

    def table(g, i):
        first = 0 if g == 0 else 3 * g - 1
        return pltpu.bitcast(mats[pl.ds((first + i) * (LANES // 2), LANES // 2), :], BF16)

    def forward(ap, beside=()):
        half = LANES // 2
        beside = list(beside)

        def feature_dft(item):
            a, g = item
            if g == 4:
                return _dot_nt(tw[pl.ds(NYQ_ROW, 8), :], u_load(a, 0))
            u0, u1 = u_load(a, 2 * g), u_load(a, 2 * g + 1)
            if g == 0:
                y0, y1 = _dot_nt(table(0, 0), u0), _dot_nt(table(0, 1), u1)
                return (jnp.concatenate([y0[:half], y1[:half]], axis=0),
                        jnp.concatenate([y0[half:], y1[half:]], axis=0))
            both = _dot_nt(table(g, 0), u0 + u1)
            im = _dot_nt(table(g, 1), u0)
            re = both - _dot_nt(table(g, 2), u1)
            return re, jnp.concatenate([im[:half] - both[:half], im[half:] + both[half:]], axis=0)

        def sequence_dft(item, y):
            a, g = item
            if g == 4:
                rows = pl.ds(KH, 8)
                both = _dot(y, ftw[a, 0])
                re, im = both, both + _dot(y, ftw[a, 1])
            else:
                rows = pl.ds(g * LANES, LANES)
                both = _dot(y[0] + y[1], ftw[a, 0])
                re, im = both - _dot(y[1], ftw[a, 2]), both + _dot(y[0], ftw[a, 1])
            if beside and g < 4:
                beside.pop(0)()
            t_store(a, rows, (re, im))

        pipelined([(2 * ap + par, g) for par in range(2) for g in range(5)],
                  feature_dft, sequence_dft, 2)

    def forward_first(ap, carry):
        forward(ap)
        return carry

    def forward_second(i, carry):
        forward(RS // 4 + i, [functools.partial(repack_right, 0, i, (hp,), w_v0, (False, True))
                              for hp in range(GROUP // 2)])
        return carry

    jax.lax.fori_loop(0, RS // 4, forward_first, 0)
    wait(cp_piece[0])
    for group in (cp_w, *cp_piece[1:], cp_bx0):
        start(group)
    start(cp_wo, priority=1)
    jax.lax.fori_loop(0, RS // 4, forward_second, 0)
    wait(cp_tokens)
    jax.lax.fori_loop(0, 4, token_sums, 0)

    def swap(z):
        return [(im, re) for re, im in z]

    def rotate(z, n):
        return [_rot16(v, n * k) for k, v in enumerate(z)]

    def apply(z, n, filt, which):
        return [_cmul(v, filt(n + 4 * k)) if k in which else v for k, v in enumerate(z)]

    def columns(n):
        return range(n, RS, 4)

    def lines(n):
        return range(4 * n, 4 * n + 4)

    passes = (
        (columns, lambda z, n, filt: rotate(_dft4(z), n), 8),
        (lines, lambda z, n, filt: apply(_dft4(z), n, filt, (0, 1, 2)), 2),
        (lines, lambda z, n, filt: rotate(_dft4(swap(apply(z, n, filt, (3,)))), n), 4),
        (columns, lambda z, n, filt: swap(_dft4(z)), 16),
    )

    def run_pass(index, row, filt, position):
        slots, step, size = passes[index]
        for first in range(0, 4, size):
            rows = pl.ds(pl.multiple_of(
                row + zeros[(4 * position + first) // size % zeros.shape[0]], 8), 8)
            group = range(first, min(first + size, 4))
            z = [[t_load(a, rows) for a in slots(n)] for n in group]
            for n, v in zip(group, z):
                for a, result in zip(slots(n), step(v, n, filt)):
                    t_store(a, rows, result)

    def filter_rows(cls, mb, f):
        block = pl.ds(pl.multiple_of(32 * mb, 32), 32)
        half, src = (_lo, _hi)[cls % 2], pl.ds(cls // 2, 8, stride=4)
        re, im = (half(ref.at[:, pl.ds(0, KH), :].bitcast(U32).at[f, block][src, :])
                  for ref in (wr, wi))
        if cls == 0:
            row = jax.lax.broadcasted_iota(jnp.int32, (8, LANES), 0)
            weight = jnp.where(row + mb == 0, 0.5, 1.0)
            re, im = re * weight, im * weight
        return re, im

    def filter_nyquist(f):
        return tuple(jnp.broadcast_to(ref[f, pl.ds(KH, 1), :].astype(F32), (8, LANES))
                     for ref in (wr, wi))

    for index in range(4):
        if index == 1:
            wait(cp_w)

        def middle(i, carry, index=index):
            pair = 2 * index + i
            precompute(w_v0[2 * pair], w_v0[2 * pair + 1], pre_v0, lambda n: 2 * pair + n)
            for n in range(4):
                mb = 4 * i + n
                for cls in range(8):
                    run_pass(index, 64 * K_CLASSES.index(cls) + 8 * mb,
                             functools.partial(filter_rows, cls, mb), 8 * n + cls)
            return carry

        jax.lax.fori_loop(0, 2, middle, 0)
        run_pass(index, KH, filter_nyquist, 0)

    def inverse(ap, beside):
        beside = list(beside)

        def sequence_idft(item):
            a, g, _ = item
            if g == 4:
                re, im = (jnp.concatenate([v] * (LANES // 8), axis=0)
                          for v in t_load(a, pl.ds(KH, 8)))
                return _dot_nt(ftw[a, 0], re + im) + _dot_nt(ftw[a, 1], im)
            re, im = t_load(a, pl.ds(g * LANES, LANES))
            both = _dot_nt(ftw[a, 0], re + im)
            return both + _dot_nt(ftw[a, 1], im), both - _dot_nt(ftw[a, 2], re)

        nyquist = {}
        low = jax.lax.broadcasted_iota(jnp.int32, (LANES, LANES), 1) < LANES // 2

        def feature_idft(item, v):
            a, g, par = item
            if g < 4:
                beside.pop(0)()
            if g == 4:
                nyquist[par] = v * (0.5 * tw[pl.ds(NYQ_ROW, 1), :])
            elif g == 0:
                re, im = v
                v0 = jnp.where(low, re, pltpu.roll(im, LANES // 2, 1))
                v1 = jnp.where(low, pltpu.roll(re, LANES // 2, 1), im)
                u_store(a, 0, _dot(v0, table(0, 0)) + nyquist.pop(par))
                u_store(a, 1, _dot(v1, table(0, 1)))
            else:
                re, im = v
                both = _dot(jnp.where(low, re - im, re + im), table(g, 0))
                u_store(a, 2 * g, both + _dot(im, table(g, 1)))
                u_store(a, 2 * g + 1, both - _dot(re, table(g, 2)))

        pipelined([(2 * ap + par, g, par) for par in range(2) for g in (4, 0, 1, 2, 3)],
                  sequence_idft, feature_idft, 3)

    def inverse_first(i, carry):
        inverse(i, [functools.partial(repack, 1, kt, w_q0, (hp, hp + 1))
                    for kt in (2 * i, 2 * i + 1) for hp in range(0, GROUP // 2, 2)])
        return carry

    def inverse_second(i, carry):
        inverse(RS // 4 + i, [functools.partial(repack_right, 2, i, (hp,), w_k0, (True, True))
                              for hp in range(GROUP // 2)])
        return carry

    wait(cp_piece[1])
    jax.lax.fori_loop(0, RS // 4, inverse_first, 0)
    wait(cp_piece[2])
    jax.lax.fori_loop(0, RS // 4, inverse_second, 0)

    def adjoint(ap):
        for b in range(0, LANES, 8):
            y = [_radix8_adj([u_load(2 * ap + par, n, b, 8) for n in range(RD)])
                 for par in range(2)]
            for j in range(RD):
                ua[RS + j, pl.ds(ap + 8 * b, 8, stride=8), :] = _pack(y[0][j], y[1][j])

    def fourth_piece(i, carry):
        for n in range(2):
            h = 2 * i + n
            work = [functools.partial(repack_right, 3, i // 2, (4 * (i % 2) + 2 * n + j,), w_v1,
                                      (False, True)) for j in range(2)]
            precompute(w_q0[h], w_k0[h], pre_qk0, lambda j: 2 * h + j, work)
        return carry

    wait(cp_piece[3])
    jax.lax.fori_loop(0, GROUP // 2, fourth_piece, 0)

    def last_pieces(i, carry):
        for n in range(2):
            pair = 2 * i + n
            work = [functools.partial(repack_right, 5, i, (4 * n + j, 4 * n + j + 1), w_k1,
                                      (True, True)) for j in (0, 2)]
            work.append(functools.partial(repack, 4, pair, w_q1))
            precompute(w_v1[2 * pair], w_v1[2 * pair + 1], pre_v1, lambda j: 2 * pair + j, work)
        return carry

    wait(cp_piece[4])
    wait(cp_piece[5])
    jax.lax.fori_loop(0, KT // 2, last_pieces, 0)

    def late(h):
        return raw.at[h // 8].reshape(D * GROUP // 2, LANES)

    def late_rows(h, i, first, n):
        return pl.ds(pl.multiple_of((2 * (h % 8) + i) * (8 * n_seg) + first, 8), n)

    def last_pairs(i, carry):
        adjoint(i)
        for h in (2 * i, 2 * i + 1):
            precompute(w_q1[h], w_k1[h], late(h), lambda n: late_rows(h, n, 0, 8 * n_seg))
        return carry

    jax.lax.fori_loop(0, GROUP // 2, last_pairs, 0)

    L = M + seg
    scale = E ** -0.5
    mem_rows = pl.ds(seg, M)

    def segment(s):
        hbuf[pl.ds(0, seg), :] = bx[s].astype(F32)
        qi = jax.lax.broadcasted_iota(jnp.int32, (L, L), 0)
        ki = jax.lax.broadcasted_iota(jnp.int32, (L, L), 1)
        mask = (qi >= seg) | (ki >= seg) | (qi >= ki)
        queries, keys, values, probs, ctx = {}, {}, {}, {}, {}

        n = seg - 16
        first, second = pl.ds(0, KH), pl.ds(KH, KH)
        plain, upper, top, bottom = pl.ds(0, n), pl.ds(0, n + 8), pl.ds(n, 8), pl.ds(n + 8, 8)
        total = hbuf[pl.ds(0, seg), first] + hbuf[pl.ds(0, seg), second]
        hsum[plain, :] = total[:n]
        hsum[top, :] = total[n:n + 8] - total[n + 8:]
        hsum[bottom, :] = hbuf[bottom, first] - hbuf[top, first]

        def weights(h, m):
            g, i = divmod(h, GROUP)
            ref = ((w_q0, w_k0, w_v0), (w_q1, w_k1, w_v1))[g][m]
            return pltpu.bitcast(ref[i], BF16)

        def ahead(h, m, i):
            g, j = divmod(h, GROUP)
            rows = pl.ds(pl.multiple_of(8 * s, 8), 8)
            if m == 2:
                v = (pre_v0, pre_v1)[g][j + i, rows, :]
            elif g == 0:
                v = pre_qk0[2 * j + i, rows, :]
            else:
                v = late(j)[late_rows(j, i, 8 * s, 8), :]
            return pltpu.bitcast(v, F32)

        def left(h, m):
            w = weights(h, m)
            return [_dot(jnp.concatenate([hbuf[upper, cols], hbuf[mem_rows, cols]], axis=0), v)
                    for cols, v in ((first, w[:KH]), (second, w[KH:]))]

        def right(h, m):
            w = weights(h, m)
            x = jnp.concatenate(
                [hbuf[plain, first], hsum[bottom, :], hbuf[mem_rows, first]], axis=0)
            y = jnp.concatenate([hsum[upper, :], hsum[mem_rows, :]], axis=0)
            return _dot(x, w[:KH]), _dot(y, w[KH:])

        def combine(h, m, l, r):
            c1, c2 = l[0] + l[1], r[0] + r[1]
            p1, p7, p3 = l[0][n:n + 8], r[0][n:n + 8], r[1][n:n + 8]
            u = p1 + ahead(h, m, 0)
            return (jnp.concatenate([c1[:n + 8], p1 + p7 + ahead(h, m, 1), c1[n + 8:]], axis=0),
                    jnp.concatenate([c2[:n], u + p3, u + p7, c2[n + 8:]], axis=0))

        def scores(h):
            sc = jnp.where(mask, _dot_nt(queries.pop(h), keys.pop(h)) * scale, -1000000000.0)
            e = jnp.exp(sc - jnp.max(sc, axis=-1, keepdims=True))
            probs[h] = e, jnp.sum(e, axis=-1, keepdims=True)

        def mix(h):
            e, norm = probs.pop(h)
            o = _dot(e, values.pop(h)) * (1.0 / norm)
            ctx[h] = jnp.concatenate([o[seg:], o[:seg]], axis=0)

        def output(h):
            rows = pl.ds(h * (E // 2), E // 2)
            w = jnp.concatenate([wo[j, rows, :] for j in range(RD)], axis=1)
            return _dot(ctx.pop(h), pltpu.bitcast(w, BF16))

        lag_scores, lag_mix, lag_output = 2, 6, 8
        acc = None
        for t in range(H + lag_output):
            if 0 <= t - lag_scores < H:
                scores(t - lag_scores)
            if t < H:
                q_parts = left(t, 0)
            if 0 <= t - lag_mix < H:
                mix(t - lag_mix)
            if t < H:
                queries[t], keys[t] = combine(t, 0, q_parts, right(t, 1))
                if t % 2 == 0:
                    v_parts = left(t, 2)
                else:
                    values[t - 1], values[t] = combine(t - 1, 2, v_parts, right(t, 2))
            if 0 <= t - lag_output < H:
                y = output(t - lag_output)
                acc = y if acc is None else acc + y
        hbuf[mem_rows, :] = acc[:M]
        hsum[mem_rows, :] = acc[:M, :KH] + acc[:M, KH:]
        yb[pl.ds(pl.multiple_of(s * seg, seg), seg), :] = acc[M:].astype(BF16)

    def yb_copy(i):
        rows = pl.ds(pl.multiple_of(i * (UNROLL * seg), UNROLL * seg), UNROLL * seg)
        return pltpu.make_async_copy(yb.at[rows], out_hbm.at[rows, pl.ds(D, D)], yb_sem)

    wait(cp_bx0)
    wait(cp_wo)
    hbuf[mem_rows, :] = mem0[...].astype(F32)
    hsum[mem_rows, :] = hbuf[mem_rows, pl.ds(0, KH)] + hbuf[mem_rows, pl.ds(KH, KH)]
    start(cp_bx1)
    start(cp_ya)

    def segments(i, carry):
        pl.when(i == 1)(functools.partial(wait, cp_bx1))

        @pl.when(i > 0)
        def _():
            yb_copy(i - 1).start()

        for u in range(UNROLL):
            segment(UNROLL * i + u)
        return carry

    jax.lax.fori_loop(0, n_seg // UNROLL, segments, 0)
    yb_copy(n_seg // UNROLL - 1).start()
    wait(cp_ya)
    pltpu.make_async_copy(yb, out_hbm.at[:, pl.ds(D, D)], yb_sem).wait()


@functools.partial(jax.jit, static_argnames=("B_seg_len",))
def pallas_concat_heads__spectral_gfnet__memory_aug_recurrent_mem_tr__prompt_kernel(
    A_x: jax.Array,
    A_w_r: jax.Array,
    A_w_i: jax.Array,
    B_x: jax.Array,
    B_mem0: jax.Array,
    B_Wq: jax.Array,
    B_Wk: jax.Array,
    B_Wv: jax.Array,
    B_Wo: jax.Array,
    B_seg_len: int,
):
    assert A_x.shape == (1, S, D) and B_x.shape == (1, S, D) and B_mem0.shape == (1, M, D)
    assert B_Wq.shape == (D, H, E) and B_Wo.shape == (H, E, D)
    seg = int(B_seg_len)
    n_seg = S // seg
    assert n_seg * seg == S and 8 * n_seg == D // 2
    mats, tw = _tables()
    vmem = pltpu.VMEM
    out = pl.pallas_call(
        functools.partial(_kernel, seg=seg, n_seg=n_seg),
        out_shape=jax.ShapeDtypeStruct((S, 2 * D), BF16),
        in_specs=[pl.BlockSpec(memory_space=pl.ANY)] * 11,
        out_specs=pl.BlockSpec(memory_space=pl.ANY),
        scratch_shapes=[
            vmem((RS + RD + GROUP, RD * LANES, LANES), U32),
            vmem((RS, KH + 1, LANES), BF16),
            vmem((RS, KH + 1, LANES), BF16),
            vmem((mats.shape[0] // 2, LANES), U32),
            vmem(tw.shape, F32),
            vmem((RS, 3, LANES, LANES), F32),
            vmem((3, RS, KROWS, LANES), U32),
            vmem((6, D, GROUP // 2, LANES), U32),
            vmem((3 * GROUP, D // 2, LANES), U32),
            vmem((3 * GROUP, D // 2, LANES), U32),
            vmem((RD, H * E // 2, LANES), U32),
            vmem((n_seg, seg, D), BF16),
            vmem((M, D), BF16),
            vmem((M + seg, D), F32),
            vmem((M + seg, KH), F32),
            vmem((S, D), BF16),
            vmem((n_seg, 16, D), BF16),
            vmem((3, 4 * n_seg, KH), U32),
            vmem((GROUP, 8 * n_seg, LANES), U32),
            pltpu.SMEM((32,), jnp.int32),
            pltpu.SemaphoreType.DMA((26,)),
        ],
        compiler_params=pltpu.CompilerParams(vmem_limit_bytes=120 * 1024 * 1024),
        name="gfnet_rmt",
    )(A_x.reshape(S, D), A_w_r.T, A_w_i.T, B_x.reshape(n_seg, seg, D), B_mem0.reshape(M, D),
      B_Wq, B_Wk, B_Wv, B_Wo.reshape(H * E, D), mats, tw)
    return out.reshape(1, S, 2 * D)
```
